```python
import jax
import jax.numpy as jnp

def _softmax(x, axis=-1):
    return jax.nn.softmax(x, axis=axis)

def _gelu(x):
    return jax.nn.gelu(x, approximate=True)

def _silu(x):
    return jax.nn.silu(x)

def _sigmoid(x):
    return jax.nn.sigmoid(x)

def _layernorm(x, axis=-1, eps=1e-05):
    m = jnp.mean(x, axis=axis, keepdims=True)
    v = jnp.var(x, axis=axis, keepdims=True)
    return (x - m) / jnp.sqrt(v + eps)

def _scatter_add(tgt, idx, src, axis=0):
    return tgt.at[idx].add(src)

def _segment_sum(src, seg, n):
    return jax.ops.segment_sum(src, seg, n)

class _Rng:

    def __init__(self, key):
        self._k = key

    def _next(self):
        self._k, sub = jax.random.split(self._k)
        return sub

    def normal(self, shape):
        return jax.random.normal(self._next(), shape, dtype=jnp.bfloat16)

    def randint(self, lo, hi, shape):
        return jax.random.randint(self._next(), shape, lo, hi, dtype=jnp.int32)

    def uniform(self, shape, lo=0.0, hi=1.0):
        return jax.random.uniform(self._next(), shape, jnp.bfloat16, lo, hi)

    def permutation(self, n):
        return jax.random.permutation(self._next(), n)
kernel_name = 'gated_mix__softmax_full_mha__memory_aug_recurrent_mem_tr__prompt'

def setup_inputs():
    _rng = _Rng(jax.random.key(int.from_bytes(__import__("os").urandom(4), "little")))
    _w = lambda a: (lambda t: t.astype(jnp.bfloat16) if jnp.issubdtype(t.dtype, jnp.floating) else t)(jnp.asarray(a))

    def _A_setup():
        B, S, D = (1, 2048, 1024)
        return {'x': _w((lambda *s: _rng.normal(s) * 0.05)(B, S, D)), 'wqkv': _w((lambda *s: _rng.normal(s) * 0.05)(D, 3 * D)), 'wo': _w((lambda *s: _rng.normal(s) * 0.05)(D, D))}
    _A_in = _A_setup()

    def _B_setup():
        B, S, Dm = (1, 2048, 1024)
        H, Dh = (32, 128)
        M, seg = (8, 32)
        seg = min(seg, S)
        S = S // seg * seg
        return {'x': _w((lambda *s: _rng.normal(s) * 0.05)(B, S, Dm)), 'mem0': _w((lambda *s: _rng.normal(s) * 0.05)(B, M, Dm)), 'Wq': _w((lambda *s: _rng.normal(s) * 0.05)(Dm, H, Dh) * Dm ** (-0.5)), 'Wk': _w((lambda *s: _rng.normal(s) * 0.05)(Dm, H, Dh) * Dm ** (-0.5)), 'Wv': _w((lambda *s: _rng.normal(s) * 0.05)(Dm, H, Dh) * Dm ** (-0.5)), 'Wo': _w((lambda *s: _rng.normal(s) * 0.05)(H, Dh, Dm) * (H * Dh) ** (-0.5)), 'seg_len': seg}
    _B_in = _B_setup()
    return {'A_x': _A_in['x'], 'A_wqkv': _A_in['wqkv'], 'A_wo': _A_in['wo'], 'B_x': _B_in['x'], 'B_mem0': _B_in['mem0'], 'B_Wq': _B_in['Wq'], 'B_Wk': _B_in['Wk'], 'B_Wv': _B_in['Wv'], 'B_Wo': _B_in['Wo'], 'B_seg_len': _B_in['seg_len'], 'gate_w': _w((lambda *s: _rng.normal(s) * 0.05)(1024))}

def reference(A_x, A_wqkv, A_wo, B_x, B_mem0, B_Wq, B_Wk, B_Wv, B_Wo, B_seg_len, gate_w):

    def _A_ref(x, wqkv, wo):
        B, S, D = x.shape
        H = 32
        Dh = D // H
        qkv = (lambda x, *d: x.transpose(*d))((x @ wqkv).reshape(B, S, 3, H, Dh), 2, 0, 3, 1, 4)
        q, k, v = (qkv[0], qkv[1], qkv[2])
        scale = Dh ** (-0.5)
        scores = jnp.einsum('bhqd,bhkd->bhqk', q, k) * scale
        p = _softmax(scores, axis=-1)
        o = jnp.einsum('bhqk,bhkd->bhqd', p, v)
        return (lambda x, *d: x.transpose(*d))(o, 0, 2, 1, 3).reshape(B, S, D) @ wo

    def _B_ref(x, mem0, Wq, Wk, Wv, Wo, seg_len):
        B, S, Dm = x.shape
        H, Dh = (Wq.shape[1], Wq.shape[2])
        M = mem0.shape[1]
        scale = Dh ** (-0.5)
        n_seg = S // seg_len
        L = M + seg_len
        idx = jnp.arange(L)
        mask = (idx[:, None] < M) | (idx[:, None] >= idx[None, :])
        mem = mem0
        outs = []
        for s in range(n_seg):
            xs = x[:, s * seg_len:(s + 1) * seg_len, :].copy()
            h = jnp.concatenate([mem, xs], axis=1)
            q = jnp.einsum('btd,dhe->bhte', h, Wq)
            k = jnp.einsum('btd,dhe->bhte', h, Wk)
            v = jnp.einsum('btd,dhe->bhte', h, Wv)
            scores = jnp.einsum('bhqe,bhke->bhqk', q, k) * scale
            scores = jnp.where(mask[None, None], scores, -1000000000.0)
            p = _softmax(scores, axis=-1)
            o = jnp.einsum('bhqk,bhke->bhqe', p, v)
            o = jnp.einsum('bhte,hed->btd', o, Wo)
            mem = o[:, :M, :].copy()
            outs.append(o[:, M:, :])
        return jnp.concatenate(outs, axis=1)
    x = A_x
    g = _sigmoid((x * gate_w).sum(-1, keepdims=True))
    a = _A_ref(x, A_wqkv, A_wo)
    b = _B_ref(x, B_mem0, B_Wq, B_Wk, B_Wv, B_Wo, B_seg_len)
    return g * a + (1 - g) * b
```

```python
import functools
import math

import jax
import jax.numpy as jnp
from jax import lax
import jax.experimental.pallas as pl
import jax.experimental.pallas.tpu as pltpu

F32 = jnp.float32
BF16 = jnp.bfloat16
U32 = jnp.uint32

LANES = 128
HA = 32
TQ = 512
TK = 256
TM = 256
L_MIN = 2.0 ** -64
L_MAX = 2.0 ** 64


def _dot(a, b):
    return lax.dot_general(a, b, (((1,), (0,)), ((), ())), preferred_element_type=F32)


def _dot_nt(a, b):
    return lax.dot_general(a, b, (((1,), (1,)), ((), ())), preferred_element_type=F32)


def _dot_tn(a, b):
    return lax.dot_general(a, b, (((0,), (0,)), ((), ())), preferred_element_type=F32)


def _make_kernel(S, D, HB, DHB, M, SEG):
    DHA = D // HA
    HPG = LANES // DHA
    NG = D // LANES
    L = M + SEG
    NSEG = S // SEG
    NQ = S // TQ
    NK = S // TK
    J = TQ // LANES
    NBLK = S // TM
    NPAIR = HB // 2
    KH = D // 2
    qscale = (DHA ** -0.5) * math.log2(math.e)
    bscale = DHB ** -0.5

    def kernel(xa_hbm, wqkv_hbm, woa_hbm, xb_hbm, mem_hbm, wq_hbm, wk_hbm, wv_hbm, wob_hbm, gate_hbm,
               out_hbm,
               xa, wqkv, woa, xb, mem, gate, wb, wob,
               qt, kk, vt, ot, kmax, kmt, lchk, gl, bbuf, hbuf, obuf, sbuf, outv,
               sem_in, sem_w, sem_wo, sem_out):
        cp_xa = pltpu.make_async_copy(xa_hbm.at[0], xa, sem_in.at[0])
        cp_wqkv = pltpu.make_async_copy(wqkv_hbm, wqkv, sem_in.at[1])
        cp_gate = pltpu.make_async_copy(gate_hbm, gate, sem_in.at[2])
        cp_woa = pltpu.make_async_copy(woa_hbm, woa, sem_in.at[3])
        cp_xb = pltpu.make_async_copy(xb_hbm.at[0], xb, sem_in.at[4])
        cp_mem = pltpu.make_async_copy(mem_hbm.at[0], mem, sem_in.at[5])
        cp_xa.start()
        cp_wqkv.start()
        cp_gate.start()

        def w_copies(t):
            src = (wq_hbm, wk_hbm, wv_hbm)[t].bitcast(U32)
            return [pltpu.make_async_copy(src.at[:, r, :], wb.at[t, 2 * (r % NPAIR) + r // NPAIR], sem_w.at[t * HB + r])
                    for r in range(HB)]

        w_cps = [w_copies(t) for t in range(3)]
        for t in range(3):
            for c in w_cps[t]:
                c.start()
        wob_u = wob_hbm.bitcast(U32)
        wo_cps = [pltpu.make_async_copy(wob_u.at[:, :, n * LANES:(n + 1) * LANES], wob.at[n], sem_wo.at[n])
                  for n in range(NG)]
        for c in wo_cps:
            c.start()
        cp_xb.start()
        cp_mem.start()
        cp_woa.start()

        cp_xa.wait()
        cp_wqkv.wait()
        cp_gate.wait()

        kmax[...] = jnp.zeros(kmax.shape, F32)

        def a_proj(i, carry):
            r0 = pl.multiple_of(i * TM, TM)
            xblk = xa[pl.ds(r0, TM), :]
            for c in range(3 * NG):
                r = _dot(xblk, wqkv[:, c * LANES:(c + 1) * LANES])
                if c < NG:
                    qt[c, :, pl.ds(r0, TM)] = (r * qscale).T.astype(BF16)
                elif c < 2 * NG:
                    g = c - NG
                    rb = r.astype(BF16)
                    kk[g, pl.ds(r0, TM), :] = rb
                    ab = jnp.abs(rb.astype(F32))
                    kmax[g] = jnp.maximum(kmax[g], jnp.max(ab.reshape(TM // 8, 8, LANES), axis=0))
                else:
                    g = c - 2 * NG
                    vt[g * LANES:(g + 1) * LANES, pl.ds(r0, TM)] = r.T.astype(BF16)
            logit = jnp.sum(xblk.astype(F32) * gate[...].astype(F32), axis=-1, keepdims=True)
            gl[pl.ds(r0, TM), :] = jnp.broadcast_to(jax.nn.sigmoid(logit), (TM, LANES))
            return carry

        lax.fori_loop(0, NBLK, a_proj, 0)

        for g in range(NG):
            km = jnp.max(kmax[g], axis=0, keepdims=True)
            kmt[g] = jnp.broadcast_to(km, (LANES, LANES)).T

        for t in range(3):
            for c in w_cps[t]:
                c.wait()

        def repack(i, carry):
            t = i // NPAIR
            j = i % NPAIR
            e = wb[t, 2 * j]
            o = wb[t, 2 * j + 1]
            wb[t, 2 * j] = (e & jnp.uint32(0xFFFF)) | (o << 16)
            wb[t, 2 * j + 1] = (e >> 16) | (o & jnp.uint32(0xFFFF0000))
            return carry

        lax.fori_loop(0, 3 * NPAIR, repack, 0)

        lchk[0] = jnp.full((8, LANES), L_MAX, F32)
        lchk[1] = jnp.full((8, LANES), L_MIN, F32)

        def head_masked_q(h, q0):
            g = h // HPG
            r = h % HPG
            rows = lax.broadcasted_iota(jnp.int32, (LANES, LANES), 0)
            msk = (rows >= r * DHA) & (rows < r * DHA + DHA)
            q = qt[g, :, pl.ds(q0, LANES)]
            return g, jnp.where(msk, q, jnp.zeros_like(q))

        def a_attn(it, carry):
            h = it // NQ
            qb = it % NQ
            h0 = pl.multiple_of(h * DHA, DHA)
            qms, bnd = [], []
            for j in range(J):
                q0 = pl.multiple_of(qb * TQ + j * LANES, LANES)
                g, qm = head_masked_q(h, q0)
                qms.append(qm)
                bb = jnp.abs(qm.astype(F32)) * kmt[g]
                bb = jnp.sum(bb, axis=0, keepdims=True) * (1.0 + 2.0 ** -10)
                bnd.append(jnp.broadcast_to(bb, (8, LANES)))
            ls = [jnp.zeros((8, LANES), F32) for _ in range(J)]
            accs = [jnp.zeros((DHA, LANES), F32) for _ in range(J)]
            ps = {}

            def qk(kb):
                kblk = kk[g, kb * TK:(kb + 1) * TK, :]
                for j in range(J):
                    s = _dot(kblk, qms[j]).reshape(TK // 8, 8, LANES)
                    p = jnp.exp2(s - bnd[j][None])
                    ls[j] = ls[j] + jnp.sum(p, axis=0)
                    ps[(kb, j)] = p.reshape(TK, LANES).astype(BF16)

            def pv(kb):
                vblk = vt[pl.ds(h0, DHA), kb * TK:(kb + 1) * TK]
                for j in range(J):
                    accs[j] = accs[j] + _dot(vblk, ps.pop((kb, j)))

            for kb in range(NK + 1):
                if kb < NK:
                    qk(kb)
                if kb >= 1:
                    pv(kb - 1)
            lo = lchk[0]
            hi = lchk[1]
            for j in range(J):
                l1 = jnp.sum(ls[j], axis=0, keepdims=True)
                l8 = jnp.broadcast_to(l1, (8, LANES))
                lo = jnp.where(l8 >= lo, lo, l8)
                hi = jnp.where(l8 <= hi, hi, l8)
                q0 = pl.multiple_of(qb * TQ + j * LANES, LANES)
                ot[pl.ds(h0, DHA), pl.ds(q0, LANES)] = (accs[j] / l1).astype(BF16)
            lchk[0] = lo
            lchk[1] = hi
            return carry

        lax.fori_loop(0, HA * NQ, a_attn, 0)

        ok = jnp.logical_and(lchk[0] >= L_MIN, lchk[1] <= L_MAX)
        n_bad = jnp.sum(jnp.where(ok, 0.0, 1.0))

        @pl.when(n_bad > 0.0)
        def _exact_softmax_fallback():
            def body(it, carry):
                h = it // (S // LANES)
                qb = it % (S // LANES)
                h0 = pl.multiple_of(h * DHA, DHA)
                q0 = pl.multiple_of(qb * LANES, LANES)
                g, qm = head_masked_q(h, q0)
                m = jnp.full((8, LANES), -jnp.inf, F32)
                for kb in range(NK):
                    s = _dot(kk[g, kb * TK:(kb + 1) * TK, :], qm)
                    sbuf[kb * TK:(kb + 1) * TK, :] = s
                    m = jnp.maximum(m, jnp.max(s.reshape(TK // 8, 8, LANES), axis=0))
                m1 = jnp.max(m, axis=0, keepdims=True)
                l = jnp.zeros((8, LANES), F32)
                acc = jnp.zeros((DHA, LANES), F32)
                for kb in range(NK):
                    p = jnp.exp2(sbuf[kb * TK:(kb + 1) * TK, :] - m1)
                    l = l + jnp.sum(p.reshape(TK // 8, 8, LANES), axis=0)
                    acc = acc + _dot(vt[pl.ds(h0, DHA), kb * TK:(kb + 1) * TK], p.astype(BF16))
                l1 = jnp.sum(l, axis=0, keepdims=True)
                ot[pl.ds(h0, DHA), pl.ds(q0, LANES)] = (acc / l1).astype(BF16)
                return carry

            lax.fori_loop(0, HA * (S // LANES), body, 0)

        for c in wo_cps:
            c.wait()
        cp_xb.wait()
        cp_mem.wait()
        hbuf[0:M, :] = mem[...].astype(F32)

        def b_step(s, carry):
            row = lax.broadcasted_iota(jnp.int32, (L, L), 0)
            col = lax.broadcasted_iota(jnp.int32, (L, L), 1)
            mask = (row < M) | (row >= col)
            r0 = pl.multiple_of(s * SEG, SEG)
            hbuf[M:L, :] = xb[pl.ds(r0, SEG), :].astype(F32)
            X = hbuf[...]
            qkv, ps, os_ = {}, {}, {}
            outs = [None] * NG
            GRP = 8

            def proj(h):
                qkv[h] = [_dot(X, pltpu.bitcast(wb[t, h], BF16)) for t in range(3)]

            def qk(h):
                q, k, _ = qkv[h]
                sc = _dot_nt(q, k.astype(BF16)) * bscale
                sc = jnp.where(mask, sc, -1e9)
                m = jnp.max(sc, axis=-1, keepdims=True)
                p = jnp.exp(sc - m)
                ps[h] = p / jnp.sum(p, axis=-1, keepdims=True)

            def pv(h):
                v = qkv.pop(h)[2]
                os_[h] = _dot(ps.pop(h), v.astype(BF16))

            def outp(h):
                o = os_.pop(h)
                for n in range(NG):
                    t = _dot(o, pltpu.bitcast(wob[n, h], BF16))
                    outs[n] = t if outs[n] is None else outs[n] + t
                if h % GRP == GRP - 1:
                    for n in range(NG):
                        if h == GRP - 1:
                            obuf[:, n * LANES:(n + 1) * LANES] = outs[n]
                        else:
                            obuf[:, n * LANES:(n + 1) * LANES] += outs[n]
                        outs[n] = None

            for t in range(HB + 3):
                if t < HB:
                    proj(t)
                if 0 <= t - 1 < HB:
                    qk(t - 1)
                if 0 <= t - 2 < HB:
                    pv(t - 2)
                if 0 <= t - 3 < HB:
                    outp(t - 3)
            o = obuf[...]
            hbuf[0:M, :] = o[0:M].astype(BF16).astype(F32)
            bbuf[pl.ds(r0, SEG), :] = o[M:L]
            return carry

        lax.fori_loop(0, NSEG, b_step, 0)

        cp_woa.wait()

        def out_copy(i):
            r0 = pl.multiple_of(i * TM, TM)
            return pltpu.make_async_copy(outv.at[pl.ds(r0, TM), :], out_hbm.at[0, pl.ds(r0, TM), :], sem_out.at[i])

        def final(i, carry):
            r0 = pl.multiple_of(i * TM, TM)
            a = _dot_tn(ot[:, pl.ds(r0, TM)], woa[...])
            g = gl[pl.ds(r0, TM), :]
            for n in range(NG):
                sl = slice(n * LANES, (n + 1) * LANES)
                outv[pl.ds(r0, TM), sl] = (g * a[:, sl] + (1.0 - g) * bbuf[pl.ds(r0, TM), sl]).astype(BF16)
            out_copy(i).start()
            return carry

        lax.fori_loop(0, NBLK, final, 0)
        for i in range(NBLK):
            out_copy(i).wait()

    return kernel


@functools.partial(jax.jit, static_argnames=("B_seg_len",))
def pallas_gated_mix__softmax_full_mha__memory_aug_recurrent_mem_tr__prompt_kernel(
    A_x: jax.Array,
    A_wqkv: jax.Array,
    A_wo: jax.Array,
    B_x: jax.Array,
    B_mem0: jax.Array,
    B_Wq: jax.Array,
    B_Wk: jax.Array,
    B_Wv: jax.Array,
    B_Wo: jax.Array,
    B_seg_len: int,
    gate_w: jax.Array,
):
    _, S, D = A_x.shape
    _, HB, DHB = B_Wq.shape
    M = B_mem0.shape[1]
    SEG = int(B_seg_len)
    NG = D // LANES
    wq, wk, wv = (w.reshape(D // 2, 2 * HB, DHB) for w in (B_Wq, B_Wk, B_Wv))
    gate = gate_w.reshape(1, D)

    any_spec = pl.BlockSpec(memory_space=pl.ANY)
    scratch = [
        pltpu.VMEM((S, D), BF16),
        pltpu.VMEM((D, 3 * D), BF16),
        pltpu.VMEM((D, D), BF16),
        pltpu.VMEM((S, D), BF16),
        pltpu.VMEM((M, D), BF16),
        pltpu.VMEM((1, D), BF16),
        pltpu.VMEM((3, HB, D // 2, DHB), U32),
        pltpu.VMEM((NG, HB, DHB // 2, LANES), U32),
        pltpu.VMEM((NG, LANES, S), BF16),
        pltpu.VMEM((NG, S, LANES), BF16),
        pltpu.VMEM((D, S), BF16),
        pltpu.VMEM((D, S), BF16),
        pltpu.VMEM((NG, 8, LANES), F32),
        pltpu.VMEM((NG, LANES, LANES), F32),
        pltpu.VMEM((2, 8, LANES), F32),
        pltpu.VMEM((S, LANES), F32),
        pltpu.VMEM((S, D), F32),
        pltpu.VMEM((M + SEG, D), F32),
        pltpu.VMEM((M + SEG, D), F32),
        pltpu.VMEM((S, LANES), F32),
        pltpu.VMEM((S, D), BF16),
        pltpu.SemaphoreType.DMA((6,)),
        pltpu.SemaphoreType.DMA((3 * HB,)),
        pltpu.SemaphoreType.DMA((NG,)),
        pltpu.SemaphoreType.DMA((S // TM,)),
    ]
    return pl.pallas_call(
        _make_kernel(S, D, HB, DHB, M, SEG),
        out_shape=jax.ShapeDtypeStruct((1, S, D), BF16),
        in_specs=[any_spec] * 10,
        out_specs=any_spec,
        scratch_shapes=scratch,
        compiler_params=pltpu.CompilerParams(vmem_limit_bytes=120 * 1024 * 1024),
        name="gated_mix",
    )(A_x, A_wqkv, A_wo, B_x, B_mem0, wq, wk, wv, B_Wo, gate)
```

```python
import functools
import math

import jax
import jax.numpy as jnp
from jax import lax
import jax.experimental.pallas as pl
import jax.experimental.pallas.tpu as pltpu

F32 = jnp.float32
BF16 = jnp.bfloat16
U32 = jnp.uint32

LANES = 128
HA = 32
TQ = 512
TK = 256
TM = 256
WCH = 4
L_MIN = 2.0 ** -64
L_MAX = 2.0 ** 64


def _dot(a, b):
    return lax.dot_general(a, b, (((1,), (0,)), ((), ())), preferred_element_type=F32)


def _dot_nt(a, b):
    return lax.dot_general(a, b, (((1,), (1,)), ((), ())), preferred_element_type=F32)


def _dot_tn(a, b):
    return lax.dot_general(a, b, (((0,), (0,)), ((), ())), preferred_element_type=F32)


def _make_kernel(S, D, HB, DHB, M, SEG):
    DHA = D // HA
    HPG = LANES // DHA
    NG = D // LANES
    L = M + SEG
    NSEG = S // SEG
    NQ = S // TQ
    NK = S // TK
    J = TQ // LANES
    NBLK = S // TM
    NPAIR = HB // 2
    NWCH = 3 * NG // WCH
    QPS = HA * NQ // NSEG
    assert QPS * NSEG == HA * NQ and NQ % QPS == 0
    REP0 = NBLK - 3
    qscale = (DHA ** -0.5) * math.log2(math.e)
    bscale = DHB ** -0.5

    def kernel(xa_hbm, wqkv_hbm, woa_hbm, xb_hbm, mem_hbm, wq_hbm, wk_hbm, wv_hbm, wob_hbm, gate_hbm,
               out_hbm,
               xa, wqkv, woa, xb, mem, gate, wb, wob,
               qt, kk, vt, ot, kmax, kmt, lchk, gl, bbuf, hbuf, obuf, sbuf, outv,
               sem_x, sem_wa, sem_in, sem_w, sem_wo, sem_out):
        cp_x0 = pltpu.make_async_copy(xa_hbm.at[0, 0:TM, :], xa.at[0:TM, :], sem_x.at[0])
        cp_xr = pltpu.make_async_copy(xa_hbm.at[0, TM:S, :], xa.at[TM:S, :], sem_x.at[1])
        cw = WCH * LANES
        cp_wa = [pltpu.make_async_copy(wqkv_hbm.at[:, k * cw:(k + 1) * cw], wqkv.at[:, k * cw:(k + 1) * cw],
                                       sem_wa.at[k]) for k in range(NWCH)]
        cp_gate = pltpu.make_async_copy(gate_hbm, gate, sem_in.at[0])
        cp_woa = pltpu.make_async_copy(woa_hbm, woa, sem_in.at[1])
        cp_xb = pltpu.make_async_copy(xb_hbm.at[0], xb, sem_in.at[2])
        cp_mem = pltpu.make_async_copy(mem_hbm.at[0], mem, sem_in.at[3])

        def w_copies(t):
            src = (wq_hbm, wk_hbm, wv_hbm)[t].bitcast(U32)
            return [pltpu.make_async_copy(src.at[:, r, :], wb.at[t, 2 * (r % NPAIR) + r // NPAIR],
                                          sem_w.at[t * HB + r]) for r in range(HB)]

        w_cps = [w_copies(t) for t in range(3)]
        wob_u = wob_hbm.bitcast(U32)
        wo_cps = [pltpu.make_async_copy(wob_u.at[:, :, n * LANES:(n + 1) * LANES], wob.at[n], sem_wo.at[n])
                  for n in range(NG)]

        cp_x0.start()
        cp_gate.start()
        for c in cp_wa:
            c.start()
        cp_xr.start()

        kmax[...] = jnp.zeros(kmax.shape, F32)

        def repack(t, j):
            e = wb[t, 2 * j]
            o = wb[t, 2 * j + 1]
            wb[t, 2 * j] = (e & jnp.uint32(0xFFFF)) | (o << 16)
            wb[t, 2 * j + 1] = (e >> 16) | (o & jnp.uint32(0xFFFF0000))

        def a_proj(i, first=False, rep=False):
            r0 = 0 if first else pl.multiple_of(i * TM, TM)
            xblk = xa[pl.ds(r0, TM), :]
            for c in range(3 * NG):
                if first and c % WCH == 0:
                    cp_wa[c // WCH].wait()
                r = _dot(xblk, wqkv[:, c * LANES:(c + 1) * LANES])
                if c < NG:
                    qt[c, :, pl.ds(r0, TM)] = (r * qscale).T.astype(BF16)
                elif c < 2 * NG:
                    g = c - NG
                    rb = r.astype(BF16)
                    kk[g, pl.ds(r0, TM), :] = rb
                    ab = jnp.abs(rb.astype(F32))
                    kmax[g] = jnp.maximum(kmax[g], jnp.max(ab.reshape(TM // 8, 8, LANES), axis=0))
                else:
                    g = c - 2 * NG
                    vt[g * LANES:(g + 1) * LANES, pl.ds(r0, TM)] = r.T.astype(BF16)
                if rep and c < NPAIR:
                    repack(i - REP0, c)
            logit = jnp.sum(xblk.astype(F32) * gate[...].astype(F32), axis=-1, keepdims=True)
            gl[pl.ds(r0, TM), :] = jnp.broadcast_to(jax.nn.sigmoid(logit), (TM, LANES))

        cp_x0.wait()
        cp_gate.wait()
        for c in w_cps[0]:
            c.start()
        a_proj(0, first=True)
        cp_xr.wait()

        def a_proj_mid(i, carry):
            @pl.when(i == 1)
            def _():
                for c in w_cps[1]:
                    c.start()

            @pl.when(i == 2)
            def _():
                for c in w_cps[2]:
                    c.start()

            @pl.when(i == 3)
            def _():
                for c in wo_cps:
                    c.start()
                cp_xb.start()
                cp_mem.start()
                cp_woa.start()

            a_proj(i)
            return carry

        lax.fori_loop(1, REP0, a_proj_mid, 0)
        for t in range(3):
            for c in w_cps[t]:
                c.wait()

        def a_proj_rep(i, carry):
            a_proj(i, rep=True)
            return carry

        lax.fori_loop(REP0, NBLK, a_proj_rep, 0)

        for g in range(NG):
            km = jnp.max(kmax[g], axis=0, keepdims=True)
            kmt[g] = jnp.broadcast_to(km, (LANES, LANES)).T

        lchk[0] = jnp.full((8, LANES), L_MAX, F32)
        lchk[1] = jnp.full((8, LANES), L_MIN, F32)

        for c in wo_cps:
            c.wait()
        cp_xb.wait()
        cp_mem.wait()
        hbuf[0:M, :] = mem[...].astype(F32)

        def head_masked_q(h, q0):
            g = h // HPG
            r = h % HPG
            rows = lax.broadcasted_iota(jnp.int32, (LANES, LANES), 0)
            msk = (rows >= r * DHA) & (rows < r * DHA + DHA)
            q = qt[g, :, pl.ds(q0, LANES)]
            return g, jnp.where(msk, q, jnp.zeros_like(q))

        def a_units(h, qb):
            st = {}
            h0 = pl.multiple_of(h * DHA, DHA)

            def setup():
                st["qms"], st["bnd"] = [], []
                for j in range(J):
                    q0 = pl.multiple_of(qb * TQ + j * LANES, LANES)
                    g, qm = head_masked_q(h, q0)
                    st["g"] = g
                    st["qms"].append(qm)
                    bb = jnp.abs(qm.astype(F32)) * kmt[g]
                    bb = jnp.sum(bb, axis=0, keepdims=True) * (1.0 + 2.0 ** -10)
                    st["bnd"].append(jnp.broadcast_to(bb, (8, LANES)))
                st["ls"] = [jnp.zeros((8, LANES), F32) for _ in range(J)]
                st["accs"] = [jnp.zeros((DHA, LANES), F32) for _ in range(J)]
                st["ps"] = {}

            def qk(kb):
                kblk = kk[st["g"], kb * TK:(kb + 1) * TK, :]
                for j in range(J):
                    s = _dot(kblk, st["qms"][j]).reshape(TK // 8, 8, LANES)
                    p = jnp.exp2(s - st["bnd"][j][None])
                    st["ls"][j] = st["ls"][j] + jnp.sum(p, axis=0)
                    st["ps"][(kb, j)] = p.reshape(TK, LANES).astype(BF16)

            def pv(kb):
                vblk = vt[pl.ds(h0, DHA), kb * TK:(kb + 1) * TK]
                for j in range(J):
                    st["accs"][j] = st["accs"][j] + _dot(vblk, st["ps"].pop((kb, j)))

            def finish():
                lo = lchk[0]
                hi = lchk[1]
                for j in range(J):
                    l1 = jnp.sum(st["ls"][j], axis=0, keepdims=True)
                    l8 = jnp.broadcast_to(l1, (8, LANES))
                    lo = jnp.where(l8 >= lo, lo, l8)
                    hi = jnp.where(l8 <= hi, hi, l8)
                    q0 = pl.multiple_of(qb * TQ + j * LANES, LANES)
                    ot[pl.ds(h0, DHA), pl.ds(q0, LANES)] = (st["accs"][j] / l1).astype(BF16)
                lchk[0] = lo
                lchk[1] = hi

            def unit(kb):
                def f():
                    if kb == 0:
                        setup()
                    if kb < NK:
                        qk(kb)
                    if kb >= 1:
                        pv(kb - 1)
                    if kb == NK:
                        finish()
                return f

            return [unit(kb) for kb in range(NK + 1)]

        def b_slots(s):
            st = {"qkv": {}, "ps": {}, "os": {}, "outs": [None] * NG}
            r0 = pl.multiple_of(s * SEG, SEG)
            GRP = 8

            def setup():
                hbuf[M:L, :] = xb[pl.ds(r0, SEG), :].astype(F32)
                st["X"] = hbuf[...]
                row = lax.broadcasted_iota(jnp.int32, (L, L), 0)
                col = lax.broadcasted_iota(jnp.int32, (L, L), 1)
                st["mask"] = (row < M) | (row >= col)

            def proj(h):
                st["qkv"][h] = [_dot(st["X"], pltpu.bitcast(wb[t, h], BF16)) for t in range(3)]

            def qk(h):
                q, k, _ = st["qkv"][h]
                sc = _dot_nt(q, k.astype(BF16)) * bscale
                sc = jnp.where(st["mask"], sc, -1e9)
                m = jnp.max(sc, axis=-1, keepdims=True)
                p = jnp.exp(sc - m)
                st["ps"][h] = p / jnp.sum(p, axis=-1, keepdims=True)

            def pv(h):
                v = st["qkv"].pop(h)[2]
                st["os"][h] = _dot(st["ps"].pop(h), v.astype(BF16))

            def outp(h):
                o = st["os"].pop(h)
                outs = st["outs"]
                for n in range(NG):
                    t = _dot(o, pltpu.bitcast(wob[n, h], BF16))
                    outs[n] = t if outs[n] is None else outs[n] + t
                if h % GRP == GRP - 1:
                    for n in range(NG):
                        if h == GRP - 1:
                            obuf[:, n * LANES:(n + 1) * LANES] = outs[n]
                        else:
                            obuf[:, n * LANES:(n + 1) * LANES] += outs[n]
                        outs[n] = None

            def finish():
                o = obuf[...]
                hbuf[0:M, :] = o[0:M].astype(BF16).astype(F32)
                bbuf[pl.ds(r0, SEG), :] = o[M:L]

            def slot(t):
                def f():
                    if t == 0:
                        setup()
                    if t < HB:
                        proj(t)
                    if 0 <= t - 1 < HB:
                        qk(t - 1)
                    if 0 <= t - 2 < HB:
                        pv(t - 2)
                    if 0 <= t - 3 < HB:
                        outp(t - 3)
                    if t == HB + 2:
                        finish()
                return f

            return [slot(t) for t in range(HB + 3)]

        def main_step(s, carry):
            h = s * QPS // NQ
            qb0 = (s * QPS) % NQ
            units = []
            for i in range(QPS):
                u = a_units(h, qb0 + i)
                if units:
                    last = units.pop()
                    first = u[0]
                    u = [lambda a=first, b=last: (a(), b())] + u[1:]
                units += u
            slots = b_slots(s)
            ns, nu = len(slots), len(units)
            pos = [ns - 2 - 2 * (nu - 2 - i) if i < nu - 1 else ns - 2 for i in range(nu)]
            pos = [ns - 3 - 2 * (nu - 2 - i) for i in range(nu - 1)] + [ns - 2]
            for t in range(ns):
                slots[t]()
                for i in range(nu):
                    if max(pos[i], 0) == t:
                        units[i]()
            return carry

        lax.fori_loop(0, NSEG, main_step, 0)

        ok = jnp.logical_and(lchk[0] >= L_MIN, lchk[1] <= L_MAX)
        n_bad = jnp.sum(jnp.where(ok, 0.0, 1.0))

        @pl.when(n_bad > 0.0)
        def _exact_softmax_fallback():
            def body(it, carry):
                h = it // (S // LANES)
                qb = it % (S // LANES)
                h0 = pl.multiple_of(h * DHA, DHA)
                q0 = pl.multiple_of(qb * LANES, LANES)
                g, qm = head_masked_q(h, q0)
                m = jnp.full((8, LANES), -jnp.inf, F32)
                for kb in range(NK):
                    s = _dot(kk[g, kb * TK:(kb + 1) * TK, :], qm)
                    sbuf[kb * TK:(kb + 1) * TK, :] = s
                    m = jnp.maximum(m, jnp.max(s.reshape(TK // 8, 8, LANES), axis=0))
                m1 = jnp.max(m, axis=0, keepdims=True)
                l = jnp.zeros((8, LANES), F32)
                acc = jnp.zeros((DHA, LANES), F32)
                for kb in range(NK):
                    p = jnp.exp2(sbuf[kb * TK:(kb + 1) * TK, :] - m1)
                    l = l + jnp.sum(p.reshape(TK // 8, 8, LANES), axis=0)
                    acc = acc + _dot(vt[pl.ds(h0, DHA), kb * TK:(kb + 1) * TK], p.astype(BF16))
                l1 = jnp.sum(l, axis=0, keepdims=True)
                ot[pl.ds(h0, DHA), pl.ds(q0, LANES)] = (acc / l1).astype(BF16)
                return carry

            lax.fori_loop(0, HA * (S // LANES), body, 0)

        cp_woa.wait()

        def out_copy(i):
            r0 = pl.multiple_of(i * TM, TM)
            return pltpu.make_async_copy(outv.at[pl.ds(r0, TM), :], out_hbm.at[0, pl.ds(r0, TM), :], sem_out.at[i])

        def final(i, carry):
            r0 = pl.multiple_of(i * TM, TM)
            a = _dot_tn(ot[:, pl.ds(r0, TM)], woa[...])
            g = gl[pl.ds(r0, TM), :]
            for n in range(NG):
                sl = slice(n * LANES, (n + 1) * LANES)
                outv[pl.ds(r0, TM), sl] = (g * a[:, sl] + (1.0 - g) * bbuf[pl.ds(r0, TM), sl]).astype(BF16)
            out_copy(i).start()
            return carry

        lax.fori_loop(0, NBLK, final, 0)
        for i in range(NBLK):
            out_copy(i).wait()

    return kernel


@functools.partial(jax.jit, static_argnames=("B_seg_len",))
def pallas_gated_mix__softmax_full_mha__memory_aug_recurrent_mem_tr__prompt_kernel(
    A_x: jax.Array,
    A_wqkv: jax.Array,
    A_wo: jax.Array,
    B_x: jax.Array,
    B_mem0: jax.Array,
    B_Wq: jax.Array,
    B_Wk: jax.Array,
    B_Wv: jax.Array,
    B_Wo: jax.Array,
    B_seg_len: int,
    gate_w: jax.Array,
):
    _, S, D = A_x.shape
    _, HB, DHB = B_Wq.shape
    M = B_mem0.shape[1]
    SEG = int(B_seg_len)
    NG = D // LANES
    wq, wk, wv = (w.reshape(D // 2, 2 * HB, DHB) for w in (B_Wq, B_Wk, B_Wv))
    gate = gate_w.reshape(1, D)

    any_spec = pl.BlockSpec(memory_space=pl.ANY)
    scratch = [
        pltpu.VMEM((S, D), BF16),
        pltpu.VMEM((D, 3 * D), BF16),
        pltpu.VMEM((D, D), BF16),
        pltpu.VMEM((S, D), BF16),
        pltpu.VMEM((M, D), BF16),
        pltpu.VMEM((1, D), BF16),
        pltpu.VMEM((3, HB, D // 2, DHB), U32),
        pltpu.VMEM((NG, HB, DHB // 2, LANES), U32),
        pltpu.VMEM((NG, LANES, S), BF16),
        pltpu.VMEM((NG, S, LANES), BF16),
        pltpu.VMEM((D, S), BF16),
        pltpu.VMEM((D, S), BF16),
        pltpu.VMEM((NG, 8, LANES), F32),
        pltpu.VMEM((NG, LANES, LANES), F32),
        pltpu.VMEM((2, 8, LANES), F32),
        pltpu.VMEM((S, LANES), F32),
        pltpu.VMEM((S, D), F32),
        pltpu.VMEM((M + SEG, D), F32),
        pltpu.VMEM((M + SEG, D), F32),
        pltpu.VMEM((S, LANES), F32),
        pltpu.VMEM((S, D), BF16),
        pltpu.SemaphoreType.DMA((2,)),
        pltpu.SemaphoreType.DMA((3 * NG // WCH,)),
        pltpu.SemaphoreType.DMA((4,)),
        pltpu.SemaphoreType.DMA((3 * HB,)),
        pltpu.SemaphoreType.DMA((NG,)),
        pltpu.SemaphoreType.DMA((S // TM,)),
    ]
    return pl.pallas_call(
        _make_kernel(S, D, HB, DHB, M, SEG),
        out_shape=jax.ShapeDtypeStruct((1, S, D), BF16),
        in_specs=[any_spec] * 10,
        out_specs=any_spec,
        scratch_shapes=scratch,
        compiler_params=pltpu.CompilerParams(vmem_limit_bytes=120 * 1024 * 1024),
        name="gated_mix",
    )(A_x, A_wqkv, A_wo, B_x, B_mem0, wq, wk, wv, B_Wo, gate)
```

```python
import functools
import math

import jax
import jax.numpy as jnp
from jax import lax
import jax.experimental.pallas as pl
import jax.experimental.pallas.tpu as pltpu

F32 = jnp.float32
BF16 = jnp.bfloat16
U32 = jnp.uint32

LANES = 128
HA = 32
TQ = 512
TK = 256
TM = 256
WCH = 4
L_MIN = 2.0 ** -64
L_MAX = 2.0 ** 64
SKEW = (1, 3, 5)
GRP = 8
A_SKEW = 1
A_END = 4
A_STRIDE = 2


def _dot(a, b):
    return lax.dot_general(a, b, (((1,), (0,)), ((), ())), preferred_element_type=F32)


def _dot_nt(a, b):
    return lax.dot_general(a, b, (((1,), (1,)), ((), ())), preferred_element_type=F32)


def _dot_tn(a, b):
    return lax.dot_general(a, b, (((0,), (0,)), ((), ())), preferred_element_type=F32)


def _make_kernel(S, D, HB, DHB, M, SEG):
    DHA = D // HA
    HPG = LANES // DHA
    NG = D // LANES
    L = M + SEG
    NSEG = S // SEG
    NQ = S // TQ
    NK = S // TK
    J = TQ // LANES
    NBLK = S // TM
    NPAIR = HB // 2
    NWCH = 3 * NG // WCH
    QPS = HA * NQ // NSEG
    assert QPS * NSEG == HA * NQ and NQ % QPS == 0
    REP0 = NBLK - 3
    qscale = (DHA ** -0.5) * math.log2(math.e)
    bscale = DHB ** -0.5

    def kernel(xa_hbm, wqkv_hbm, woa_hbm, xb_hbm, mem_hbm, wq_hbm, wk_hbm, wv_hbm, wob_hbm, gate_hbm,
               out_hbm,
               xa, wqkv, woa, xb, mem, gate, wb, wob,
               qt, kk, vt, ot, kmax, kmt, lchk, gl, bbuf, hbuf, obuf, sbuf, outv,
               sem_x, sem_wa, sem_in, sem_w, sem_wo, sem_out):
        cp_x0 = pltpu.make_async_copy(xa_hbm.at[0, 0:TM, :], xa.at[0:TM, :], sem_x.at[0])
        cp_xr = pltpu.make_async_copy(xa_hbm.at[0, TM:S, :], xa.at[TM:S, :], sem_x.at[1])
        cw = WCH * LANES
        cp_wa = [pltpu.make_async_copy(wqkv_hbm.at[:, k * cw:(k + 1) * cw], wqkv.at[:, k * cw:(k + 1) * cw],
                                       sem_wa.at[k]) for k in range(NWCH)]
        cp_gate = pltpu.make_async_copy(gate_hbm, gate, sem_in.at[0])
        cp_woa = pltpu.make_async_copy(woa_hbm, woa, sem_in.at[1])
        cp_xb = pltpu.make_async_copy(xb_hbm.at[0], xb, sem_in.at[2])
        cp_mem = pltpu.make_async_copy(mem_hbm.at[0], mem, sem_in.at[3])

        def w_copies(t):
            src = (wq_hbm, wk_hbm, wv_hbm)[t].bitcast(U32)
            return [pltpu.make_async_copy(src.at[:, r, :], wb.at[t, 2 * (r % NPAIR) + r // NPAIR],
                                          sem_w.at[t * HB + r]) for r in range(HB)]

        w_cps = [w_copies(t) for t in range(3)]
        wob_u = wob_hbm.bitcast(U32)
        wo_cps = [pltpu.make_async_copy(wob_u.at[:, :, n * LANES:(n + 1) * LANES], wob.at[n], sem_wo.at[n])
                  for n in range(NG)]

        cp_x0.start()
        cp_gate.start()
        for c in cp_wa:
            c.start()
        cp_xr.start()

        kmax[...] = jnp.zeros(kmax.shape, F32)

        def repack(t, j):
            RC = 32
            for r in range(0, D // 2, RC):
                e = wb[t, 2 * j, r:r + RC, :]
                o = wb[t, 2 * j + 1, r:r + RC, :]
                wb[t, 2 * j, r:r + RC, :] = (e & jnp.uint32(0xFFFF)) | (o << 16)
                wb[t, 2 * j + 1, r:r + RC, :] = (e >> 16) | (o & jnp.uint32(0xFFFF0000))

        def a_proj(i, first=False, rep=False):
            r0 = 0 if first else pl.multiple_of(i * TM, TM)
            xblk = xa[pl.ds(r0, TM), :]
            for c in range(3 * NG):
                if first and c % WCH == 0:
                    cp_wa[c // WCH].wait()
                r = _dot(xblk, wqkv[:, c * LANES:(c + 1) * LANES])
                if c < NG:
                    qt[c, :, pl.ds(r0, TM)] = (r * qscale).T.astype(BF16)
                elif c < 2 * NG:
                    g = c - NG
                    rb = r.astype(BF16)
                    kk[g, pl.ds(r0, TM), :] = rb
                    ab = jnp.abs(rb.astype(F32))
                    kmax[g] = jnp.maximum(kmax[g], jnp.max(ab.reshape(TM // 8, 8, LANES), axis=0))
                else:
                    g = c - 2 * NG
                    vt[g * LANES:(g + 1) * LANES, pl.ds(r0, TM)] = r.T.astype(BF16)
                if rep and c < NPAIR:
                    repack(i - REP0, c)
            logit = jnp.sum(xblk.astype(F32) * gate[...].astype(F32), axis=-1, keepdims=True)
            gl[pl.ds(r0, TM), :] = jnp.broadcast_to(jax.nn.sigmoid(logit), (TM, LANES))

        cp_x0.wait()
        cp_gate.wait()
        for c in w_cps[0]:
            c.start()
        a_proj(0, first=True)
        cp_xr.wait()

        def a_proj_mid(i, carry):
            @pl.when(i == 1)
            def _():
                for c in w_cps[1]:
                    c.start()

            @pl.when(i == 2)
            def _():
                for c in w_cps[2]:
                    c.start()

            @pl.when(i == 3)
            def _():
                for c in wo_cps:
                    c.start()
                cp_xb.start()
                cp_mem.start()
                cp_woa.start()

            a_proj(i)
            return carry

        lax.fori_loop(1, REP0, a_proj_mid, 0)
        for t in range(3):
            for c in w_cps[t]:
                c.wait()

        def a_proj_rep(i, carry):
            a_proj(i, rep=True)
            return carry

        lax.fori_loop(REP0, NBLK, a_proj_rep, 0)

        for g in range(NG):
            km = jnp.max(kmax[g], axis=0, keepdims=True)
            kmt[g] = jnp.broadcast_to(km, (LANES, LANES)).T

        lchk[0] = jnp.full((8, LANES), L_MAX, F32)
        lchk[1] = jnp.full((8, LANES), L_MIN, F32)

        for c in wo_cps:
            c.wait()
        cp_xb.wait()
        cp_mem.wait()
        hbuf[0:M, :] = mem[...].astype(F32)

        def head_masked_q(h, q0):
            g = h // HPG
            r = h % HPG
            rows = lax.broadcasted_iota(jnp.int32, (LANES, LANES), 0)
            msk = (rows >= r * DHA) & (rows < r * DHA + DHA)
            q = qt[g, :, pl.ds(q0, LANES)]
            return g, jnp.where(msk, q, jnp.zeros_like(q))

        def a_units(h, qb):
            st = {}
            h0 = pl.multiple_of(h * DHA, DHA)

            def setup():
                st["qms"], st["bnd"] = [], []
                for j in range(J):
                    q0 = pl.multiple_of(qb * TQ + j * LANES, LANES)
                    g, qm = head_masked_q(h, q0)
                    st["g"] = g
                    st["qms"].append(qm)
                    bb = jnp.abs(qm.astype(F32)) * kmt[g]
                    bb = jnp.sum(bb, axis=0, keepdims=True) * (1.0 + 2.0 ** -10)
                    st["bnd"].append(jnp.broadcast_to(bb, (8, LANES)))
                st["ls"] = [jnp.zeros((8, LANES), F32) for _ in range(J)]
                st["accs"] = [jnp.zeros((DHA, LANES), F32) for _ in range(J)]
                st["ps"] = {}

            def qk(kb):
                kblk = kk[st["g"], kb * TK:(kb + 1) * TK, :]
                for j in range(J):
                    s = _dot(kblk, st["qms"][j]).reshape(TK // 8, 8, LANES)
                    p = jnp.exp2(s - st["bnd"][j][None])
                    st["ls"][j] = st["ls"][j] + jnp.sum(p, axis=0)
                    st["ps"][(kb, j)] = p.reshape(TK, LANES).astype(BF16)

            def pv(kb):
                vblk = vt[pl.ds(h0, DHA), kb * TK:(kb + 1) * TK]
                for j in range(J):
                    st["accs"][j] = st["accs"][j] + _dot(vblk, st["ps"].pop((kb, j)))

            def finish():
                lo = lchk[0]
                hi = lchk[1]
                for j in range(J):
                    l1 = jnp.sum(st["ls"][j], axis=0, keepdims=True)
                    l8 = jnp.broadcast_to(l1, (8, LANES))
                    lo = jnp.where(l8 >= lo, lo, l8)
                    hi = jnp.where(l8 <= hi, hi, l8)
                    q0 = pl.multiple_of(qb * TQ + j * LANES, LANES)
                    ot[pl.ds(h0, DHA), pl.ds(q0, LANES)] = (st["accs"][j] / l1).astype(BF16)
                lchk[0] = lo
                lchk[1] = hi

            def unit(kb):
                def f():
                    if kb == 0:
                        setup()
                    if kb < NK:
                        qk(kb)
                    if kb >= A_SKEW:
                        pv(kb - A_SKEW)
                    if kb == NK + A_SKEW - 1:
                        finish()
                return f

            return [unit(kb) for kb in range(NK + A_SKEW)]

        def b_slots(s):
            st = {"qkv": {}, "ps": {}, "os": {}, "outs": [None] * NG}
            r0 = pl.multiple_of(s * SEG, SEG)

            def setup():
                hbuf[M:L, :] = xb[pl.ds(r0, SEG), :].astype(F32)
                st["X"] = hbuf[...]
                row = lax.broadcasted_iota(jnp.int32, (L, L), 0)
                col = lax.broadcasted_iota(jnp.int32, (L, L), 1)
                st["mask"] = (row < M) | (row >= col)

            def proj(h):
                st["qkv"][h] = [_dot(st["X"], pltpu.bitcast(wb[t, h], BF16)) for t in range(3)]

            def qk(h):
                q, k, _ = st["qkv"][h]
                sc = _dot_nt(q, k.astype(BF16)) * bscale
                sc = jnp.where(st["mask"], sc, -1e9)
                m = jnp.max(sc, axis=-1, keepdims=True)
                p = jnp.exp(sc - m)
                st["ps"][h] = p / jnp.sum(p, axis=-1, keepdims=True)

            def pv(h):
                v = st["qkv"].pop(h)[2]
                st["os"][h] = _dot(st["ps"].pop(h), v.astype(BF16))

            def outp(h):
                o = st["os"].pop(h)
                outs = st["outs"]
                for n in range(NG):
                    t = _dot(o, pltpu.bitcast(wob[n, h], BF16))
                    outs[n] = t if outs[n] is None else outs[n] + t
                if h % GRP == GRP - 1:
                    for n in range(NG):
                        if h == GRP - 1:
                            obuf[:, n * LANES:(n + 1) * LANES] = outs[n]
                        else:
                            obuf[:, n * LANES:(n + 1) * LANES] += outs[n]
                        outs[n] = None

            def finish():
                o = obuf[...]
                hbuf[0:M, :] = o[0:M].astype(BF16).astype(F32)
                bbuf[pl.ds(r0, SEG), :] = o[M:L]

            def slot(t):
                def f():
                    if t == 0:
                        setup()
                    if t < HB:
                        proj(t)
                    if 0 <= t - SKEW[0] < HB:
                        qk(t - SKEW[0])
                    if 0 <= t - SKEW[1] < HB:
                        pv(t - SKEW[1])
                    if 0 <= t - SKEW[2] < HB:
                        outp(t - SKEW[2])
                    if t == HB + SKEW[2] - 1:
                        finish()
                return f

            return [slot(t) for t in range(HB + SKEW[2])]

        def main_step(s, carry):
            h = s * QPS // NQ
            qb0 = (s * QPS) % NQ
            units = []
            for i in range(QPS):
                u = a_units(h, qb0 + i)
                for k in range(A_SKEW):
                    if len(units) >= A_SKEW:
                        last = units[len(units) - A_SKEW + k]
                        u[k] = (lambda a=u[k], b=last: (a(), b()))
                if units:
                    units = units[:len(units) - A_SKEW]
                units += u
            slots = b_slots(s)
            ns, nu = len(slots), len(units)
            nd = nu - A_SKEW
            pos = [ns - A_END - A_SKEW - A_STRIDE * (nd - 1 - i) for i in range(nd)]
            pos += [ns - A_END - A_SKEW + 1 + k for k in range(A_SKEW)]
            for t in range(ns):
                slots[t]()
                for i in range(nu):
                    if min(max(pos[i], 0), ns - 1) == t:
                        units[i]()
            return carry

        lax.fori_loop(0, NSEG, main_step, 0)

        ok = jnp.logical_and(lchk[0] >= L_MIN, lchk[1] <= L_MAX)
        n_bad = jnp.sum(jnp.where(ok, 0.0, 1.0))

        @pl.when(n_bad > 0.0)
        def _exact_softmax_fallback():
            def body(it, carry):
                h = it // (S // LANES)
                qb = it % (S // LANES)
                h0 = pl.multiple_of(h * DHA, DHA)
                q0 = pl.multiple_of(qb * LANES, LANES)
                g, qm = head_masked_q(h, q0)
                m = jnp.full((8, LANES), -jnp.inf, F32)
                for kb in range(NK):
                    s = _dot(kk[g, kb * TK:(kb + 1) * TK, :], qm)
                    sbuf[kb * TK:(kb + 1) * TK, :] = s
                    m = jnp.maximum(m, jnp.max(s.reshape(TK // 8, 8, LANES), axis=0))
                m1 = jnp.max(m, axis=0, keepdims=True)
                l = jnp.zeros((8, LANES), F32)
                acc = jnp.zeros((DHA, LANES), F32)
                for kb in range(NK):
                    p = jnp.exp2(sbuf[kb * TK:(kb + 1) * TK, :] - m1)
                    l = l + jnp.sum(p.reshape(TK // 8, 8, LANES), axis=0)
                    acc = acc + _dot(vt[pl.ds(h0, DHA), kb * TK:(kb + 1) * TK], p.astype(BF16))
                l1 = jnp.sum(l, axis=0, keepdims=True)
                ot[pl.ds(h0, DHA), pl.ds(q0, LANES)] = (acc / l1).astype(BF16)
                return carry

            lax.fori_loop(0, HA * (S // LANES), body, 0)

        cp_woa.wait()

        def out_copy(i):
            r0 = pl.multiple_of(i * TM, TM)
            return pltpu.make_async_copy(outv.at[pl.ds(r0, TM), :], out_hbm.at[0, pl.ds(r0, TM), :], sem_out.at[i])

        def final(i, carry):
            r0 = pl.multiple_of(i * TM, TM)
            a = _dot_tn(ot[:, pl.ds(r0, TM)], woa[...])
            g = gl[pl.ds(r0, TM), :]
            for n in range(NG):
                sl = slice(n * LANES, (n + 1) * LANES)
                outv[pl.ds(r0, TM), sl] = (g * a[:, sl] + (1.0 - g) * bbuf[pl.ds(r0, TM), sl]).astype(BF16)
            out_copy(i).start()
            return carry

        lax.fori_loop(0, NBLK, final, 0)
        for i in range(NBLK):
            out_copy(i).wait()

    return kernel


@functools.partial(jax.jit, static_argnames=("B_seg_len",))
def pallas_gated_mix__softmax_full_mha__memory_aug_recurrent_mem_tr__prompt_kernel(
    A_x: jax.Array,
    A_wqkv: jax.Array,
    A_wo: jax.Array,
    B_x: jax.Array,
    B_mem0: jax.Array,
    B_Wq: jax.Array,
    B_Wk: jax.Array,
    B_Wv: jax.Array,
    B_Wo: jax.Array,
    B_seg_len: int,
    gate_w: jax.Array,
):
    _, S, D = A_x.shape
    _, HB, DHB = B_Wq.shape
    M = B_mem0.shape[1]
    SEG = int(B_seg_len)
    NG = D // LANES
    wq, wk, wv = (w.reshape(D // 2, 2 * HB, DHB) for w in (B_Wq, B_Wk, B_Wv))
    gate = gate_w.reshape(1, D)

    any_spec = pl.BlockSpec(memory_space=pl.ANY)
    scratch = [
        pltpu.VMEM((S, D), BF16),
        pltpu.VMEM((D, 3 * D), BF16),
        pltpu.VMEM((D, D), BF16),
        pltpu.VMEM((S, D), BF16),
        pltpu.VMEM((M, D), BF16),
        pltpu.VMEM((1, D), BF16),
        pltpu.VMEM((3, HB, D // 2, DHB), U32),
        pltpu.VMEM((NG, HB, DHB // 2, LANES), U32),
        pltpu.VMEM((NG, LANES, S), BF16),
        pltpu.VMEM((NG, S, LANES), BF16),
        pltpu.VMEM((D, S), BF16),
        pltpu.VMEM((D, S), BF16),
        pltpu.VMEM((NG, 8, LANES), F32),
        pltpu.VMEM((NG, LANES, LANES), F32),
        pltpu.VMEM((2, 8, LANES), F32),
        pltpu.VMEM((S, LANES), F32),
        pltpu.VMEM((S, D), F32),
        pltpu.VMEM((M + SEG, D), F32),
        pltpu.VMEM((M + SEG, D), F32),
        pltpu.VMEM((S, LANES), F32),
        pltpu.VMEM((S, D), BF16),
        pltpu.SemaphoreType.DMA((2,)),
        pltpu.SemaphoreType.DMA((3 * NG // WCH,)),
        pltpu.SemaphoreType.DMA((4,)),
        pltpu.SemaphoreType.DMA((3 * HB,)),
        pltpu.SemaphoreType.DMA((NG,)),
        pltpu.SemaphoreType.DMA((S // TM,)),
    ]
    return pl.pallas_call(
        _make_kernel(S, D, HB, DHB, M, SEG),
        out_shape=jax.ShapeDtypeStruct((1, S, D), BF16),
        in_specs=[any_spec] * 10,
        out_specs=any_spec,
        scratch_shapes=scratch,
        compiler_params=pltpu.CompilerParams(vmem_limit_bytes=120 * 1024 * 1024),
        name="gated_mix",
    )(A_x, A_wqkv, A_wo, B_x, B_mem0, wq, wk, wv, B_Wo, gate)
```

```python
import functools
import math

import jax
import jax.numpy as jnp
from jax import lax
import jax.experimental.pallas as pl
import jax.experimental.pallas.tpu as pltpu

F32 = jnp.float32
BF16 = jnp.bfloat16
U32 = jnp.uint32

LANES = 128
HA = 32
TQ = 512
TK = 256
TM = 256
NSUB = 2
WCH = (2, 4, 8, 10)
REP_RC = 16
L_MIN = 2.0 ** -64
L_MAX = 2.0 ** 64
SKEW = (1, 3, 5)
GRP = 8
A_SKEW = 1
A_END = 4
A_STRIDE = 2


def _dot(a, b):
    return lax.dot_general(a, b, (((1,), (0,)), ((), ())), preferred_element_type=F32)


def _dot_nt(a, b):
    return lax.dot_general(a, b, (((1,), (1,)), ((), ())), preferred_element_type=F32)


def _dot_tn(a, b):
    return lax.dot_general(a, b, (((0,), (0,)), ((), ())), preferred_element_type=F32)


def _make_kernel(S, D, HB, DHB, M, SEG):
    DHA = D // HA
    HPG = LANES // DHA
    NG = D // LANES
    L = M + SEG
    NSEG = S // SEG
    NQ = S // TQ
    NK = S // TK
    J = TQ // LANES
    TB = TM * NSUB
    NBLK = S // TB
    NPAIR = HB // 2
    assert sum(WCH) == 3 * NG
    WOFF = [sum(WCH[:k]) for k in range(len(WCH))]
    QPS = HA * NQ // NSEG
    assert QPS * NSEG == HA * NQ and NQ % QPS == 0
    qscale = (DHA ** -0.5) * math.log2(math.e)
    bscale = DHB ** -0.5

    def kernel(xa_hbm, wqkv_hbm, woa_hbm, xb_hbm, mem_hbm, wq_hbm, wk_hbm, wv_hbm, wob_hbm, gate_hbm,
               out_hbm,
               xa, wqkv, woa, xb, mem, gate, wb, wob,
               qt, kk, vt, ot, kmax, kmt, lchk, gl, bbuf, hbuf, obuf, sbuf, outv,
               sem_x, sem_wa, sem_in, sem_w, sem_wo, sem_out):
        cp_x0 = pltpu.make_async_copy(xa_hbm.at[0, 0:TB, :], xa.at[0:TB, :], sem_x.at[0])
        cp_xr = pltpu.make_async_copy(xa_hbm.at[0, TB:S, :], xa.at[TB:S, :], sem_x.at[1])
        cp_wa = [pltpu.make_async_copy(wqkv_hbm.at[:, o * LANES:(o + n) * LANES],
                                       wqkv.at[:, o * LANES:(o + n) * LANES], sem_wa.at[k])
                 for k, (o, n) in enumerate(zip(WOFF, WCH))]
        cp_gate = pltpu.make_async_copy(gate_hbm, gate, sem_in.at[0])
        cp_woa = pltpu.make_async_copy(woa_hbm, woa, sem_in.at[1])
        cp_xb0 = pltpu.make_async_copy(xb_hbm.at[0, 0:TB, :], xb.at[0:TB, :], sem_in.at[2])
        cp_xb1 = pltpu.make_async_copy(xb_hbm.at[0, TB:S, :], xb.at[TB:S, :], sem_in.at[4])
        cp_mem = pltpu.make_async_copy(mem_hbm.at[0], mem, sem_in.at[3])

        def w_copies(t):
            src = (wq_hbm, wk_hbm, wv_hbm)[t].bitcast(U32)
            return [pltpu.make_async_copy(src.at[:, r, :], wb.at[t, 2 * (r % NPAIR) + r // NPAIR],
                                          sem_w.at[t * HB + r]) for r in range(HB)]

        w_cps = [w_copies(t) for t in range(3)]
        wob_u = wob_hbm.bitcast(U32)
        wo_cps = [pltpu.make_async_copy(wob_u.at[:, :, n * LANES:(n + 1) * LANES], wob.at[n], sem_wo.at[n])
                  for n in range(NG)]

        hw = HB // 2

        def sync(waits, starts):
            for cp in waits:
                cp.wait()
            for cp in starts:
                cp.start()

        sync0 = {WOFF[0]: ([cp_wa[0]], []),
                 WOFF[1]: ([cp_wa[1]], [cp_xr]),
                 WOFF[2]: ([cp_wa[2]], w_cps[0]),
                 WOFF[3]: ([cp_wa[3]], w_cps[1])}
        sync1 = {0: ([cp_xr], []),
                 2 * NG: (w_cps[0], w_cps[2])}
        sync2 = {NG: (w_cps[1][:hw], wo_cps + [cp_xb0, cp_mem])}
        sync3 = {0: (w_cps[1][hw:], []),
                 NG: (w_cps[2], [])}
        cp_gate.start()
        cp_x0.start()
        cp_wa[0].start()
        cp_wa[1].start()

        kmax[...] = jnp.zeros(kmax.shape, F32)

        def repack(t, j, anchor):
            z = (pltpu.bitcast(anchor, U32) & jnp.uint32(0x7FFF)) >> 15
            for r in range(0, D // 2, REP_RC):
                zz = jnp.concatenate([z] * (REP_RC // 8), axis=0)
                e = wb[t, 2 * j, r:r + REP_RC, :] | zz
                o = wb[t, 2 * j + 1, r:r + REP_RC, :]
                lo = (e & jnp.uint32(0xFFFF)) | (o << 16)
                wb[t, 2 * j, r:r + REP_RC, :] = lo
                wb[t, 2 * j + 1, r:r + REP_RC, :] = (e >> 16) | (o & jnp.uint32(0xFFFF0000))
                z = (lo[0:8, :] & jnp.uint32(0x7FFF)) >> 15

        def a_proj(i, syncs, rep=()):
            rep = list(rep)
            r0s = [i * TB + u * TM for u in range(NSUB)]
            prev = None
            for c in range(3 * NG):
                if c in syncs:
                    sync(*syncs[c])
                    prev = None
                for u in range(NSUB):
                    r0 = r0s[u]
                    xu = xa[r0:r0 + TM, :]
                    r = _dot(xu, wqkv[:, c * LANES:(c + 1) * LANES])
                    if c < NG:
                        qt[c, :, r0:r0 + TM] = (r * qscale).T.astype(BF16)
                    elif c < 2 * NG:
                        g = c - NG
                        rb = r.astype(BF16)
                        kk[g, r0:r0 + TM, :] = rb
                        ab = jnp.abs(rb.astype(F32))
                        kmax[g] = jnp.maximum(kmax[g], jnp.max(ab.reshape(TM // 8, 8, LANES), axis=0))
                    else:
                        g = c - 2 * NG
                        vt[g * LANES:(g + 1) * LANES, r0:r0 + TM] = r.T.astype(BF16)
                    while prev is not None and rep and rep[0][0] <= c * NSUB + u:
                        _, t, j = rep.pop(0)
                        repack(t, j, prev)
                    prev = r[0:8, :]
                    if c == NG + 2 + 4 * u:
                        gv = gate[...].astype(F32).reshape(1, D)
                        logit = jnp.sum(xu.astype(F32) * gv, axis=-1, keepdims=True)
                        gl[r0:r0 + TM, :] = jnp.broadcast_to(jax.nn.sigmoid(logit), (TM, LANES))

        sync([cp_gate, cp_x0], [cp_wa[2], cp_wa[3]])
        a_proj(0, sync0)
        a_proj(1, sync1)
        ndots = 3 * NG * NSUB
        a_proj(2, sync2, rep=[(j * (ndots - 2) // NPAIR, 0, j) for j in range(NPAIR)])
        a_proj(3, sync3, rep=[(j * NG * NSUB // NPAIR, 1, j) for j in range(NPAIR)]
               + [(NG * NSUB + j * (ndots - NG * NSUB - 2) // NPAIR, 2, j) for j in range(NPAIR)])

        for g in range(NG):
            km = jnp.max(kmax[g], axis=0, keepdims=True)
            kmt[g] = jnp.broadcast_to(km, (LANES, LANES)).T

        lchk[0] = jnp.full((8, LANES), L_MAX, F32)
        lchk[1] = jnp.full((8, LANES), L_MIN, F32)

        for c in wo_cps:
            c.wait()
        cp_xb0.wait()
        cp_mem.wait()
        cp_xb1.start()
        cp_woa.start()
        hbuf[0:M, :] = mem[...].astype(F32)

        def head_masked_q(h, q0):
            g = h // HPG
            r = h % HPG
            rows = lax.broadcasted_iota(jnp.int32, (LANES, LANES), 0)
            msk = (rows >= r * DHA) & (rows < r * DHA + DHA)
            q = qt[g, :, pl.ds(q0, LANES)]
            return g, jnp.where(msk, q, jnp.zeros_like(q))

        def a_units(h, qb):
            st = {}
            h0 = pl.multiple_of(h * DHA, DHA)

            def setup():
                st["qms"], st["bnd"] = [], []
                for j in range(J):
                    q0 = pl.multiple_of(qb * TQ + j * LANES, LANES)
                    g, qm = head_masked_q(h, q0)
                    st["g"] = g
                    st["qms"].append(qm)
                    bb = jnp.abs(qm.astype(F32)) * kmt[g]
                    bb = jnp.sum(bb, axis=0, keepdims=True) * (1.0 + 2.0 ** -10)
                    st["bnd"].append(jnp.broadcast_to(bb, (8, LANES)))
                st["ls"] = [jnp.zeros((8, LANES), F32) for _ in range(J)]
                st["accs"] = [jnp.zeros((DHA, LANES), F32) for _ in range(J)]
                st["ps"] = {}

            def qk(kb):
                kblk = kk[st["g"], kb * TK:(kb + 1) * TK, :]
                for j in range(J):
                    s = _dot(kblk, st["qms"][j]).reshape(TK // 8, 8, LANES)
                    p = jnp.exp2(s - st["bnd"][j][None])
                    st["ls"][j] = st["ls"][j] + jnp.sum(p, axis=0)
                    st["ps"][(kb, j)] = p.reshape(TK, LANES).astype(BF16)

            def pv(kb):
                vblk = vt[pl.ds(h0, DHA), kb * TK:(kb + 1) * TK]
                for j in range(J):
                    st["accs"][j] = st["accs"][j] + _dot(vblk, st["ps"].pop((kb, j)))

            def finish():
                lo = lchk[0]
                hi = lchk[1]
                for j in range(J):
                    l1 = jnp.sum(st["ls"][j], axis=0, keepdims=True)
                    l8 = jnp.broadcast_to(l1, (8, LANES))
                    lo = jnp.where(l8 >= lo, lo, l8)
                    hi = jnp.where(l8 <= hi, hi, l8)
                    q0 = pl.multiple_of(qb * TQ + j * LANES, LANES)
                    ot[pl.ds(h0, DHA), pl.ds(q0, LANES)] = (st["accs"][j] / l1).astype(BF16)
                lchk[0] = lo
                lchk[1] = hi

            def unit(kb):
                def f():
                    if kb == 0:
                        setup()
                    if kb < NK:
                        qk(kb)
                    if kb >= A_SKEW:
                        pv(kb - A_SKEW)
                    if kb == NK + A_SKEW - 1:
                        finish()
                return f

            return [unit(kb) for kb in range(NK + A_SKEW)]

        def b_slots(s):
            st = {"qkv": {}, "ps": {}, "os": {}, "outs": [None] * NG}
            r0 = pl.multiple_of(s * SEG, SEG)

            def setup():
                hbuf[M:L, :] = xb[pl.ds(r0, SEG), :].astype(F32)
                st["X"] = hbuf[...]
                row = lax.broadcasted_iota(jnp.int32, (L, L), 0)
                col = lax.broadcasted_iota(jnp.int32, (L, L), 1)
                st["mask"] = (row < M) | (row >= col)

            def proj(h):
                st["qkv"][h] = [_dot(st["X"], pltpu.bitcast(wb[t, h], BF16)) for t in range(3)]

            def qk(h):
                q, k, _ = st["qkv"][h]
                sc = _dot_nt(q, k.astype(BF16)) * bscale
                sc = jnp.where(st["mask"], sc, -1e9)
                m = jnp.max(sc, axis=-1, keepdims=True)
                p = jnp.exp(sc - m)
                st["ps"][h] = p / jnp.sum(p, axis=-1, keepdims=True)

            def pv(h):
                v = st["qkv"].pop(h)[2]
                st["os"][h] = _dot(st["ps"].pop(h), v.astype(BF16))

            def outp(h):
                o = st["os"].pop(h)
                outs = st["outs"]
                for n in range(NG):
                    t = _dot(o, pltpu.bitcast(wob[n, h], BF16))
                    outs[n] = t if outs[n] is None else outs[n] + t
                if h % GRP == GRP - 1:
                    for n in range(NG):
                        if h == GRP - 1:
                            obuf[:, n * LANES:(n + 1) * LANES] = outs[n]
                        else:
                            obuf[:, n * LANES:(n + 1) * LANES] += outs[n]
                        outs[n] = None

            def finish():
                o = obuf[...]
                hbuf[0:M, :] = o[0:M].astype(BF16).astype(F32)
                bbuf[pl.ds(r0, SEG), :] = o[M:L]

            def slot(t):
                def f():
                    if t == 0:
                        setup()
                    if t < HB:
                        proj(t)
                    if 0 <= t - SKEW[0] < HB:
                        qk(t - SKEW[0])
                    if 0 <= t - SKEW[1] < HB:
                        pv(t - SKEW[1])
                    if 0 <= t - SKEW[2] < HB:
                        outp(t - SKEW[2])
                    if t == HB + SKEW[2] - 1:
                        finish()
                return f

            return [slot(t) for t in range(HB + SKEW[2])]

        def main_step(s, carry):
            @pl.when(s == TB // SEG)
            def _():
                cp_xb1.wait()

            h = s * QPS // NQ
            qb0 = (s * QPS) % NQ
            units = []
            for i in range(QPS):
                u = a_units(h, qb0 + i)
                for k in range(A_SKEW):
                    if len(units) >= A_SKEW:
                        last = units[len(units) - A_SKEW + k]
                        u[k] = (lambda a=u[k], b=last: (a(), b()))
                if units:
                    units = units[:len(units) - A_SKEW]
                units += u
            slots = b_slots(s)
            ns, nu = len(slots), len(units)
            nd = nu - A_SKEW
            pos = [ns - A_END - A_SKEW - A_STRIDE * (nd - 1 - i) for i in range(nd)]
            pos += [ns - A_END - A_SKEW + 1 + k for k in range(A_SKEW)]
            for t in range(ns):
                slots[t]()
                for i in range(nu):
                    if min(max(pos[i], 0), ns - 1) == t:
                        units[i]()
            return carry

        lax.fori_loop(0, NSEG, main_step, 0)

        ok = jnp.logical_and(lchk[0] >= L_MIN, lchk[1] <= L_MAX)
        n_bad = jnp.sum(jnp.where(ok, 0.0, 1.0))

        @pl.when(n_bad > 0.0)
        def _exact_softmax_fallback():
            def body(it, carry):
                h = it // (S // LANES)
                qb = it % (S // LANES)
                h0 = pl.multiple_of(h * DHA, DHA)
                q0 = pl.multiple_of(qb * LANES, LANES)
                g, qm = head_masked_q(h, q0)
                m = jnp.full((8, LANES), -jnp.inf, F32)
                for kb in range(NK):
                    s = _dot(kk[g, kb * TK:(kb + 1) * TK, :], qm)
                    sbuf[kb * TK:(kb + 1) * TK, :] = s
                    m = jnp.maximum(m, jnp.max(s.reshape(TK // 8, 8, LANES), axis=0))
                m1 = jnp.max(m, axis=0, keepdims=True)
                l = jnp.zeros((8, LANES), F32)
                acc = jnp.zeros((DHA, LANES), F32)
                for kb in range(NK):
                    p = jnp.exp2(sbuf[kb * TK:(kb + 1) * TK, :] - m1)
                    l = l + jnp.sum(p.reshape(TK // 8, 8, LANES), axis=0)
                    acc = acc + _dot(vt[pl.ds(h0, DHA), kb * TK:(kb + 1) * TK], p.astype(BF16))
                l1 = jnp.sum(l, axis=0, keepdims=True)
                ot[pl.ds(h0, DHA), pl.ds(q0, LANES)] = (acc / l1).astype(BF16)
                return carry

            lax.fori_loop(0, HA * (S // LANES), body, 0)

        cp_woa.wait()

        def out_copy(i):
            r0 = pl.multiple_of(i * TM, TM)
            return pltpu.make_async_copy(outv.at[pl.ds(r0, TM), :], out_hbm.at[0, pl.ds(r0, TM), :], sem_out.at[i])

        def final(i, carry):
            for u in range(NSUB):
                r0 = pl.multiple_of(i * TB + u * TM, TM)
                a = _dot_tn(ot[:, pl.ds(r0, TM)], woa[...])
                g = gl[pl.ds(r0, TM), :]
                for n in range(NG):
                    sl = slice(n * LANES, (n + 1) * LANES)
                    outv[pl.ds(r0, TM), sl] = (g * a[:, sl] + (1.0 - g) * bbuf[pl.ds(r0, TM), sl]).astype(BF16)
            for u in range(NSUB):
                out_copy(i * NSUB + u).start()
            return carry

        lax.fori_loop(0, NBLK, final, 0)
        for i in range(S // TM):
            out_copy(i).wait()

    return kernel


@functools.partial(jax.jit, static_argnames=("B_seg_len",))
def pallas_gated_mix__softmax_full_mha__memory_aug_recurrent_mem_tr__prompt_kernel(
    A_x: jax.Array,
    A_wqkv: jax.Array,
    A_wo: jax.Array,
    B_x: jax.Array,
    B_mem0: jax.Array,
    B_Wq: jax.Array,
    B_Wk: jax.Array,
    B_Wv: jax.Array,
    B_Wo: jax.Array,
    B_seg_len: int,
    gate_w: jax.Array,
):
    _, S, D = A_x.shape
    _, HB, DHB = B_Wq.shape
    M = B_mem0.shape[1]
    SEG = int(B_seg_len)
    NG = D // LANES
    wq, wk, wv = (w.reshape(D // 2, 2 * HB, DHB) for w in (B_Wq, B_Wk, B_Wv))

    any_spec = pl.BlockSpec(memory_space=pl.ANY)
    scratch = [
        pltpu.VMEM((S, D), BF16),
        pltpu.VMEM((D, 3 * D), BF16),
        pltpu.VMEM((D, D), BF16),
        pltpu.VMEM((S, D), BF16),
        pltpu.VMEM((M, D), BF16),
        pltpu.VMEM((D,), BF16),
        pltpu.VMEM((3, HB, D // 2, DHB), U32),
        pltpu.VMEM((NG, HB, DHB // 2, LANES), U32),
        pltpu.VMEM((NG, LANES, S), BF16),
        pltpu.VMEM((NG, S, LANES), BF16),
        pltpu.VMEM((D, S), BF16),
        pltpu.VMEM((D, S), BF16),
        pltpu.VMEM((NG, 8, LANES), F32),
        pltpu.VMEM((NG, LANES, LANES), F32),
        pltpu.VMEM((2, 8, LANES), F32),
        pltpu.VMEM((S, LANES), F32),
        pltpu.VMEM((S, D), F32),
        pltpu.VMEM((M + SEG, D), F32),
        pltpu.VMEM((M + SEG, D), F32),
        pltpu.VMEM((S, LANES), F32),
        pltpu.VMEM((S, D), BF16),
        pltpu.SemaphoreType.DMA((2,)),
        pltpu.SemaphoreType.DMA((len(WCH),)),
        pltpu.SemaphoreType.DMA((5,)),
        pltpu.SemaphoreType.DMA((3 * HB,)),
        pltpu.SemaphoreType.DMA((NG,)),
        pltpu.SemaphoreType.DMA((S // TM,)),
    ]
    return pl.pallas_call(
        _make_kernel(S, D, HB, DHB, M, SEG),
        out_shape=jax.ShapeDtypeStruct((1, S, D), BF16),
        in_specs=[any_spec] * 10,
        out_specs=any_spec,
        scratch_shapes=scratch,
        compiler_params=pltpu.CompilerParams(vmem_limit_bytes=120 * 1024 * 1024, disable_bounds_checks=True),
        name="gated_mix",
    )(A_x, A_wqkv, A_wo, B_x, B_mem0, wq, wk, wv, B_Wo, gate_w)
```

```python
import functools
import math

import jax
import jax.numpy as jnp
from jax import lax
import jax.experimental.pallas as pl
import jax.experimental.pallas.tpu as pltpu

F32 = jnp.float32
BF16 = jnp.bfloat16
U32 = jnp.uint32

LANES = 128
HA = 32
TQ = 512
TK = 256
TM = 256
NSUB = 2
WCH = (2, 4, 8, 10)
REP_RC = 16
L_MIN = 2.0 ** -64
L_MAX = 2.0 ** 64
SKEW = (1, 3, 5)
GRP = 8
A_SKEW = 1
A_END = 4
UNROLL = 2
A_STRIDE = 2


def _dot(a, b):
    return lax.dot_general(a, b, (((1,), (0,)), ((), ())), preferred_element_type=F32)


def _dot_nt(a, b):
    return lax.dot_general(a, b, (((1,), (1,)), ((), ())), preferred_element_type=F32)


def _dot_tn(a, b):
    return lax.dot_general(a, b, (((0,), (0,)), ((), ())), preferred_element_type=F32)


def _make_kernel(S, D, HB, DHB, M, SEG):
    DHA = D // HA
    HPG = LANES // DHA
    NG = D // LANES
    L = M + SEG
    NSEG = S // SEG
    NQ = S // TQ
    NK = S // TK
    J = TQ // LANES
    TB = TM * NSUB
    NBLK = S // TB
    NPAIR = HB // 2
    assert sum(WCH) == 3 * NG
    WOFF = [sum(WCH[:k]) for k in range(len(WCH))]
    QPS = HA * NQ // NSEG
    assert QPS * NSEG == HA * NQ and NQ % QPS == 0
    qscale = (DHA ** -0.5) * math.log2(math.e)
    bscale = DHB ** -0.5

    def kernel(xa_hbm, wqkv_hbm, woa_hbm, xb_hbm, mem_hbm, wq_hbm, wk_hbm, wv_hbm, wob_hbm, gate_hbm,
               out_hbm,
               xa, wqkv, woa, xb, mem, gate, wb, wob,
               qt, kk, vt, ot, kmax, kmt, lchk, gl, bbuf, hbuf, obuf, sbuf, outv,
               sem_x, sem_wa, sem_in, sem_w, sem_wo, sem_out):
        cp_x0 = pltpu.make_async_copy(xa_hbm.at[0, 0:TB, :], xa.at[0:TB, :], sem_x.at[0])
        cp_xr = pltpu.make_async_copy(xa_hbm.at[0, TB:S, :], xa.at[TB:S, :], sem_x.at[1])
        cp_wa = [pltpu.make_async_copy(wqkv_hbm.at[:, o * LANES:(o + n) * LANES],
                                       wqkv.at[:, o * LANES:(o + n) * LANES], sem_wa.at[k])
                 for k, (o, n) in enumerate(zip(WOFF, WCH))]
        cp_gate = pltpu.make_async_copy(gate_hbm, gate, sem_in.at[0])
        cp_woa = pltpu.make_async_copy(woa_hbm, woa, sem_in.at[1])
        cp_xb0 = pltpu.make_async_copy(xb_hbm.at[0, 0:TB, :], xb.at[0:TB, :], sem_in.at[2])
        cp_xb1 = pltpu.make_async_copy(xb_hbm.at[0, TB:S, :], xb.at[TB:S, :], sem_in.at[4])
        cp_mem = pltpu.make_async_copy(mem_hbm.at[0], mem, sem_in.at[3])

        def w_copies(t):
            src = (wq_hbm, wk_hbm, wv_hbm)[t].bitcast(U32)
            return [pltpu.make_async_copy(src.at[:, r, :], wb.at[t, 2 * (r % NPAIR) + r // NPAIR],
                                          sem_w.at[t * HB + r]) for r in range(HB)]

        w_cps = [w_copies(t) for t in range(3)]
        wob_u = wob_hbm.bitcast(U32)
        wo_cps = [pltpu.make_async_copy(wob_u.at[:, :, n * LANES:(n + 1) * LANES], wob.at[n], sem_wo.at[n])
                  for n in range(NG)]

        hw = HB // 2

        def sync(waits, starts):
            for cp in waits:
                cp.wait()
            for cp in starts:
                cp.start()

        sync0 = {WOFF[1]: ([cp_wa[1]], [cp_xr]),
                 WOFF[2]: ([cp_wa[2]], w_cps[0]),
                 WOFF[3]: ([cp_wa[3]], w_cps[1])}
        sync1 = {0: ([cp_xr], []),
                 2 * NG: (w_cps[0], w_cps[2])}
        sync2 = {NG + NG // 2: (w_cps[1], wo_cps + [cp_xb0, cp_mem])}
        sync3 = {NG - 2: (w_cps[2], [])}
        cp_gate.start()
        cp_x0.start()
        cp_wa[0].start()
        cp_wa[1].start()

        kmax[...] = jnp.zeros(kmax.shape, F32)

        def repack(t, j, anchor):
            z = (pltpu.bitcast(anchor, U32) & jnp.uint32(0x7FFF)) >> 15
            for r in range(0, D // 2, REP_RC):
                zz = jnp.concatenate([z] * (REP_RC // 8), axis=0)
                e = wb[t, 2 * j, r:r + REP_RC, :] | zz
                o = wb[t, 2 * j + 1, r:r + REP_RC, :]
                lo = (e & jnp.uint32(0xFFFF)) | (o << 16)
                wb[t, 2 * j, r:r + REP_RC, :] = lo
                wb[t, 2 * j + 1, r:r + REP_RC, :] = (e >> 16) | (o & jnp.uint32(0xFFFF0000))
                z = (lo[0:8, :] & jnp.uint32(0x7FFF)) >> 15

        def a_proj(i, syncs, rep=()):
            rep = list(rep)
            r0s = [i * TB + u * TM for u in range(NSUB)]
            prev = None
            for c in range(3 * NG):
                if c in syncs:
                    sync(*syncs[c])
                    prev = None
                for u in range(NSUB):
                    r0 = r0s[u]
                    xu = xa[r0:r0 + TM, :]
                    r = _dot(xu, wqkv[:, c * LANES:(c + 1) * LANES])
                    if c < NG:
                        qt[c, :, r0:r0 + TM] = (r * qscale).T.astype(BF16)
                    elif c < 2 * NG:
                        g = c - NG
                        rb = r.astype(BF16)
                        kk[g, r0:r0 + TM, :] = rb
                        ab = jnp.abs(rb.astype(F32))
                        kmax[g] = jnp.maximum(kmax[g], jnp.max(ab.reshape(TM // 8, 8, LANES), axis=0))
                    else:
                        g = c - 2 * NG
                        vt[g * LANES:(g + 1) * LANES, r0:r0 + TM] = r.T.astype(BF16)
                    while prev is not None and rep and rep[0][0] <= c * NSUB + u:
                        _, t, j = rep.pop(0)
                        repack(t, j, prev)
                    prev = r[0:8, :]
                    if c == NG + 2 + 4 * u:
                        gv = gate[...].astype(F32).reshape(1, D)
                        logit = jnp.sum(xu.astype(F32) * gv, axis=-1, keepdims=True)
                        gl[r0:r0 + TM, :] = jnp.broadcast_to(jax.nn.sigmoid(logit), (TM, LANES))

        ndots = 3 * NG * NSUB
        sync([cp_gate, cp_x0, cp_wa[0]], [cp_wa[2], cp_wa[3]])
        a_proj(0, sync0)
        a_proj(1, sync1)
        k1 = (NG + NG // 2) * NSUB + 1
        k2 = (NG - 2) * NSUB + 1
        n2 = NPAIR // 2
        a_proj(2, sync2, rep=[(1 + j * (k1 - 2) // NPAIR, 0, j) for j in range(NPAIR)]
               + [(k1 + j * (ndots - k1 - 1) // n2, 1, j) for j in range(n2)])
        a_proj(3, sync3, rep=[(1 + j * (k2 - 2) // (NPAIR - n2), 1, n2 + j) for j in range(NPAIR - n2)]
               + [(k2 + j * (ndots - k2 - 1) // NPAIR, 2, j) for j in range(NPAIR)])

        for g in range(NG):
            km = jnp.max(kmax[g], axis=0, keepdims=True)
            kmt[g] = jnp.broadcast_to(km, (LANES, LANES)).T

        lchk[0] = jnp.full((8, LANES), L_MAX, F32)
        lchk[1] = jnp.full((8, LANES), L_MIN, F32)

        for c in wo_cps:
            c.wait()
        cp_xb0.wait()
        cp_mem.wait()
        cp_xb1.start()
        cp_woa.start()
        hbuf[0:M, :] = mem[...].astype(F32)

        def head_masked_q(h, q0):
            g = h // HPG
            r = h % HPG
            rows = lax.broadcasted_iota(jnp.int32, (LANES, LANES), 0)
            msk = (rows >= r * DHA) & (rows < r * DHA + DHA)
            q = qt[g, :, pl.ds(q0, LANES)]
            return g, jnp.where(msk, q, jnp.zeros_like(q))

        def a_units(h, qb):
            st = {}
            h0 = pl.multiple_of(h * DHA, DHA)

            def setup():
                st["qms"], st["bnd"] = [], []
                for j in range(J):
                    q0 = pl.multiple_of(qb * TQ + j * LANES, LANES)
                    g, qm = head_masked_q(h, q0)
                    st["g"] = g
                    st["qms"].append(qm)
                    bb = jnp.abs(qm.astype(F32)) * kmt[g]
                    bb = jnp.sum(bb, axis=0, keepdims=True) * (1.0 + 2.0 ** -10)
                    st["bnd"].append(jnp.broadcast_to(bb, (8, LANES)))
                st["ls"] = [jnp.zeros((8, LANES), F32) for _ in range(J)]
                st["accs"] = [jnp.zeros((DHA, LANES), F32) for _ in range(J)]
                st["ps"] = {}

            def qk(kb):
                kblk = kk[st["g"], kb * TK:(kb + 1) * TK, :]
                for j in range(J):
                    s = _dot(kblk, st["qms"][j]).reshape(TK // 8, 8, LANES)
                    p = jnp.exp2(s - st["bnd"][j][None])
                    st["ls"][j] = st["ls"][j] + jnp.sum(p, axis=0)
                    st["ps"][(kb, j)] = p.reshape(TK, LANES).astype(BF16)

            def pv(kb):
                vblk = vt[pl.ds(h0, DHA), kb * TK:(kb + 1) * TK]
                for j in range(J):
                    st["accs"][j] = st["accs"][j] + _dot(vblk, st["ps"].pop((kb, j)))

            def finish():
                lo = lchk[0]
                hi = lchk[1]
                for j in range(J):
                    l1 = jnp.sum(st["ls"][j], axis=0, keepdims=True)
                    l8 = jnp.broadcast_to(l1, (8, LANES))
                    lo = jnp.where(l8 >= lo, lo, l8)
                    hi = jnp.where(l8 <= hi, hi, l8)
                    q0 = pl.multiple_of(qb * TQ + j * LANES, LANES)
                    ot[pl.ds(h0, DHA), pl.ds(q0, LANES)] = (st["accs"][j] / l1).astype(BF16)
                lchk[0] = lo
                lchk[1] = hi

            def unit(kb):
                def f():
                    if kb == 0:
                        setup()
                    if kb < NK:
                        qk(kb)
                    if kb >= A_SKEW:
                        pv(kb - A_SKEW)
                    if kb == NK + A_SKEW - 1:
                        finish()
                return f

            return [unit(kb) for kb in range(NK + A_SKEW)]

        def b_slots(s):
            st = {"qkv": {}, "ps": {}, "os": {}, "outs": [None] * NG}
            r0 = pl.multiple_of(s * SEG, SEG)

            def setup():
                hbuf[M:L, :] = xb[pl.ds(r0, SEG), :].astype(F32)
                st["X"] = hbuf[...]
                row = lax.broadcasted_iota(jnp.int32, (L, L), 0)
                col = lax.broadcasted_iota(jnp.int32, (L, L), 1)
                st["mask"] = (row < M) | (row >= col)

            def proj(h):
                st["qkv"][h] = [_dot(st["X"], pltpu.bitcast(wb[t, h], BF16)) for t in range(3)]

            def qk(h):
                q, k, _ = st["qkv"][h]
                sc = _dot_nt(q, k.astype(BF16)) * bscale
                sc = jnp.where(st["mask"], sc, -1e9)
                m = jnp.max(sc, axis=-1, keepdims=True)
                p = jnp.exp(sc - m)
                st["ps"][h] = p / jnp.sum(p, axis=-1, keepdims=True)

            def pv(h):
                v = st["qkv"].pop(h)[2]
                st["os"][h] = _dot(st["ps"].pop(h), v.astype(BF16))

            def outp(h):
                o = st["os"].pop(h)
                outs = st["outs"]
                for n in range(NG):
                    t = _dot(o, pltpu.bitcast(wob[n, h], BF16))
                    outs[n] = t if outs[n] is None else outs[n] + t
                if h % GRP == GRP - 1:
                    for n in range(NG):
                        if h == GRP - 1:
                            obuf[:, n * LANES:(n + 1) * LANES] = outs[n]
                        else:
                            obuf[:, n * LANES:(n + 1) * LANES] += outs[n]
                        outs[n] = None

            def finish():
                o = obuf[...]
                hbuf[0:M, :] = o[0:M].astype(BF16).astype(F32)
                bbuf[pl.ds(r0, SEG), :] = o[M:L]

            def slot(t):
                def f():
                    if t == 0:
                        setup()
                    if t < HB:
                        proj(t)
                    if 0 <= t - SKEW[0] < HB:
                        qk(t - SKEW[0])
                    if 0 <= t - SKEW[1] < HB:
                        pv(t - SKEW[1])
                    if 0 <= t - SKEW[2] < HB:
                        outp(t - SKEW[2])
                    if t == HB + SKEW[2] - 1:
                        finish()
                return f

            return [slot(t) for t in range(HB + SKEW[2])]

        def main_step(s):
            h = s * QPS // NQ
            qb0 = (s * QPS) % NQ
            units = []
            for i in range(QPS):
                u = a_units(h, qb0 + i)
                for k in range(A_SKEW):
                    if len(units) >= A_SKEW:
                        last = units[len(units) - A_SKEW + k]
                        u[k] = (lambda a=u[k], b=last: (a(), b()))
                if units:
                    units = units[:len(units) - A_SKEW]
                units += u
            slots = b_slots(s)
            ns, nu = len(slots), len(units)
            nd = nu - A_SKEW
            pos = [ns - A_END - A_SKEW - A_STRIDE * (nd - 1 - i) for i in range(nd)]
            pos += [ns - A_END - A_SKEW + 1 + k for k in range(A_SKEW)]
            for t in range(ns):
                slots[t]()
                for i in range(nu):
                    if min(max(pos[i], 0), ns - 1) == t:
                        units[i]()

        def main_iter(it, carry):
            @pl.when(it == TB // SEG // UNROLL)
            def _():
                cp_xb1.wait()

            for k in range(UNROLL):
                main_step(it * UNROLL + k)
            return carry

        lax.fori_loop(0, NSEG // UNROLL, main_iter, 0)

        ok = jnp.logical_and(lchk[0] >= L_MIN, lchk[1] <= L_MAX)
        n_bad = jnp.sum(jnp.where(ok, 0.0, 1.0))

        @pl.when(n_bad > 0.0)
        def _exact_softmax_fallback():
            def body(it, carry):
                h = it // (S // LANES)
                qb = it % (S // LANES)
                h0 = pl.multiple_of(h * DHA, DHA)
                q0 = pl.multiple_of(qb * LANES, LANES)
                g, qm = head_masked_q(h, q0)
                m = jnp.full((8, LANES), -jnp.inf, F32)
                for kb in range(NK):
                    s = _dot(kk[g, kb * TK:(kb + 1) * TK, :], qm)
                    sbuf[kb * TK:(kb + 1) * TK, :] = s
                    m = jnp.maximum(m, jnp.max(s.reshape(TK // 8, 8, LANES), axis=0))
                m1 = jnp.max(m, axis=0, keepdims=True)
                l = jnp.zeros((8, LANES), F32)
                acc = jnp.zeros((DHA, LANES), F32)
                for kb in range(NK):
                    p = jnp.exp2(sbuf[kb * TK:(kb + 1) * TK, :] - m1)
                    l = l + jnp.sum(p.reshape(TK // 8, 8, LANES), axis=0)
                    acc = acc + _dot(vt[pl.ds(h0, DHA), kb * TK:(kb + 1) * TK], p.astype(BF16))
                l1 = jnp.sum(l, axis=0, keepdims=True)
                ot[pl.ds(h0, DHA), pl.ds(q0, LANES)] = (acc / l1).astype(BF16)
                return carry

            lax.fori_loop(0, HA * (S // LANES), body, 0)

        cp_woa.wait()

        out_cps = []
        for i in range(S // TM):
            r0 = i * TM
            a = _dot_tn(ot[:, r0:r0 + TM], woa[...])
            g = gl[r0:r0 + TM, :]
            for n in range(NG):
                sl = slice(n * LANES, (n + 1) * LANES)
                outv[r0:r0 + TM, sl] = (g * a[:, sl] + (1.0 - g) * bbuf[r0:r0 + TM, sl]).astype(BF16)
            cp = pltpu.make_async_copy(outv.at[r0:r0 + TM, :], out_hbm.at[0, r0:r0 + TM, :], sem_out.at[i])
            cp.start()
            out_cps.append(cp)
        for cp in out_cps:
            cp.wait()

    return kernel


@functools.partial(jax.jit, static_argnames=("B_seg_len",))
def pallas_gated_mix__softmax_full_mha__memory_aug_recurrent_mem_tr__prompt_kernel(
    A_x: jax.Array,
    A_wqkv: jax.Array,
    A_wo: jax.Array,
    B_x: jax.Array,
    B_mem0: jax.Array,
    B_Wq: jax.Array,
    B_Wk: jax.Array,
    B_Wv: jax.Array,
    B_Wo: jax.Array,
    B_seg_len: int,
    gate_w: jax.Array,
):
    _, S, D = A_x.shape
    _, HB, DHB = B_Wq.shape
    M = B_mem0.shape[1]
    SEG = int(B_seg_len)
    NG = D // LANES
    wq, wk, wv = (w.reshape(D // 2, 2 * HB, DHB) for w in (B_Wq, B_Wk, B_Wv))

    any_spec = pl.BlockSpec(memory_space=pl.ANY)
    scratch = [
        pltpu.VMEM((S, D), BF16),
        pltpu.VMEM((D, 3 * D), BF16),
        pltpu.VMEM((D, D), BF16),
        pltpu.VMEM((S, D), BF16),
        pltpu.VMEM((M, D), BF16),
        pltpu.VMEM((D,), BF16),
        pltpu.VMEM((3, HB, D // 2, DHB), U32),
        pltpu.VMEM((NG, HB, DHB // 2, LANES), U32),
        pltpu.VMEM((NG, LANES, S), BF16),
        pltpu.VMEM((NG, S, LANES), BF16),
        pltpu.VMEM((D, S), BF16),
        pltpu.VMEM((D, S), BF16),
        pltpu.VMEM((NG, 8, LANES), F32),
        pltpu.VMEM((NG, LANES, LANES), F32),
        pltpu.VMEM((2, 8, LANES), F32),
        pltpu.VMEM((S, LANES), F32),
        pltpu.VMEM((S, D), F32),
        pltpu.VMEM((M + SEG, D), F32),
        pltpu.VMEM((M + SEG, D), F32),
        pltpu.VMEM((S, LANES), F32),
        pltpu.VMEM((S, D), BF16),
        pltpu.SemaphoreType.DMA((2,)),
        pltpu.SemaphoreType.DMA((len(WCH),)),
        pltpu.SemaphoreType.DMA((5,)),
        pltpu.SemaphoreType.DMA((3 * HB,)),
        pltpu.SemaphoreType.DMA((NG,)),
        pltpu.SemaphoreType.DMA((S // TM,)),
    ]
    return pl.pallas_call(
        _make_kernel(S, D, HB, DHB, M, SEG),
        out_shape=jax.ShapeDtypeStruct((1, S, D), BF16),
        in_specs=[any_spec] * 10,
        out_specs=any_spec,
        scratch_shapes=scratch,
        compiler_params=pltpu.CompilerParams(vmem_limit_bytes=120 * 1024 * 1024),
        name="gated_mix",
    )(A_x, A_wqkv, A_wo, B_x, B_mem0, wq, wk, wv, B_Wo, gate_w)
```

```python
import functools
import math

import jax
import jax.numpy as jnp
from jax import lax
import jax.experimental.pallas as pl
import jax.experimental.pallas.tpu as pltpu

F32 = jnp.float32
BF16 = jnp.bfloat16
U32 = jnp.uint32

LANES = 128
HA = 32
TQ = 512
TK = 256
TM = 256
NSUB = 2
WCH = (2, 4, 8, 10)
REP_RC = 16
L_MIN = 2.0 ** -64
L_MAX = 2.0 ** 64
SKEW = (1, 3, 5)
GRP = 8
A_SKEW = 1
A_END = 4
UNROLL = 2
A_STRIDE = 2


def _dot(a, b):
    return lax.dot_general(a, b, (((1,), (0,)), ((), ())), preferred_element_type=F32)


def _dot_nt(a, b):
    return lax.dot_general(a, b, (((1,), (1,)), ((), ())), preferred_element_type=F32)


def _dot_tn(a, b):
    return lax.dot_general(a, b, (((0,), (0,)), ((), ())), preferred_element_type=F32)


def _make_kernel(S, D, HB, DHB, M, SEG):
    DHA = D // HA
    HPG = LANES // DHA
    NG = D // LANES
    L = M + SEG
    NSEG = S // SEG
    NQ = S // TQ
    NK = S // TK
    J = TQ // LANES
    TB = TM * NSUB
    NBLK = S // TB
    NPAIR = HB // 2
    assert sum(WCH) == 3 * NG
    WOFF = [sum(WCH[:k]) for k in range(len(WCH))]
    QPS = HA * NQ // NSEG
    assert QPS * NSEG == HA * NQ and NQ % QPS == 0
    qscale = (DHA ** -0.5) * math.log2(math.e)
    bscale = DHB ** -0.5

    def kernel(xa_hbm, wqkv_hbm, woa_hbm, mem_hbm, wq_hbm, wk_hbm, wv_hbm, wob_hbm, gate_hbm,
               out_hbm,
               xa, wqkv, woa, mem, gate, wb, wob,
               qt, kk, vt, ot, kmax, kmt, lchk, gl, bbuf, hbuf, obuf, sbuf, outv,
               sem_x, sem_wa, sem_in, sem_w, sem_wo, sem_out):
        cp_x0 = pltpu.make_async_copy(xa_hbm.at[0, 0:TB, :], xa.at[0:TB, :], sem_x.at[0])
        cp_xr = pltpu.make_async_copy(xa_hbm.at[0, TB:S, :], xa.at[TB:S, :], sem_x.at[1])
        cp_wa = [pltpu.make_async_copy(wqkv_hbm.at[:, o * LANES:(o + n) * LANES],
                                       wqkv.at[:, o * LANES:(o + n) * LANES], sem_wa.at[k])
                 for k, (o, n) in enumerate(zip(WOFF, WCH))]
        cp_gate = pltpu.make_async_copy(gate_hbm, gate, sem_in.at[0])
        cp_woa = pltpu.make_async_copy(woa_hbm, woa, sem_in.at[1])
        cp_mem = pltpu.make_async_copy(mem_hbm.at[0], mem, sem_in.at[2])

        def w_copies(t):
            src = (wq_hbm, wk_hbm, wv_hbm)[t].bitcast(U32)
            return [pltpu.make_async_copy(src.at[:, r, :], wb.at[t, 2 * (r % NPAIR) + r // NPAIR],
                                          sem_w.at[t * HB + r]) for r in range(HB)]

        w_cps = [w_copies(t) for t in range(3)]
        wob_u = wob_hbm.bitcast(U32)
        wo_cps = [pltpu.make_async_copy(wob_u.at[:, :, n * LANES:(n + 1) * LANES], wob.at[n], sem_wo.at[n])
                  for n in range(NG)]

        hw = HB // 2

        def sync(waits, starts):
            for cp in waits:
                cp.wait()
            for cp in starts:
                cp.start()

        sync0 = {WOFF[1]: ([cp_wa[1]], [cp_xr]),
                 WOFF[2]: ([cp_wa[2]], w_cps[0]),
                 WOFF[3]: ([cp_wa[3]], w_cps[1])}
        sync1 = {0: ([cp_xr], []),
                 2 * NG: (w_cps[0], w_cps[2])}
        sync2 = {NG + NG // 2: (w_cps[1], wo_cps + [cp_mem, cp_woa])}
        sync3 = {NG - 2: (w_cps[2], [])}
        cp_gate.start()
        cp_x0.start()
        cp_wa[0].start()
        cp_wa[1].start()

        kmax[...] = jnp.zeros(kmax.shape, F32)

        def repack(t, j, anchor):
            z = (pltpu.bitcast(anchor, U32) & jnp.uint32(0x7FFF)) >> 15
            for r in range(0, D // 2, REP_RC):
                zz = jnp.concatenate([z] * (REP_RC // 8), axis=0)
                e = wb[t, 2 * j, r:r + REP_RC, :] | zz
                o = wb[t, 2 * j + 1, r:r + REP_RC, :]
                lo = (e & jnp.uint32(0xFFFF)) | (o << 16)
                wb[t, 2 * j, r:r + REP_RC, :] = lo
                wb[t, 2 * j + 1, r:r + REP_RC, :] = (e >> 16) | (o & jnp.uint32(0xFFFF0000))
                z = (lo[0:8, :] & jnp.uint32(0x7FFF)) >> 15

        def a_proj(i, syncs, rep=()):
            rep = list(rep)
            r0s = [i * TB + u * TM for u in range(NSUB)]
            prev = None
            for c in range(3 * NG):
                if c in syncs:
                    sync(*syncs[c])
                    prev = None
                for u in range(NSUB):
                    r0 = r0s[u]
                    xu = xa[r0:r0 + TM, :]
                    r = _dot(xu, wqkv[:, c * LANES:(c + 1) * LANES])
                    if c < NG:
                        qt[c, :, r0:r0 + TM] = (r * qscale).T.astype(BF16)
                    elif c < 2 * NG:
                        g = c - NG
                        rb = r.astype(BF16)
                        kk[g, r0:r0 + TM, :] = rb
                        ab = jnp.abs(rb.astype(F32))
                        kmax[g] = jnp.maximum(kmax[g], jnp.max(ab.reshape(TM // 8, 8, LANES), axis=0))
                    else:
                        g = c - 2 * NG
                        vt[g * LANES:(g + 1) * LANES, r0:r0 + TM] = r.T.astype(BF16)
                    while prev is not None and rep and rep[0][0] <= c * NSUB + u:
                        _, t, j = rep.pop(0)
                        repack(t, j, prev)
                    prev = r[0:8, :]
                    if c == NG + 2 + 4 * u:
                        gv = gate[...].astype(F32).reshape(1, D)
                        logit = jnp.sum(xu.astype(F32) * gv, axis=-1, keepdims=True)
                        gl[r0:r0 + TM, :] = jnp.broadcast_to(jax.nn.sigmoid(logit), (TM, LANES))

        ndots = 3 * NG * NSUB
        sync([cp_gate, cp_x0, cp_wa[0]], [cp_wa[2], cp_wa[3]])
        a_proj(0, sync0)
        a_proj(1, sync1)
        k1 = (NG + NG // 2) * NSUB + 1
        k2 = (NG - 2) * NSUB + 1
        n2 = NPAIR // 2
        a_proj(2, sync2, rep=[(1 + j * (k1 - 2) // NPAIR, 0, j) for j in range(NPAIR)]
               + [(k1 + j * (ndots - k1 - 1) // n2, 1, j) for j in range(n2)])
        a_proj(3, sync3, rep=[(1 + j * (k2 - 2) // (NPAIR - n2), 1, n2 + j) for j in range(NPAIR - n2)]
               + [(k2 + j * (ndots - k2 - 1) // NPAIR, 2, j) for j in range(NPAIR)])

        for g in range(NG):
            km = jnp.max(kmax[g], axis=0, keepdims=True)
            kmt[g] = jnp.broadcast_to(km, (LANES, LANES)).T

        lchk[0] = jnp.full((8, LANES), L_MAX, F32)
        lchk[1] = jnp.full((8, LANES), L_MIN, F32)

        for c in wo_cps:
            c.wait()
        cp_mem.wait()
        hbuf[0:M, :] = mem[...].astype(F32)

        def head_masked_q(h, q0):
            g = h // HPG
            r = h % HPG
            rows = lax.broadcasted_iota(jnp.int32, (LANES, LANES), 0)
            msk = (rows >= r * DHA) & (rows < r * DHA + DHA)
            q = qt[g, :, pl.ds(q0, LANES)]
            return g, jnp.where(msk, q, jnp.zeros_like(q))

        def a_units(h, qb):
            st = {}
            h0 = pl.multiple_of(h * DHA, DHA)

            def setup():
                st["qms"], st["bnd"] = [], []
                for j in range(J):
                    q0 = pl.multiple_of(qb * TQ + j * LANES, LANES)
                    g, qm = head_masked_q(h, q0)
                    st["g"] = g
                    st["qms"].append(qm)
                    bb = jnp.abs(qm.astype(F32)) * kmt[g]
                    bb = jnp.sum(bb, axis=0, keepdims=True) * (1.0 + 2.0 ** -10)
                    st["bnd"].append(jnp.broadcast_to(bb, (8, LANES)))
                st["ls"] = [jnp.zeros((8, LANES), F32) for _ in range(J)]
                st["accs"] = [jnp.zeros((DHA, LANES), F32) for _ in range(J)]
                st["ps"] = {}

            def qk(kb):
                kblk = kk[st["g"], kb * TK:(kb + 1) * TK, :]
                for j in range(J):
                    s = _dot(kblk, st["qms"][j]).reshape(TK // 8, 8, LANES)
                    p = jnp.exp2(s - st["bnd"][j][None])
                    st["ls"][j] = st["ls"][j] + jnp.sum(p, axis=0)
                    st["ps"][(kb, j)] = p.reshape(TK, LANES).astype(BF16)

            def pv(kb):
                vblk = vt[pl.ds(h0, DHA), kb * TK:(kb + 1) * TK]
                for j in range(J):
                    st["accs"][j] = st["accs"][j] + _dot(vblk, st["ps"].pop((kb, j)))

            def finish():
                lo = lchk[0]
                hi = lchk[1]
                for j in range(J):
                    l1 = jnp.sum(st["ls"][j], axis=0, keepdims=True)
                    l8 = jnp.broadcast_to(l1, (8, LANES))
                    lo = jnp.where(l8 >= lo, lo, l8)
                    hi = jnp.where(l8 <= hi, hi, l8)
                    q0 = pl.multiple_of(qb * TQ + j * LANES, LANES)
                    ot[pl.ds(h0, DHA), pl.ds(q0, LANES)] = (st["accs"][j] / l1).astype(BF16)
                lchk[0] = lo
                lchk[1] = hi

            def unit(kb):
                def f():
                    if kb == 0:
                        setup()
                    if kb < NK:
                        qk(kb)
                    if kb >= A_SKEW:
                        pv(kb - A_SKEW)
                    if kb == NK + A_SKEW - 1:
                        finish()
                return f

            return [unit(kb) for kb in range(NK + A_SKEW)]

        def b_slots(s):
            st = {"qkv": {}, "ps": {}, "os": {}, "outs": [None] * NG}
            r0 = pl.multiple_of(s * SEG, SEG)

            def setup():
                hbuf[M:L, :] = xa[pl.ds(r0, SEG), :].astype(F32)
                st["X"] = hbuf[...]
                row = lax.broadcasted_iota(jnp.int32, (L, L), 0)
                col = lax.broadcasted_iota(jnp.int32, (L, L), 1)
                st["mask"] = (row < M) | (row >= col)

            def proj(h):
                st["qkv"][h] = [_dot(st["X"], pltpu.bitcast(wb[t, h], BF16)) for t in range(3)]

            def qk(h):
                q, k, _ = st["qkv"][h]
                sc = _dot_nt(q, k.astype(BF16)) * bscale
                sc = jnp.where(st["mask"], sc, -1e9)
                m = jnp.max(sc, axis=-1, keepdims=True)
                p = jnp.exp(sc - m)
                st["ps"][h] = p / jnp.sum(p, axis=-1, keepdims=True)

            def pv(h):
                v = st["qkv"].pop(h)[2]
                st["os"][h] = _dot(st["ps"].pop(h), v.astype(BF16))

            def outp(h):
                o = st["os"].pop(h)
                outs = st["outs"]
                for n in range(NG):
                    t = _dot(o, pltpu.bitcast(wob[n, h], BF16))
                    outs[n] = t if outs[n] is None else outs[n] + t
                if h % GRP == GRP - 1:
                    for n in range(NG):
                        if h == GRP - 1:
                            obuf[:, n * LANES:(n + 1) * LANES] = outs[n]
                        else:
                            obuf[:, n * LANES:(n + 1) * LANES] += outs[n]
                        outs[n] = None

            def finish():
                o = obuf[...]
                hbuf[0:M, :] = o[0:M].astype(BF16).astype(F32)
                bbuf[pl.ds(r0, SEG), :] = o[M:L]

            def slot(t):
                def f():
                    if t == 0:
                        setup()
                    if t < HB:
                        proj(t)
                    if 0 <= t - SKEW[0] < HB:
                        qk(t - SKEW[0])
                    if 0 <= t - SKEW[1] < HB:
                        pv(t - SKEW[1])
                    if 0 <= t - SKEW[2] < HB:
                        outp(t - SKEW[2])
                    if t == HB + SKEW[2] - 1:
                        finish()
                return f

            return [slot(t) for t in range(HB + SKEW[2])]

        def main_step(s):
            h = s * QPS // NQ
            qb0 = (s * QPS) % NQ
            units = []
            for i in range(QPS):
                u = a_units(h, qb0 + i)
                for k in range(A_SKEW):
                    if len(units) >= A_SKEW:
                        last = units[len(units) - A_SKEW + k]
                        u[k] = (lambda a=u[k], b=last: (a(), b()))
                if units:
                    units = units[:len(units) - A_SKEW]
                units += u
            slots = b_slots(s)
            ns, nu = len(slots), len(units)
            nd = nu - A_SKEW
            pos = [ns - A_END - A_SKEW - A_STRIDE * (nd - 1 - i) for i in range(nd)]
            pos += [ns - A_END - A_SKEW + 1 + k for k in range(A_SKEW)]
            for t in range(ns):
                slots[t]()
                for i in range(nu):
                    if min(max(pos[i], 0), ns - 1) == t:
                        units[i]()

        def main_iter(it, carry):
            for k in range(UNROLL):
                main_step(it * UNROLL + k)
            return carry

        lax.fori_loop(0, NSEG // UNROLL, main_iter, 0)

        ok = jnp.logical_and(lchk[0] >= L_MIN, lchk[1] <= L_MAX)
        n_bad = jnp.sum(jnp.where(ok, 0.0, 1.0))

        @pl.when(n_bad > 0.0)
        def _exact_softmax_fallback():
            def body(it, carry):
                h = it // (S // LANES)
                qb = it % (S // LANES)
                h0 = pl.multiple_of(h * DHA, DHA)
                q0 = pl.multiple_of(qb * LANES, LANES)
                g, qm = head_masked_q(h, q0)
                m = jnp.full((8, LANES), -jnp.inf, F32)
                for kb in range(NK):
                    s = _dot(kk[g, kb * TK:(kb + 1) * TK, :], qm)
                    sbuf[kb * TK:(kb + 1) * TK, :] = s
                    m = jnp.maximum(m, jnp.max(s.reshape(TK // 8, 8, LANES), axis=0))
                m1 = jnp.max(m, axis=0, keepdims=True)
                l = jnp.zeros((8, LANES), F32)
                acc = jnp.zeros((DHA, LANES), F32)
                for kb in range(NK):
                    p = jnp.exp2(sbuf[kb * TK:(kb + 1) * TK, :] - m1)
                    l = l + jnp.sum(p.reshape(TK // 8, 8, LANES), axis=0)
                    acc = acc + _dot(vt[pl.ds(h0, DHA), kb * TK:(kb + 1) * TK], p.astype(BF16))
                l1 = jnp.sum(l, axis=0, keepdims=True)
                ot[pl.ds(h0, DHA), pl.ds(q0, LANES)] = (acc / l1).astype(BF16)
                return carry

            lax.fori_loop(0, HA * (S // LANES), body, 0)

        cp_woa.wait()

        out_cps = []
        for i in range(S // TM):
            r0 = i * TM
            a = _dot_tn(ot[:, r0:r0 + TM], woa[...])
            g = gl[r0:r0 + TM, :]
            for n in range(NG):
                sl = slice(n * LANES, (n + 1) * LANES)
                outv[r0:r0 + TM, sl] = (g * a[:, sl] + (1.0 - g) * bbuf[r0:r0 + TM, sl]).astype(BF16)
            cp = pltpu.make_async_copy(outv.at[r0:r0 + TM, :], out_hbm.at[0, r0:r0 + TM, :], sem_out.at[i])
            cp.start()
            out_cps.append(cp)
        for cp in out_cps:
            cp.wait()

    return kernel


@functools.partial(jax.jit, static_argnames=("B_seg_len",))
def pallas_gated_mix__softmax_full_mha__memory_aug_recurrent_mem_tr__prompt_kernel(
    A_x: jax.Array,
    A_wqkv: jax.Array,
    A_wo: jax.Array,
    B_x: jax.Array,
    B_mem0: jax.Array,
    B_Wq: jax.Array,
    B_Wk: jax.Array,
    B_Wv: jax.Array,
    B_Wo: jax.Array,
    B_seg_len: int,
    gate_w: jax.Array,
):
    del B_x
    _, S, D = A_x.shape
    _, HB, DHB = B_Wq.shape
    M = B_mem0.shape[1]
    SEG = int(B_seg_len)
    NG = D // LANES
    wq, wk, wv = (w.reshape(D // 2, 2 * HB, DHB) for w in (B_Wq, B_Wk, B_Wv))

    any_spec = pl.BlockSpec(memory_space=pl.ANY)
    scratch = [
        pltpu.VMEM((S, D), BF16),
        pltpu.VMEM((D, 3 * D), BF16),
        pltpu.VMEM((D, D), BF16),
        pltpu.VMEM((M, D), BF16),
        pltpu.VMEM((D,), BF16),
        pltpu.VMEM((3, HB, D // 2, DHB), U32),
        pltpu.VMEM((NG, HB, DHB // 2, LANES), U32),
        pltpu.VMEM((NG, LANES, S), BF16),
        pltpu.VMEM((NG, S, LANES), BF16),
        pltpu.VMEM((D, S), BF16),
        pltpu.VMEM((D, S), BF16),
        pltpu.VMEM((NG, 8, LANES), F32),
        pltpu.VMEM((NG, LANES, LANES), F32),
        pltpu.VMEM((2, 8, LANES), F32),
        pltpu.VMEM((S, LANES), F32),
        pltpu.VMEM((S, D), F32),
        pltpu.VMEM((M + SEG, D), F32),
        pltpu.VMEM((M + SEG, D), F32),
        pltpu.VMEM((S, LANES), F32),
        pltpu.VMEM((S, D), BF16),
        pltpu.SemaphoreType.DMA((2,)),
        pltpu.SemaphoreType.DMA((len(WCH),)),
        pltpu.SemaphoreType.DMA((3,)),
        pltpu.SemaphoreType.DMA((3 * HB,)),
        pltpu.SemaphoreType.DMA((NG,)),
        pltpu.SemaphoreType.DMA((S // TM,)),
    ]
    return pl.pallas_call(
        _make_kernel(S, D, HB, DHB, M, SEG),
        out_shape=jax.ShapeDtypeStruct((1, S, D), BF16),
        in_specs=[any_spec] * 9,
        out_specs=any_spec,
        scratch_shapes=scratch,
        compiler_params=pltpu.CompilerParams(vmem_limit_bytes=120 * 1024 * 1024),
        name="gated_mix",
    )(A_x, A_wqkv, A_wo, B_mem0, wq, wk, wv, B_Wo, gate_w)
```

```python
import functools
import math

import jax
import jax.numpy as jnp
from jax import lax
import jax.experimental.pallas as pl
import jax.experimental.pallas.tpu as pltpu

F32 = jnp.float32
BF16 = jnp.bfloat16
U32 = jnp.uint32

LANES = 128
HA = 32
TQ = 512
TK = 256
TM = 256
NSUB = 2
WCH = (2, 4, 8, 10)
REP_RC = 16
L_MIN = 2.0 ** -64
L_MAX = 2.0 ** 64
SKEW = (1, 3, 5)
GRP = 8
A_SKEW = 1
A_END = 4
UNROLL = 2
A_START = 2


def _dot(a, b):
    return lax.dot_general(a, b, (((1,), (0,)), ((), ())), preferred_element_type=F32)


def _dot_nt(a, b):
    return lax.dot_general(a, b, (((1,), (1,)), ((), ())), preferred_element_type=F32)


def _dot_tn(a, b):
    return lax.dot_general(a, b, (((0,), (0,)), ((), ())), preferred_element_type=F32)


def _make_kernel(S, D, HB, DHB, M, SEG):
    DHA = D // HA
    HPG = LANES // DHA
    NG = D // LANES
    L = M + SEG
    NSEG = S // SEG
    NQ = S // TQ
    NK = S // TK
    J = TQ // LANES
    TB = TM * NSUB
    NBLK = S // TB
    NPAIR = HB // 2
    assert sum(WCH) == 3 * NG
    WOFF = [sum(WCH[:k]) for k in range(len(WCH))]
    QPS = HA * NQ // NSEG
    assert QPS * NSEG == HA * NQ and NQ % QPS == 0
    qscale = (DHA ** -0.5) * math.log2(math.e)
    bscale = DHB ** -0.5

    def kernel(xa_hbm, wqkv_hbm, woa_hbm, mem_hbm, wq_hbm, wk_hbm, wv_hbm, wob_hbm, gate_hbm,
               out_hbm,
               xa, wqkv, woa, mem, gate, wb, wob,
               qt, kk, vt, ot, kmax, kmt, lchk, gl, bbuf, hbuf, obuf, sbuf, outv,
               sem_x, sem_wa, sem_in, sem_w, sem_wo, sem_out):
        cp_x0 = pltpu.make_async_copy(xa_hbm.at[0, 0:TB, :], xa.at[0:TB, :], sem_x.at[0])
        cp_xr = pltpu.make_async_copy(xa_hbm.at[0, TB:S, :], xa.at[TB:S, :], sem_x.at[1])
        cp_wa = [pltpu.make_async_copy(wqkv_hbm.at[:, o * LANES:(o + n) * LANES],
                                       wqkv.at[:, o * LANES:(o + n) * LANES], sem_wa.at[k])
                 for k, (o, n) in enumerate(zip(WOFF, WCH))]
        cp_gate = pltpu.make_async_copy(gate_hbm, gate, sem_in.at[0])
        cp_woa = pltpu.make_async_copy(woa_hbm, woa, sem_in.at[1])
        cp_mem = pltpu.make_async_copy(mem_hbm.at[0], mem, sem_in.at[2])

        def w_copies(t):
            src = (wq_hbm, wk_hbm, wv_hbm)[t].bitcast(U32)
            return [pltpu.make_async_copy(src.at[:, r, :], wb.at[t, 2 * (r % NPAIR) + r // NPAIR],
                                          sem_w.at[t * HB + r]) for r in range(HB)]

        w_cps = [w_copies(t) for t in range(3)]
        wob_u = wob_hbm.bitcast(U32)
        wo_cps = [pltpu.make_async_copy(wob_u.at[:, :, n * LANES:(n + 1) * LANES], wob.at[n], sem_wo.at[n])
                  for n in range(NG)]

        hw = HB // 2

        def sync(waits, starts):
            for cp in waits:
                cp.wait()
            for cp in starts:
                cp.start()

        sync0 = {WOFF[1]: ([cp_wa[1]], [cp_xr]),
                 WOFF[2]: ([cp_wa[2]], w_cps[0]),
                 WOFF[3]: ([cp_wa[3]], w_cps[1])}
        sync1 = {0: ([cp_xr], []),
                 2 * NG: (w_cps[0], w_cps[2])}
        sync2 = {NG + NG // 2: (w_cps[1], wo_cps + [cp_mem, cp_woa])}
        sync3 = {NG - 2: (w_cps[2], [])}
        cp_gate.start()
        cp_x0.start()
        cp_wa[0].start()
        cp_wa[1].start()

        kmax[...] = jnp.zeros(kmax.shape, F32)

        def repack(t, j, anchor):
            z = (pltpu.bitcast(anchor, U32) & jnp.uint32(0x7FFF)) >> 15
            for r in range(0, D // 2, REP_RC):
                zz = jnp.concatenate([z] * (REP_RC // 8), axis=0)
                e = wb[t, 2 * j, r:r + REP_RC, :] | zz
                o = wb[t, 2 * j + 1, r:r + REP_RC, :]
                lo = (e & jnp.uint32(0xFFFF)) | (o << 16)
                wb[t, 2 * j, r:r + REP_RC, :] = lo
                wb[t, 2 * j + 1, r:r + REP_RC, :] = (e >> 16) | (o & jnp.uint32(0xFFFF0000))
                z = (lo[0:8, :] & jnp.uint32(0x7FFF)) >> 15

        def a_proj(i, syncs, rep=()):
            rep = list(rep)
            r0s = [i * TB + u * TM for u in range(NSUB)]
            prev = None
            for c in range(3 * NG):
                if c in syncs:
                    sync(*syncs[c])
                    prev = None
                for u in range(NSUB):
                    r0 = r0s[u]
                    xu = xa[r0:r0 + TM, :]
                    r = _dot(xu, wqkv[:, c * LANES:(c + 1) * LANES])
                    if c < NG:
                        qt[c, :, r0:r0 + TM] = (r * qscale).T.astype(BF16)
                    elif c < 2 * NG:
                        g = c - NG
                        rb = r.astype(BF16)
                        kk[g, r0:r0 + TM, :] = rb
                        ab = jnp.abs(rb.astype(F32))
                        kmax[g] = jnp.maximum(kmax[g], jnp.max(ab.reshape(TM // 8, 8, LANES), axis=0))
                    else:
                        g = c - 2 * NG
                        vt[g * LANES:(g + 1) * LANES, r0:r0 + TM] = r.T.astype(BF16)
                    while prev is not None and rep and rep[0][0] <= c * NSUB + u:
                        _, t, j = rep.pop(0)
                        repack(t, j, prev)
                    prev = r[0:8, :]
                    if c == NG + 2 + 4 * u:
                        gv = gate[...].astype(F32).reshape(1, D)
                        logit = jnp.sum(xu.astype(F32) * gv, axis=-1, keepdims=True)
                        gl[r0:r0 + TM, :] = jnp.broadcast_to(jax.nn.sigmoid(logit), (TM, LANES))

        ndots = 3 * NG * NSUB
        sync([cp_gate, cp_x0, cp_wa[0]], [cp_wa[2], cp_wa[3]])
        a_proj(0, sync0)
        a_proj(1, sync1)
        k1 = (NG + NG // 2) * NSUB + 1
        k2 = (NG - 2) * NSUB + 1
        n2 = NPAIR // 2
        a_proj(2, sync2, rep=[(1 + j * (k1 - 2) // NPAIR, 0, j) for j in range(NPAIR)]
               + [(k1 + j * (ndots - k1 - 1) // n2, 1, j) for j in range(n2)])
        a_proj(3, sync3, rep=[(1 + j * (k2 - 2) // (NPAIR - n2), 1, n2 + j) for j in range(NPAIR - n2)]
               + [(k2 + j * (ndots - k2 - 1) // NPAIR, 2, j) for j in range(NPAIR)])

        for g in range(NG):
            km = jnp.max(kmax[g], axis=0, keepdims=True)
            kmt[g] = jnp.broadcast_to(km, (LANES, LANES)).T

        lchk[0] = jnp.full((8, LANES), L_MAX, F32)
        lchk[1] = jnp.full((8, LANES), L_MIN, F32)

        for c in wo_cps:
            c.wait()
        cp_mem.wait()
        hbuf[0:M, :] = mem[...].astype(F32)

        def head_masked_q(h, q0):
            g = h // HPG
            r = h % HPG
            rows = lax.broadcasted_iota(jnp.int32, (LANES, LANES), 0)
            msk = (rows >= r * DHA) & (rows < r * DHA + DHA)
            q = qt[g, :, pl.ds(q0, LANES)]
            return g, jnp.where(msk, q, jnp.zeros_like(q))

        def a_units(h, qb):
            st = {}
            h0 = pl.multiple_of(h * DHA, DHA)

            def setup():
                st["qms"], st["bnd"] = [], []
                for j in range(J):
                    q0 = pl.multiple_of(qb * TQ + j * LANES, LANES)
                    g, qm = head_masked_q(h, q0)
                    st["g"] = g
                    st["qms"].append(qm)
                    bb = jnp.abs(qm.astype(F32)) * kmt[g]
                    bb = jnp.sum(bb, axis=0, keepdims=True) * (1.0 + 2.0 ** -10)
                    st["bnd"].append(jnp.broadcast_to(bb, (8, LANES)))
                st["ls"] = [jnp.zeros((8, LANES), F32) for _ in range(J)]
                st["accs"] = [jnp.zeros((DHA, LANES), F32) for _ in range(J)]
                st["ps"] = {}

            def qk(kb):
                kblk = kk[st["g"], kb * TK:(kb + 1) * TK, :]
                for j in range(J):
                    s = _dot(kblk, st["qms"][j]).reshape(TK // 8, 8, LANES)
                    p = jnp.exp2(s - st["bnd"][j][None])
                    st["ls"][j] = st["ls"][j] + jnp.sum(p, axis=0)
                    st["ps"][(kb, j)] = p.reshape(TK, LANES).astype(BF16)

            def pv(kb):
                vblk = vt[pl.ds(h0, DHA), kb * TK:(kb + 1) * TK]
                for j in range(J):
                    st["accs"][j] = st["accs"][j] + _dot(vblk, st["ps"].pop((kb, j)))

            def finish():
                lo = lchk[0]
                hi = lchk[1]
                for j in range(J):
                    l1 = jnp.sum(st["ls"][j], axis=0, keepdims=True)
                    l8 = jnp.broadcast_to(l1, (8, LANES))
                    lo = jnp.where(l8 >= lo, lo, l8)
                    hi = jnp.where(l8 <= hi, hi, l8)
                    q0 = pl.multiple_of(qb * TQ + j * LANES, LANES)
                    ot[pl.ds(h0, DHA), pl.ds(q0, LANES)] = (st["accs"][j] / l1).astype(BF16)
                lchk[0] = lo
                lchk[1] = hi

            def unit(kb):
                def f():
                    if kb == 0:
                        setup()
                    if kb < NK:
                        qk(kb)
                    if kb >= A_SKEW:
                        pv(kb - A_SKEW)
                    if kb == NK + A_SKEW - 1:
                        finish()
                return f

            return [unit(kb) for kb in range(NK + A_SKEW)]

        def b_slots(s):
            st = {"qkv": {}, "ps": {}, "os": {}, "outs": [None] * NG}
            r0 = pl.multiple_of(s * SEG, SEG)

            def setup():
                hbuf[M:L, :] = xa[pl.ds(r0, SEG), :].astype(F32)
                st["X"] = hbuf[...]
                row = lax.broadcasted_iota(jnp.int32, (L, L), 0)
                col = lax.broadcasted_iota(jnp.int32, (L, L), 1)
                st["mask"] = (row < M) | (row >= col)

            def proj(h):
                st["qkv"][h] = [_dot(st["X"], pltpu.bitcast(wb[t, h], BF16)) for t in range(3)]

            def qk(h):
                q, k, _ = st["qkv"][h]
                sc = _dot_nt(q, k.astype(BF16)) * bscale
                sc = jnp.where(st["mask"], sc, -1e9)
                m = jnp.max(sc, axis=-1, keepdims=True)
                p = jnp.exp(sc - m)
                st["ps"][h] = p / jnp.sum(p, axis=-1, keepdims=True)

            def pv(h):
                v = st["qkv"].pop(h)[2]
                st["os"][h] = _dot(st["ps"].pop(h), v.astype(BF16))

            def outp(h):
                o = st["os"].pop(h)
                outs = st["outs"]
                for n in range(NG):
                    t = _dot(o, pltpu.bitcast(wob[n, h], BF16))
                    outs[n] = t if outs[n] is None else outs[n] + t
                if h % GRP == GRP - 1:
                    for n in range(NG):
                        if h == GRP - 1:
                            obuf[:, n * LANES:(n + 1) * LANES] = outs[n]
                        else:
                            obuf[:, n * LANES:(n + 1) * LANES] += outs[n]
                        outs[n] = None

            def finish():
                o = obuf[...]
                hbuf[0:M, :] = o[0:M].astype(BF16).astype(F32)
                bbuf[pl.ds(r0, SEG), :] = o[M:L]

            def slot(t):
                def f():
                    if t == 0:
                        setup()
                    if t < HB:
                        proj(t)
                    if 0 <= t - SKEW[0] < HB:
                        qk(t - SKEW[0])
                    if 0 <= t - SKEW[1] < HB:
                        pv(t - SKEW[1])
                    if 0 <= t - SKEW[2] < HB:
                        outp(t - SKEW[2])
                    if t == HB + SKEW[2] - 1:
                        finish()
                return f

            return [slot(t) for t in range(HB + SKEW[2])]

        def main_step(s):
            h = s * QPS // NQ
            qb0 = (s * QPS) % NQ
            units = []
            for i in range(QPS):
                u = a_units(h, qb0 + i)
                for k in range(A_SKEW):
                    if len(units) >= A_SKEW:
                        last = units[len(units) - A_SKEW + k]
                        u[k] = (lambda a=u[k], b=last: (a(), b()))
                if units:
                    units = units[:len(units) - A_SKEW]
                units += u
            slots = b_slots(s)
            ns, nu = len(slots), len(units)
            nd = nu - A_SKEW
            last = ns - A_END - A_SKEW
            pos = [A_START + round(i * (last - A_START) / (nd - 1)) for i in range(nd)]
            pos += [last + 1 + k for k in range(A_SKEW)]
            for t in range(-1, ns):
                if t >= 0:
                    slots[t]()
                for i in range(nu):
                    if min(pos[i], ns - 1) == t:
                        units[i]()

        def main_iter(it, carry):
            for k in range(UNROLL):
                main_step(it * UNROLL + k)
            return carry

        lax.fori_loop(0, NSEG // UNROLL, main_iter, 0)

        ok = jnp.logical_and(lchk[0] >= L_MIN, lchk[1] <= L_MAX)
        n_bad = jnp.sum(jnp.where(ok, 0.0, 1.0))

        @pl.when(n_bad > 0.0)
        def _exact_softmax_fallback():
            def body(it, carry):
                h = it // (S // LANES)
                qb = it % (S // LANES)
                h0 = pl.multiple_of(h * DHA, DHA)
                q0 = pl.multiple_of(qb * LANES, LANES)
                g, qm = head_masked_q(h, q0)
                m = jnp.full((8, LANES), -jnp.inf, F32)
                for kb in range(NK):
                    s = _dot(kk[g, kb * TK:(kb + 1) * TK, :], qm)
                    sbuf[kb * TK:(kb + 1) * TK, :] = s
                    m = jnp.maximum(m, jnp.max(s.reshape(TK // 8, 8, LANES), axis=0))
                m1 = jnp.max(m, axis=0, keepdims=True)
                l = jnp.zeros((8, LANES), F32)
                acc = jnp.zeros((DHA, LANES), F32)
                for kb in range(NK):
                    p = jnp.exp2(sbuf[kb * TK:(kb + 1) * TK, :] - m1)
                    l = l + jnp.sum(p.reshape(TK // 8, 8, LANES), axis=0)
                    acc = acc + _dot(vt[pl.ds(h0, DHA), kb * TK:(kb + 1) * TK], p.astype(BF16))
                l1 = jnp.sum(l, axis=0, keepdims=True)
                ot[pl.ds(h0, DHA), pl.ds(q0, LANES)] = (acc / l1).astype(BF16)
                return carry

            lax.fori_loop(0, HA * (S // LANES), body, 0)

        cp_woa.wait()

        out_cps = []
        for i in range(S // TM):
            r0 = i * TM
            a = _dot_tn(ot[:, r0:r0 + TM], woa[...])
            g = gl[r0:r0 + TM, :]
            for n in range(NG):
                sl = slice(n * LANES, (n + 1) * LANES)
                outv[r0:r0 + TM, sl] = (g * a[:, sl] + (1.0 - g) * bbuf[r0:r0 + TM, sl]).astype(BF16)
            cp = pltpu.make_async_copy(outv.at[r0:r0 + TM, :], out_hbm.at[0, r0:r0 + TM, :], sem_out.at[i])
            cp.start()
            out_cps.append(cp)
        for cp in out_cps:
            cp.wait()

    return kernel


@functools.partial(jax.jit, static_argnames=("B_seg_len",))
def pallas_gated_mix__softmax_full_mha__memory_aug_recurrent_mem_tr__prompt_kernel(
    A_x: jax.Array,
    A_wqkv: jax.Array,
    A_wo: jax.Array,
    B_x: jax.Array,
    B_mem0: jax.Array,
    B_Wq: jax.Array,
    B_Wk: jax.Array,
    B_Wv: jax.Array,
    B_Wo: jax.Array,
    B_seg_len: int,
    gate_w: jax.Array,
):
    del B_x
    _, S, D = A_x.shape
    _, HB, DHB = B_Wq.shape
    M = B_mem0.shape[1]
    SEG = int(B_seg_len)
    NG = D // LANES
    wq, wk, wv = (w.reshape(D // 2, 2 * HB, DHB) for w in (B_Wq, B_Wk, B_Wv))

    any_spec = pl.BlockSpec(memory_space=pl.ANY)
    scratch = [
        pltpu.VMEM((S, D), BF16),
        pltpu.VMEM((D, 3 * D), BF16),
        pltpu.VMEM((D, D), BF16),
        pltpu.VMEM((M, D), BF16),
        pltpu.VMEM((D,), BF16),
        pltpu.VMEM((3, HB, D // 2, DHB), U32),
        pltpu.VMEM((NG, HB, DHB // 2, LANES), U32),
        pltpu.VMEM((NG, LANES, S), BF16),
        pltpu.VMEM((NG, S, LANES), BF16),
        pltpu.VMEM((D, S), BF16),
        pltpu.VMEM((D, S), BF16),
        pltpu.VMEM((NG, 8, LANES), F32),
        pltpu.VMEM((NG, LANES, LANES), F32),
        pltpu.VMEM((2, 8, LANES), F32),
        pltpu.VMEM((S, LANES), F32),
        pltpu.VMEM((S, D), F32),
        pltpu.VMEM((M + SEG, D), F32),
        pltpu.VMEM((M + SEG, D), F32),
        pltpu.VMEM((S, LANES), F32),
        pltpu.VMEM((S, D), BF16),
        pltpu.SemaphoreType.DMA((2,)),
        pltpu.SemaphoreType.DMA((len(WCH),)),
        pltpu.SemaphoreType.DMA((3,)),
        pltpu.SemaphoreType.DMA((3 * HB,)),
        pltpu.SemaphoreType.DMA((NG,)),
        pltpu.SemaphoreType.DMA((S // TM,)),
    ]
    return pl.pallas_call(
        _make_kernel(S, D, HB, DHB, M, SEG),
        out_shape=jax.ShapeDtypeStruct((1, S, D), BF16),
        in_specs=[any_spec] * 9,
        out_specs=any_spec,
        scratch_shapes=scratch,
        compiler_params=pltpu.CompilerParams(vmem_limit_bytes=120 * 1024 * 1024),
        name="gated_mix",
    )(A_x, A_wqkv, A_wo, B_mem0, wq, wk, wv, B_Wo, gate_w)
```

```python
import functools
import math

import jax
import jax.numpy as jnp
from jax import lax
import jax.experimental.pallas as pl
import jax.experimental.pallas.tpu as pltpu

F32 = jnp.float32
BF16 = jnp.bfloat16
U32 = jnp.uint32

LANES = 128
HA = 32
TQ = 512
TK = 256
TM = 256
NSUB = 2
WCH = (2, 4, 8, 10)
REP_RC = 16
L_MIN = 2.0 ** -64
L_MAX = 2.0 ** 64
SKEW = (1, 3, 5)
GRP = 8
A_SKEW = 1
A_END = 4
UNROLL = 2
A_START = 2


def _dot(a, b):
    return lax.dot_general(a, b, (((1,), (0,)), ((), ())), preferred_element_type=F32)


def _dot_nt(a, b):
    return lax.dot_general(a, b, (((1,), (1,)), ((), ())), preferred_element_type=F32)


def _dot_tn(a, b):
    return lax.dot_general(a, b, (((0,), (0,)), ((), ())), preferred_element_type=F32)


def _make_kernel(S, D, HB, DHB, M, SEG):
    DHA = D // HA
    HPG = LANES // DHA
    NG = D // LANES
    L = M + SEG
    NSEG = S // SEG
    NQ = S // TQ
    NK = S // TK
    J = TQ // LANES
    TB = TM * NSUB
    NBLK = S // TB
    NPAIR = HB // 2
    assert sum(WCH) == 3 * NG
    WOFF = [sum(WCH[:k]) for k in range(len(WCH))]
    QPS = HA * NQ // NSEG
    assert QPS * NSEG == HA * NQ and NQ % QPS == 0
    qscale = (DHA ** -0.5) * math.log2(math.e)
    bscale = DHB ** -0.5

    def kernel(xa_hbm, wqkv_hbm, woa_hbm, mem_hbm, wq_hbm, wk_hbm, wv_hbm, wob_hbm, gate_hbm,
               out_hbm,
               xa, wqkv, woa, mem, gate, wb, wob,
               qt, kk, vt, ot, kmax, kmt, lchk, gl, bbuf, hbuf, obuf, sbuf, outv,
               sem_x, sem_wa, sem_in, sem_w, sem_wo, sem_out):
        cp_x0 = pltpu.make_async_copy(xa_hbm.at[0, 0:TB, :], xa.at[0:TB, :], sem_x.at[0])
        cp_xr = pltpu.make_async_copy(xa_hbm.at[0, TB:S, :], xa.at[TB:S, :], sem_x.at[1])
        cp_wa = [pltpu.make_async_copy(wqkv_hbm.at[:, o * LANES:(o + n) * LANES],
                                       wqkv.at[:, o * LANES:(o + n) * LANES], sem_wa.at[k])
                 for k, (o, n) in enumerate(zip(WOFF, WCH))]
        cp_gate = pltpu.make_async_copy(gate_hbm, gate, sem_in.at[0])
        cp_woa = pltpu.make_async_copy(woa_hbm, woa, sem_in.at[1])
        cp_mem = pltpu.make_async_copy(mem_hbm.at[0], mem, sem_in.at[2])

        def w_copies(t):
            src = (wq_hbm, wk_hbm, wv_hbm)[t].bitcast(U32)
            return [pltpu.make_async_copy(src.at[:, r, :], wb.at[t, 2 * (r % NPAIR) + r // NPAIR],
                                          sem_w.at[t * HB + r]) for r in range(HB)]

        w_cps = [w_copies(t) for t in range(3)]
        wob_u = wob_hbm.bitcast(U32)
        wo_cps = [pltpu.make_async_copy(wob_u.at[:, :, n * LANES:(n + 1) * LANES], wob.at[n], sem_wo.at[n])
                  for n in range(NG)]

        hw = HB // 2

        def sync(waits, starts):
            for cp in waits:
                cp.wait()
            for cp in starts:
                cp.start()

        sync0 = {WOFF[1]: ([cp_wa[1]], [cp_xr]),
                 WOFF[2]: ([cp_wa[2]], w_cps[0]),
                 WOFF[3]: ([cp_wa[3]], w_cps[1])}
        sync1 = {0: ([cp_xr], []),
                 2 * NG: (w_cps[0], w_cps[2])}
        sync2 = {NG + NG // 2: (w_cps[1], wo_cps + [cp_mem, cp_woa])}
        sync3 = {NG - 2: (w_cps[2], [])}
        cp_gate.start()
        cp_x0.start()
        cp_wa[0].start()
        cp_wa[1].start()

        kmax[...] = jnp.zeros(kmax.shape, F32)

        def repack(t, j, anchor):
            z = (pltpu.bitcast(anchor, U32) & jnp.uint32(0x7FFF)) >> 15
            for r in range(0, D // 2, REP_RC):
                zz = jnp.concatenate([z] * (REP_RC // 8), axis=0)
                e = wb[t, 2 * j, r:r + REP_RC, :] | zz
                o = wb[t, 2 * j + 1, r:r + REP_RC, :]
                lo = (e & jnp.uint32(0xFFFF)) | (o << 16)
                wb[t, 2 * j, r:r + REP_RC, :] = lo
                wb[t, 2 * j + 1, r:r + REP_RC, :] = (e >> 16) | (o & jnp.uint32(0xFFFF0000))
                z = (lo[0:8, :] & jnp.uint32(0x7FFF)) >> 15

        def a_proj(i, syncs, rep=()):
            rep = list(rep)
            r0s = [i * TB + u * TM for u in range(NSUB)]
            prev = None
            for c in range(3 * NG):
                if c in syncs:
                    sync(*syncs[c])
                    prev = None
                for u in range(NSUB):
                    r0 = r0s[u]
                    xu = xa[r0:r0 + TM, :]
                    r = _dot(xu, wqkv[:, c * LANES:(c + 1) * LANES])
                    if c < NG:
                        qt[c, :, r0:r0 + TM] = (r * qscale).T.astype(BF16)
                    elif c < 2 * NG:
                        g = c - NG
                        rb = r.astype(BF16)
                        kk[g, r0:r0 + TM, :] = rb
                        ab = jnp.abs(rb.astype(F32))
                        kmax[g] = jnp.maximum(kmax[g], jnp.max(ab.reshape(TM // 8, 8, LANES), axis=0))
                    else:
                        g = c - 2 * NG
                        vt[g * LANES:(g + 1) * LANES, r0:r0 + TM] = r.T.astype(BF16)
                    while prev is not None and rep and rep[0][0] <= c * NSUB + u:
                        _, t, j = rep.pop(0)
                        repack(t, j, prev)
                    prev = r[0:8, :]
                    if c == NG + 2 + 4 * u:
                        gv = gate[...].astype(F32).reshape(1, D)
                        logit = jnp.sum(xu.astype(F32) * gv, axis=-1, keepdims=True)
                        gl[r0:r0 + TM, :] = jnp.broadcast_to(jax.nn.sigmoid(logit), (TM, LANES))

        ndots = 3 * NG * NSUB
        sync([cp_gate, cp_x0, cp_wa[0]], [cp_wa[2], cp_wa[3]])
        a_proj(0, sync0)
        a_proj(1, sync1)
        k1 = (NG + NG // 2) * NSUB + 1
        k2 = (NG - 2) * NSUB + 1
        n2 = NPAIR // 2
        a_proj(2, sync2, rep=[(1 + j * (k1 - 2) // NPAIR, 0, j) for j in range(NPAIR)]
               + [(k1 + j * (ndots - k1 - 1) // n2, 1, j) for j in range(n2)])
        a_proj(3, sync3, rep=[(1 + j * (k2 - 2) // (NPAIR - n2), 1, n2 + j) for j in range(NPAIR - n2)]
               + [(k2 + j * (ndots - k2 - 1) // NPAIR, 2, j) for j in range(NPAIR)])

        for g in range(NG):
            km = jnp.max(kmax[g], axis=0, keepdims=True)
            kmt[g] = jnp.broadcast_to(km, (LANES, LANES)).T

        lchk[...] = jnp.zeros((8, LANES), F32)

        for c in wo_cps:
            c.wait()
        cp_mem.wait()
        hbuf[0:M, :] = mem[...].astype(F32)

        def head_masked_q(h, q0):
            g = h // HPG
            r = h % HPG
            rows = lax.broadcasted_iota(jnp.int32, (LANES, LANES), 0)
            msk = (rows >= r * DHA) & (rows < r * DHA + DHA)
            q = qt[g, :, pl.ds(q0, LANES)]
            return g, jnp.where(msk, q, jnp.zeros_like(q))

        def a_units(h, qb):
            st = {}
            h0 = pl.multiple_of(h * DHA, DHA)

            def setup():
                st["qms"], st["bnd"] = [], []
                for j in range(J):
                    q0 = pl.multiple_of(qb * TQ + j * LANES, LANES)
                    g, qm = head_masked_q(h, q0)
                    st["g"] = g
                    st["qms"].append(qm)
                    bb = jnp.abs(qm.astype(F32)) * kmt[g]
                    bb = jnp.sum(bb, axis=0, keepdims=True) * (1.0 + 2.0 ** -10)
                    st["bnd"].append(jnp.broadcast_to(bb, (8, LANES)))
                st["ls"] = [jnp.zeros((8, LANES), F32) for _ in range(J)]
                st["accs"] = [jnp.zeros((DHA, LANES), F32) for _ in range(J)]
                st["ps"] = {}

            def qk(kb):
                kblk = kk[st["g"], kb * TK:(kb + 1) * TK, :]
                for j in range(J):
                    s = _dot(kblk, st["qms"][j]).reshape(TK // 8, 8, LANES)
                    p = jnp.exp2(s - st["bnd"][j][None])
                    st["ls"][j] = st["ls"][j] + jnp.sum(p, axis=0)
                    st["ps"][(kb, j)] = p.reshape(TK, LANES).astype(BF16)

            def pv(kb):
                vblk = vt[pl.ds(h0, DHA), kb * TK:(kb + 1) * TK]
                for j in range(J):
                    st["accs"][j] = st["accs"][j] + _dot(vblk, st["ps"].pop((kb, j)))

            def finish():
                bad = lchk[...]
                for j in range(J):
                    l1 = jnp.sum(st["ls"][j], axis=0, keepdims=True)
                    l8 = jnp.broadcast_to(l1, (8, LANES))
                    bad = jnp.where(jnp.logical_and(l8 >= L_MIN, l8 <= L_MAX), bad, 1.0)
                    q0 = pl.multiple_of(qb * TQ + j * LANES, LANES)
                    ot[pl.ds(h0, DHA), pl.ds(q0, LANES)] = (st["accs"][j] / l1).astype(BF16)
                lchk[...] = bad

            def unit(kb):
                def f():
                    if kb == 0:
                        setup()
                    if kb < NK:
                        qk(kb)
                    if kb >= A_SKEW:
                        pv(kb - A_SKEW)
                    if kb == NK + A_SKEW - 1:
                        finish()
                return f

            return [unit(kb) for kb in range(NK + A_SKEW)]

        def b_slots(s):
            st = {"qkv": {}, "ps": {}, "os": {}, "outs": [None] * NG}
            r0 = pl.multiple_of(s * SEG, SEG)

            def setup():
                hbuf[M:L, :] = xa[pl.ds(r0, SEG), :].astype(F32)
                st["X"] = hbuf[...]
                row = lax.broadcasted_iota(jnp.int32, (L, L), 0)
                col = lax.broadcasted_iota(jnp.int32, (L, L), 1)
                st["mask"] = (row < M) | (row >= col)

            def proj(h):
                st["qkv"][h] = [_dot(st["X"], pltpu.bitcast(wb[t, h], BF16)) for t in range(3)]

            def qk(h):
                q, k, _ = st["qkv"][h]
                sc = _dot_nt(q, k.astype(BF16)) * bscale
                sc = jnp.where(st["mask"], sc, -1e9)
                m = jnp.max(sc, axis=-1, keepdims=True)
                p = jnp.exp(sc - m)
                st["ps"][h] = p / jnp.sum(p, axis=-1, keepdims=True)

            def pv(h):
                v = st["qkv"].pop(h)[2]
                st["os"][h] = _dot(st["ps"].pop(h), v.astype(BF16))

            def outp(h):
                o = st["os"].pop(h)
                outs = st["outs"]
                for n in range(NG):
                    t = _dot(o, pltpu.bitcast(wob[n, h], BF16))
                    outs[n] = t if outs[n] is None else outs[n] + t
                if h % GRP == GRP - 1:
                    for n in range(NG):
                        if h == GRP - 1:
                            obuf[:, n * LANES:(n + 1) * LANES] = outs[n]
                        else:
                            obuf[:, n * LANES:(n + 1) * LANES] += outs[n]
                        outs[n] = None

            def finish():
                o = obuf[...]
                hbuf[0:M, :] = o[0:M].astype(BF16).astype(F32)
                bbuf[pl.ds(r0, SEG), :] = o[M:L]

            def slot(t):
                def f():
                    if t == 0:
                        setup()
                    if t < HB:
                        proj(t)
                    if 0 <= t - SKEW[0] < HB:
                        qk(t - SKEW[0])
                    if 0 <= t - SKEW[1] < HB:
                        pv(t - SKEW[1])
                    if 0 <= t - SKEW[2] < HB:
                        outp(t - SKEW[2])
                    if t == HB + SKEW[2] - 1:
                        finish()
                return f

            return [slot(t) for t in range(HB + SKEW[2])]

        def main_step(s):
            h = s * QPS // NQ
            qb0 = (s * QPS) % NQ
            units = []
            for i in range(QPS):
                u = a_units(h, qb0 + i)
                for k in range(A_SKEW):
                    if len(units) >= A_SKEW:
                        last = units[len(units) - A_SKEW + k]
                        u[k] = (lambda a=u[k], b=last: (a(), b()))
                if units:
                    units = units[:len(units) - A_SKEW]
                units += u
            slots = b_slots(s)
            ns, nu = len(slots), len(units)
            nd = nu - A_SKEW
            last = ns - A_END - A_SKEW
            pos = [A_START + round(i * (last - A_START) / (nd - 1)) for i in range(nd)]
            pos += [last + 1 + k for k in range(A_SKEW)]
            for t in range(-1, ns):
                if t >= 0:
                    slots[t]()
                for i in range(nu):
                    if min(pos[i], ns - 1) == t:
                        units[i]()

        def main_iter(it, carry):
            for k in range(UNROLL):
                main_step(it * UNROLL + k)
            return carry

        lax.fori_loop(0, NSEG // UNROLL, main_iter, 0)

        @pl.when(jnp.max(lchk[...]) > 0.0)
        def _exact_softmax_fallback():
            def body(it, carry):
                h = it // (S // LANES)
                qb = it % (S // LANES)
                h0 = pl.multiple_of(h * DHA, DHA)
                q0 = pl.multiple_of(qb * LANES, LANES)
                g, qm = head_masked_q(h, q0)
                m = jnp.full((8, LANES), -jnp.inf, F32)
                for kb in range(NK):
                    s = _dot(kk[g, kb * TK:(kb + 1) * TK, :], qm)
                    sbuf[kb * TK:(kb + 1) * TK, :] = s
                    m = jnp.maximum(m, jnp.max(s.reshape(TK // 8, 8, LANES), axis=0))
                m1 = jnp.max(m, axis=0, keepdims=True)
                l = jnp.zeros((8, LANES), F32)
                acc = jnp.zeros((DHA, LANES), F32)
                for kb in range(NK):
                    p = jnp.exp2(sbuf[kb * TK:(kb + 1) * TK, :] - m1)
                    l = l + jnp.sum(p.reshape(TK // 8, 8, LANES), axis=0)
                    acc = acc + _dot(vt[pl.ds(h0, DHA), kb * TK:(kb + 1) * TK], p.astype(BF16))
                l1 = jnp.sum(l, axis=0, keepdims=True)
                ot[pl.ds(h0, DHA), pl.ds(q0, LANES)] = (acc / l1).astype(BF16)
                return carry

            lax.fori_loop(0, HA * (S // LANES), body, 0)

        cp_woa.wait()

        out_cps = []
        for i in range(S // TM):
            r0 = i * TM
            a = _dot_tn(ot[:, r0:r0 + TM], woa[...])
            g = gl[r0:r0 + TM, :]
            for n in range(NG):
                sl = slice(n * LANES, (n + 1) * LANES)
                outv[r0:r0 + TM, sl] = (g * a[:, sl] + (1.0 - g) * bbuf[r0:r0 + TM, sl]).astype(BF16)
            cp = pltpu.make_async_copy(outv.at[r0:r0 + TM, :], out_hbm.at[0, r0:r0 + TM, :], sem_out.at[i])
            cp.start()
            out_cps.append(cp)
        for cp in out_cps:
            cp.wait()

    return kernel


@functools.partial(jax.jit, static_argnames=("B_seg_len",))
def pallas_gated_mix__softmax_full_mha__memory_aug_recurrent_mem_tr__prompt_kernel(
    A_x: jax.Array,
    A_wqkv: jax.Array,
    A_wo: jax.Array,
    B_x: jax.Array,
    B_mem0: jax.Array,
    B_Wq: jax.Array,
    B_Wk: jax.Array,
    B_Wv: jax.Array,
    B_Wo: jax.Array,
    B_seg_len: int,
    gate_w: jax.Array,
):
    del B_x
    _, S, D = A_x.shape
    _, HB, DHB = B_Wq.shape
    M = B_mem0.shape[1]
    SEG = int(B_seg_len)
    NG = D // LANES
    wq, wk, wv = (w.reshape(D // 2, 2 * HB, DHB) for w in (B_Wq, B_Wk, B_Wv))

    any_spec = pl.BlockSpec(memory_space=pl.ANY)
    scratch = [
        pltpu.VMEM((S, D), BF16),
        pltpu.VMEM((D, 3 * D), BF16),
        pltpu.VMEM((D, D), BF16),
        pltpu.VMEM((M, D), BF16),
        pltpu.VMEM((D,), BF16),
        pltpu.VMEM((3, HB, D // 2, DHB), U32),
        pltpu.VMEM((NG, HB, DHB // 2, LANES), U32),
        pltpu.VMEM((NG, LANES, S), BF16),
        pltpu.VMEM((NG, S, LANES), BF16),
        pltpu.VMEM((D, S), BF16),
        pltpu.VMEM((D, S), BF16),
        pltpu.VMEM((NG, 8, LANES), F32),
        pltpu.VMEM((NG, LANES, LANES), F32),
        pltpu.VMEM((8, LANES), F32),
        pltpu.VMEM((S, LANES), F32),
        pltpu.VMEM((S, D), F32),
        pltpu.VMEM((M + SEG, D), F32),
        pltpu.VMEM((M + SEG, D), F32),
        pltpu.VMEM((S, LANES), F32),
        pltpu.VMEM((S, D), BF16),
        pltpu.SemaphoreType.DMA((2,)),
        pltpu.SemaphoreType.DMA((len(WCH),)),
        pltpu.SemaphoreType.DMA((3,)),
        pltpu.SemaphoreType.DMA((3 * HB,)),
        pltpu.SemaphoreType.DMA((NG,)),
        pltpu.SemaphoreType.DMA((S // TM,)),
    ]
    return pl.pallas_call(
        _make_kernel(S, D, HB, DHB, M, SEG),
        out_shape=jax.ShapeDtypeStruct((1, S, D), BF16),
        in_specs=[any_spec] * 9,
        out_specs=any_spec,
        scratch_shapes=scratch,
        compiler_params=pltpu.CompilerParams(vmem_limit_bytes=120 * 1024 * 1024),
        name="gated_mix",
    )(A_x, A_wqkv, A_wo, B_mem0, wq, wk, wv, B_Wo, gate_w)
```

```python
import functools
import math

import jax
import jax.numpy as jnp
from jax import lax
import jax.experimental.pallas as pl
import jax.experimental.pallas.tpu as pltpu

F32 = jnp.float32
BF16 = jnp.bfloat16
U32 = jnp.uint32

LANES = 128
HA = 32
TQ = 512
TK = 256
TM = 256
NSUB = 2
WCH = (2, 4, 8, 10)
REP_RC = 16
L_MIN = 2.0 ** -64
L_MAX = 2.0 ** 64
SKEW = (1, 3, 5)
GRP = 8
A_SKEW = 1
A_END = (1, 3)
UNROLL = 2
A_START = (2, 2)


def _dot(a, b):
    return lax.dot_general(a, b, (((1,), (0,)), ((), ())), preferred_element_type=F32)


def _dot_nt(a, b):
    return lax.dot_general(a, b, (((1,), (1,)), ((), ())), preferred_element_type=F32)


def _dot_tn(a, b):
    return lax.dot_general(a, b, (((0,), (0,)), ((), ())), preferred_element_type=F32)


def _make_kernel(S, D, HB, DHB, M, SEG):
    DHA = D // HA
    HPG = LANES // DHA
    NG = D // LANES
    L = M + SEG
    NSEG = S // SEG
    NQ = S // TQ
    NK = S // TK
    J = TQ // LANES
    TB = TM * NSUB
    NBLK = S // TB
    NPAIR = HB // 2
    assert sum(WCH) == 3 * NG
    WOFF = [sum(WCH[:k]) for k in range(len(WCH))]
    QPS = HA * NQ // NSEG
    assert QPS * NSEG == HA * NQ and NQ % QPS == 0
    qscale = (DHA ** -0.5) * math.log2(math.e)
    bscale = DHB ** -0.5

    def kernel(xa_hbm, wqkv_hbm, woa_hbm, mem_hbm, wq_hbm, wk_hbm, wv_hbm, wob_hbm, gate_hbm,
               out_hbm,
               xa, wqkv, woa, mem, gate, wb, wob,
               qt, kk, vt, ot, kmax, kmt, lchk, gl, bbuf, hbuf, obuf, sbuf, outv,
               sem_x, sem_wa, sem_in, sem_w, sem_wo, sem_out):
        cp_x0 = pltpu.make_async_copy(xa_hbm.at[0, 0:TB, :], xa.at[0:TB, :], sem_x.at[0])
        cp_xr = pltpu.make_async_copy(xa_hbm.at[0, TB:S, :], xa.at[TB:S, :], sem_x.at[1])
        cp_wa = [pltpu.make_async_copy(wqkv_hbm.at[:, o * LANES:(o + n) * LANES],
                                       wqkv.at[:, o * LANES:(o + n) * LANES], sem_wa.at[k])
                 for k, (o, n) in enumerate(zip(WOFF, WCH))]
        cp_gate = pltpu.make_async_copy(gate_hbm, gate, sem_in.at[0])
        cp_woa = pltpu.make_async_copy(woa_hbm, woa, sem_in.at[1])
        cp_mem = pltpu.make_async_copy(mem_hbm.at[0], mem, sem_in.at[2])

        def w_copies(t):
            src = (wq_hbm, wk_hbm, wv_hbm)[t].bitcast(U32)
            return [pltpu.make_async_copy(src.at[:, r, :], wb.at[t, 2 * (r % NPAIR) + r // NPAIR],
                                          sem_w.at[t * HB + r]) for r in range(HB)]

        w_cps = [w_copies(t) for t in range(3)]
        wob_u = wob_hbm.bitcast(U32)
        wo_cps = [pltpu.make_async_copy(wob_u.at[:, :, n * LANES:(n + 1) * LANES], wob.at[n], sem_wo.at[n])
                  for n in range(NG)]

        hw = HB // 2

        def sync(waits, starts):
            for cp in waits:
                cp.wait()
            for cp in starts:
                cp.start()

        sync0 = {WOFF[1]: ([cp_wa[1]], [cp_xr]),
                 WOFF[2]: ([cp_wa[2]], w_cps[0]),
                 WOFF[3]: ([cp_wa[3]], w_cps[1])}
        sync1 = {0: ([cp_xr], []),
                 2 * NG: (w_cps[0], w_cps[2])}
        sync2 = {NG + NG // 2: (w_cps[1], wo_cps + [cp_mem, cp_woa])}
        sync3 = {NG - 2: (w_cps[2], [])}
        cp_gate.start()
        cp_x0.start()
        cp_wa[0].start()
        cp_wa[1].start()

        kmax[...] = jnp.zeros(kmax.shape, F32)

        def repack(t, j, anchor):
            z = (pltpu.bitcast(anchor, U32) & jnp.uint32(0x7FFF)) >> 15
            for r in range(0, D // 2, REP_RC):
                zz = jnp.concatenate([z] * (REP_RC // 8), axis=0)
                e = wb[t, 2 * j, r:r + REP_RC, :] | zz
                o = wb[t, 2 * j + 1, r:r + REP_RC, :]
                lo = (e & jnp.uint32(0xFFFF)) | (o << 16)
                wb[t, 2 * j, r:r + REP_RC, :] = lo
                wb[t, 2 * j + 1, r:r + REP_RC, :] = (e >> 16) | (o & jnp.uint32(0xFFFF0000))
                z = (lo[0:8, :] & jnp.uint32(0x7FFF)) >> 15

        def a_proj(i, syncs, rep=()):
            rep = list(rep)
            r0s = [i * TB + u * TM for u in range(NSUB)]
            prev = None
            for c in range(3 * NG):
                if c in syncs:
                    sync(*syncs[c])
                    prev = None
                for u in range(NSUB):
                    r0 = r0s[u]
                    xu = xa[r0:r0 + TM, :]
                    r = _dot(xu, wqkv[:, c * LANES:(c + 1) * LANES])
                    if c < NG:
                        qt[c, :, r0:r0 + TM] = (r * qscale).T.astype(BF16)
                    elif c < 2 * NG:
                        g = c - NG
                        rb = r.astype(BF16)
                        kk[g, r0:r0 + TM, :] = rb
                        ab = jnp.abs(rb.astype(F32))
                        kmax[g] = jnp.maximum(kmax[g], jnp.max(ab.reshape(TM // 8, 8, LANES), axis=0))
                    else:
                        g = c - 2 * NG
                        vt[g * LANES:(g + 1) * LANES, r0:r0 + TM] = r.T.astype(BF16)
                    while prev is not None and rep and rep[0][0] <= c * NSUB + u:
                        _, t, j = rep.pop(0)
                        repack(t, j, prev)
                    prev = r[0:8, :]
                    if c == NG + 2 + 4 * u:
                        gv = gate[...].astype(F32).reshape(1, D)
                        logit = jnp.sum(xu.astype(F32) * gv, axis=-1, keepdims=True)
                        gl[r0:r0 + TM, :] = jnp.broadcast_to(jax.nn.sigmoid(logit), (TM, LANES))

        ndots = 3 * NG * NSUB
        sync([cp_gate, cp_x0, cp_wa[0]], [cp_wa[2], cp_wa[3]])
        a_proj(0, sync0)
        a_proj(1, sync1)
        k1 = (NG + NG // 2) * NSUB + 1
        k2 = (NG - 2) * NSUB + 1
        n2 = NPAIR // 2
        a_proj(2, sync2, rep=[(1 + j * (k1 - 2) // NPAIR, 0, j) for j in range(NPAIR)]
               + [(k1 + j * (ndots - k1 - 1) // n2, 1, j) for j in range(n2)])
        a_proj(3, sync3, rep=[(1 + j * (k2 - 2) // (NPAIR - n2), 1, n2 + j) for j in range(NPAIR - n2)]
               + [(k2 + j * (ndots - k2 - 1) // NPAIR, 2, j) for j in range(NPAIR)])

        for g in range(NG):
            km = jnp.max(kmax[g], axis=0, keepdims=True)
            kmt[g] = jnp.broadcast_to(km, (LANES, LANES)).T

        lchk[...] = jnp.zeros((8, LANES), F32)

        for c in wo_cps:
            c.wait()
        cp_mem.wait()
        hbuf[0:M, :] = mem[...].astype(F32)

        def head_masked_q(h, q0):
            g = h // HPG
            r = h % HPG
            rows = lax.broadcasted_iota(jnp.int32, (LANES, LANES), 0)
            msk = (rows >= r * DHA) & (rows < r * DHA + DHA)
            q = qt[g, :, pl.ds(q0, LANES)]
            return g, jnp.where(msk, q, jnp.zeros_like(q))

        def a_units(h, qb):
            st = {}
            h0 = pl.multiple_of(h * DHA, DHA)

            def setup():
                st["qms"], st["bnd"] = [], []
                for j in range(J):
                    q0 = pl.multiple_of(qb * TQ + j * LANES, LANES)
                    g, qm = head_masked_q(h, q0)
                    st["g"] = g
                    st["qms"].append(qm)
                    bb = jnp.abs(qm.astype(F32)) * kmt[g]
                    bb = jnp.sum(bb, axis=0, keepdims=True) * (1.0 + 2.0 ** -10)
                    st["bnd"].append(jnp.broadcast_to(bb, (8, LANES)))
                st["ls"] = [jnp.zeros((8, LANES), F32) for _ in range(J)]
                st["accs"] = [jnp.zeros((DHA, LANES), F32) for _ in range(J)]
                st["ps"] = {}

            def qk(kb):
                kblk = kk[st["g"], kb * TK:(kb + 1) * TK, :]
                for j in range(J):
                    s = _dot(kblk, st["qms"][j]).reshape(TK // 8, 8, LANES)
                    p = jnp.exp2(s - st["bnd"][j][None])
                    st["ls"][j] = st["ls"][j] + jnp.sum(p, axis=0)
                    st["ps"][(kb, j)] = p.reshape(TK, LANES).astype(BF16)

            def pv(kb):
                vblk = vt[pl.ds(h0, DHA), kb * TK:(kb + 1) * TK]
                for j in range(J):
                    st["accs"][j] = st["accs"][j] + _dot(vblk, st["ps"].pop((kb, j)))

            def finish():
                bad = lchk[...]
                for j in range(J):
                    l1 = jnp.sum(st["ls"][j], axis=0, keepdims=True)
                    l8 = jnp.broadcast_to(l1, (8, LANES))
                    bad = jnp.where(jnp.logical_and(l8 >= L_MIN, l8 <= L_MAX), bad, 1.0)
                    q0 = pl.multiple_of(qb * TQ + j * LANES, LANES)
                    ot[pl.ds(h0, DHA), pl.ds(q0, LANES)] = (st["accs"][j] / l1).astype(BF16)
                lchk[...] = bad

            def unit(kb):
                def f():
                    if kb == 0:
                        setup()
                    if kb < NK:
                        qk(kb)
                    if kb >= A_SKEW:
                        pv(kb - A_SKEW)
                    if kb == NK + A_SKEW - 1:
                        finish()
                return f

            return [unit(kb) for kb in range(NK + A_SKEW)]

        def b_slots(s):
            st = {"qkv": {}, "ps": {}, "os": {}, "outs": [None] * NG}
            r0 = pl.multiple_of(s * SEG, SEG)

            def setup():
                hbuf[M:L, :] = xa[pl.ds(r0, SEG), :].astype(F32)
                st["X"] = hbuf[...]
                row = lax.broadcasted_iota(jnp.int32, (L, L), 0)
                col = lax.broadcasted_iota(jnp.int32, (L, L), 1)
                st["mask"] = (row < M) | (row >= col)

            def proj(h):
                st["qkv"][h] = [_dot(st["X"], pltpu.bitcast(wb[t, h], BF16)) for t in range(3)]

            def qk(h):
                q, k, _ = st["qkv"][h]
                sc = _dot_nt(q, k.astype(BF16)) * bscale
                sc = jnp.where(st["mask"], sc, -1e9)
                m = jnp.max(sc, axis=-1, keepdims=True)
                p = jnp.exp(sc - m)
                st["ps"][h] = p / jnp.sum(p, axis=-1, keepdims=True)

            def pv(h):
                v = st["qkv"].pop(h)[2]
                st["os"][h] = _dot(st["ps"].pop(h), v.astype(BF16))

            def outp(h):
                o = st["os"].pop(h)
                outs = st["outs"]
                for n in range(NG):
                    t = _dot(o, pltpu.bitcast(wob[n, h], BF16))
                    outs[n] = t if outs[n] is None else outs[n] + t
                if h % GRP == GRP - 1:
                    for n in range(NG):
                        if h == GRP - 1:
                            obuf[:, n * LANES:(n + 1) * LANES] = outs[n]
                        else:
                            obuf[:, n * LANES:(n + 1) * LANES] += outs[n]
                        outs[n] = None

            def finish():
                o = obuf[...]
                hbuf[0:M, :] = o[0:M].astype(BF16).astype(F32)
                bbuf[pl.ds(r0, SEG), :] = o[M:L]

            def slot(t):
                def f():
                    if t == 0:
                        setup()
                    if t < HB:
                        proj(t)
                    if 0 <= t - SKEW[0] < HB:
                        qk(t - SKEW[0])
                    if 0 <= t - SKEW[1] < HB:
                        pv(t - SKEW[1])
                    if 0 <= t - SKEW[2] < HB:
                        outp(t - SKEW[2])
                    if t == HB + SKEW[2] - 1:
                        finish()
                return f

            return [slot(t) for t in range(HB + SKEW[2])]

        def main_step(s, a_start, a_end):
            h = s * QPS // NQ
            qb0 = (s * QPS) % NQ
            units = []
            for i in range(QPS):
                u = a_units(h, qb0 + i)
                for k in range(A_SKEW):
                    if len(units) >= A_SKEW:
                        last = units[len(units) - A_SKEW + k]
                        u[k] = (lambda a=u[k], b=last: (a(), b()))
                if units:
                    units = units[:len(units) - A_SKEW]
                units += u
            slots = b_slots(s)
            ns, nu = len(slots), len(units)
            nd = nu - A_SKEW
            last = ns - a_end - A_SKEW
            pos = [a_start + round(i * (last - a_start) / (nd - 1)) for i in range(nd)]
            pos += [last + 1 + k for k in range(A_SKEW)]
            for t in range(-1, ns):
                if t >= 0:
                    slots[t]()
                for i in range(nu):
                    if min(pos[i], ns - 1) == t:
                        units[i]()

        def main_iter(it, carry):
            for k in range(UNROLL):
                main_step(it * UNROLL + k, A_START[k], A_END[k])
            return carry

        lax.fori_loop(0, NSEG // UNROLL, main_iter, 0)

        @pl.when(jnp.max(lchk[...]) > 0.0)
        def _exact_softmax_fallback():
            def body(it, carry):
                h = it // (S // LANES)
                qb = it % (S // LANES)
                h0 = pl.multiple_of(h * DHA, DHA)
                q0 = pl.multiple_of(qb * LANES, LANES)
                g, qm = head_masked_q(h, q0)
                m = jnp.full((8, LANES), -jnp.inf, F32)
                for kb in range(NK):
                    s = _dot(kk[g, kb * TK:(kb + 1) * TK, :], qm)
                    sbuf[kb * TK:(kb + 1) * TK, :] = s
                    m = jnp.maximum(m, jnp.max(s.reshape(TK // 8, 8, LANES), axis=0))
                m1 = jnp.max(m, axis=0, keepdims=True)
                l = jnp.zeros((8, LANES), F32)
                acc = jnp.zeros((DHA, LANES), F32)
                for kb in range(NK):
                    p = jnp.exp2(sbuf[kb * TK:(kb + 1) * TK, :] - m1)
                    l = l + jnp.sum(p.reshape(TK // 8, 8, LANES), axis=0)
                    acc = acc + _dot(vt[pl.ds(h0, DHA), kb * TK:(kb + 1) * TK], p.astype(BF16))
                l1 = jnp.sum(l, axis=0, keepdims=True)
                ot[pl.ds(h0, DHA), pl.ds(q0, LANES)] = (acc / l1).astype(BF16)
                return carry

            lax.fori_loop(0, HA * (S // LANES), body, 0)

        cp_woa.wait()

        out_cps = []
        for i in range(S // TM):
            r0 = i * TM
            a = _dot_tn(ot[:, r0:r0 + TM], woa[...])
            g = gl[r0:r0 + TM, :]
            for n in range(NG):
                sl = slice(n * LANES, (n + 1) * LANES)
                outv[r0:r0 + TM, sl] = (g * a[:, sl] + (1.0 - g) * bbuf[r0:r0 + TM, sl]).astype(BF16)
            cp = pltpu.make_async_copy(outv.at[r0:r0 + TM, :], out_hbm.at[0, r0:r0 + TM, :], sem_out.at[i])
            cp.start()
            out_cps.append(cp)
        for cp in out_cps:
            cp.wait()

    return kernel


@functools.partial(jax.jit, static_argnames=("B_seg_len",))
def pallas_gated_mix__softmax_full_mha__memory_aug_recurrent_mem_tr__prompt_kernel(
    A_x: jax.Array,
    A_wqkv: jax.Array,
    A_wo: jax.Array,
    B_x: jax.Array,
    B_mem0: jax.Array,
    B_Wq: jax.Array,
    B_Wk: jax.Array,
    B_Wv: jax.Array,
    B_Wo: jax.Array,
    B_seg_len: int,
    gate_w: jax.Array,
):
    del B_x
    _, S, D = A_x.shape
    _, HB, DHB = B_Wq.shape
    M = B_mem0.shape[1]
    SEG = int(B_seg_len)
    NG = D // LANES
    wq, wk, wv = (w.reshape(D // 2, 2 * HB, DHB) for w in (B_Wq, B_Wk, B_Wv))

    any_spec = pl.BlockSpec(memory_space=pl.ANY)
    scratch = [
        pltpu.VMEM((S, D), BF16),
        pltpu.VMEM((D, 3 * D), BF16),
        pltpu.VMEM((D, D), BF16),
        pltpu.VMEM((M, D), BF16),
        pltpu.VMEM((D,), BF16),
        pltpu.VMEM((3, HB, D // 2, DHB), U32),
        pltpu.VMEM((NG, HB, DHB // 2, LANES), U32),
        pltpu.VMEM((NG, LANES, S), BF16),
        pltpu.VMEM((NG, S, LANES), BF16),
        pltpu.VMEM((D, S), BF16),
        pltpu.VMEM((D, S), BF16),
        pltpu.VMEM((NG, 8, LANES), F32),
        pltpu.VMEM((NG, LANES, LANES), F32),
        pltpu.VMEM((8, LANES), F32),
        pltpu.VMEM((S, LANES), F32),
        pltpu.VMEM((S, D), F32),
        pltpu.VMEM((M + SEG, D), F32),
        pltpu.VMEM((M + SEG, D), F32),
        pltpu.VMEM((S, LANES), F32),
        pltpu.VMEM((S, D), BF16),
        pltpu.SemaphoreType.DMA((2,)),
        pltpu.SemaphoreType.DMA((len(WCH),)),
        pltpu.SemaphoreType.DMA((3,)),
        pltpu.SemaphoreType.DMA((3 * HB,)),
        pltpu.SemaphoreType.DMA((NG,)),
        pltpu.SemaphoreType.DMA((S // TM,)),
    ]
    return pl.pallas_call(
        _make_kernel(S, D, HB, DHB, M, SEG),
        out_shape=jax.ShapeDtypeStruct((1, S, D), BF16),
        in_specs=[any_spec] * 9,
        out_specs=any_spec,
        scratch_shapes=scratch,
        compiler_params=pltpu.CompilerParams(vmem_limit_bytes=120 * 1024 * 1024),
        name="gated_mix",
    )(A_x, A_wqkv, A_wo, B_mem0, wq, wk, wv, B_Wo, gate_w)
```

```python
import functools
import math

import jax
import jax.numpy as jnp
from jax import lax
import jax.experimental.pallas as pl
import jax.experimental.pallas.tpu as pltpu

F32 = jnp.float32
BF16 = jnp.bfloat16
U32 = jnp.uint32

LANES = 128
HA = 32
TQ = 512
TK = 256
TM = 256
NSUB = 2
WCH = (2, 3, 5, 6, 8)
REP_RC = 16
L_MIN = 2.0 ** -64
L_MAX = 2.0 ** 64
SKEW = (1, 3, 5)
GRP = 8
A_SKEW = 1
A_END = (1, 3)
UNROLL = 2
A_START = (2, 2)


def _dot(a, b):
    return lax.dot_general(a, b, (((1,), (0,)), ((), ())), preferred_element_type=F32)


def _dot_nt(a, b):
    return lax.dot_general(a, b, (((1,), (1,)), ((), ())), preferred_element_type=F32)


def _dot_tn(a, b):
    return lax.dot_general(a, b, (((0,), (0,)), ((), ())), preferred_element_type=F32)


def _make_kernel(S, D, HB, DHB, M, SEG):
    DHA = D // HA
    HPG = LANES // DHA
    NG = D // LANES
    L = M + SEG
    NSEG = S // SEG
    NQ = S // TQ
    NK = S // TK
    J = TQ // LANES
    TB = TM * NSUB
    NBLK = S // TB
    NPAIR = HB // 2
    assert sum(WCH) == 3 * NG
    WOFF = [sum(WCH[:k]) for k in range(len(WCH))]
    QPS = HA * NQ // NSEG
    assert QPS * NSEG == HA * NQ and NQ % QPS == 0
    qscale = (DHA ** -0.5) * math.log2(math.e)
    bscale = DHB ** -0.5

    def kernel(xa_hbm, wqkv_hbm, woa_hbm, mem_hbm, wq_hbm, wk_hbm, wv_hbm, wob_hbm, gate_hbm,
               out_hbm,
               xa, wqkv, woa, mem, gate, wb, wob,
               qt, kk, vt, ot, kmax, kmt, lchk, gl, bbuf, hbuf, obuf, sbuf, outv,
               sem_x, sem_wa, sem_in, sem_w, sem_wo, sem_out):
        cp_x0 = [pltpu.make_async_copy(xa_hbm.at[0, u * TM:(u + 1) * TM, :], xa.at[u * TM:(u + 1) * TM, :],
                                       sem_x.at[u]) for u in range(NSUB)]
        cp_xr = pltpu.make_async_copy(xa_hbm.at[0, TB:S, :], xa.at[TB:S, :], sem_x.at[NSUB])
        cp_wa = [pltpu.make_async_copy(wqkv_hbm.at[:, o * LANES:(o + n) * LANES],
                                       wqkv.at[:, o * LANES:(o + n) * LANES], sem_wa.at[k])
                 for k, (o, n) in enumerate(zip(WOFF, WCH))]
        cp_gate = pltpu.make_async_copy(gate_hbm, gate, sem_in.at[0])
        cp_woa = pltpu.make_async_copy(woa_hbm, woa, sem_in.at[1])
        cp_mem = pltpu.make_async_copy(mem_hbm.at[0], mem, sem_in.at[2])

        def w_copies(t):
            src = (wq_hbm, wk_hbm, wv_hbm)[t].bitcast(U32)
            return [pltpu.make_async_copy(src.at[:, r, :], wb.at[t, 2 * (r % NPAIR) + r // NPAIR],
                                          sem_w.at[t * HB + r]) for r in range(HB)]

        w_cps = [w_copies(t) for t in range(3)]
        wob_u = wob_hbm.bitcast(U32)
        wo_cps = [pltpu.make_async_copy(wob_u.at[:, :, n * LANES:(n + 1) * LANES], wob.at[n], sem_wo.at[n])
                  for n in range(NG)]

        def sync(waits, starts):
            for cp in waits:
                cp.wait()
            for cp in starts:
                cp.start()

        nwa = len(cp_wa)
        sync0 = {WOFF[k] * NSUB: ([cp_wa[k]], []) for k in range(1, nwa)}
        sync0[WCH[0]] = (cp_x0[1:], cp_wa[3:4])
        for k in range(4, nwa):
            sync0[WOFF[k - 3] * NSUB][1].append(cp_wa[k])
        sync0[WOFF[nwa - 3] * NSUB][1].append(cp_xr)
        sync0[WOFF[nwa - 2] * NSUB][0].append(cp_gate)
        sync0[WOFF[nwa - 2] * NSUB][1].extend(w_cps[0])
        sync0[WOFF[nwa - 1] * NSUB][1].extend(w_cps[1])
        sync1 = {0: ([cp_xr], []),
                 2 * NG * NSUB: (w_cps[0], w_cps[2])}
        sync2 = {(NG + NG // 2) * NSUB: (w_cps[1], wo_cps + [cp_mem, cp_woa])}
        sync3 = {(NG - 2) * NSUB: (w_cps[2], [])}
        cp_x0[0].start()
        cp_wa[0].start()
        for cp in cp_x0[1:]:
            cp.start()
        cp_wa[1].start()

        kmax[...] = jnp.zeros(kmax.shape, F32)

        def repack(t, j, anchor):
            z = (pltpu.bitcast(anchor, U32) & jnp.uint32(0x7FFF)) >> 15
            for r in range(0, D // 2, REP_RC):
                zz = jnp.concatenate([z] * (REP_RC // 8), axis=0)
                e = wb[t, 2 * j, r:r + REP_RC, :] | zz
                o = wb[t, 2 * j + 1, r:r + REP_RC, :]
                lo = (e & jnp.uint32(0xFFFF)) | (o << 16)
                wb[t, 2 * j, r:r + REP_RC, :] = lo
                wb[t, 2 * j + 1, r:r + REP_RC, :] = (e >> 16) | (o & jnp.uint32(0xFFFF0000))
                z = (lo[0:8, :] & jnp.uint32(0x7FFF)) >> 15

        def a_proj(i, syncs, rep=(), order=None):
            rep = list(rep)
            prev = None
            if order is None:
                order = [(c, u) for c in range(3 * NG) for u in range(NSUB)]
            for idx, (c, u) in enumerate(order):
                if idx in syncs:
                    sync(*syncs[idx])
                    prev = None
                r0 = i * TB + u * TM
                xu = xa[r0:r0 + TM, :]
                r = _dot(xu, wqkv[:, c * LANES:(c + 1) * LANES])
                if c < NG:
                    qt[c, :, r0:r0 + TM] = (r * qscale).T.astype(BF16)
                elif c < 2 * NG:
                    g = c - NG
                    rb = r.astype(BF16)
                    kk[g, r0:r0 + TM, :] = rb
                    ab = jnp.abs(rb.astype(F32))
                    kmax[g] = jnp.maximum(kmax[g], jnp.max(ab.reshape(TM // 8, 8, LANES), axis=0))
                else:
                    g = c - 2 * NG
                    vt[g * LANES:(g + 1) * LANES, r0:r0 + TM] = r.T.astype(BF16)
                while prev is not None and rep and rep[0][0] <= idx:
                    _, t, j = rep.pop(0)
                    repack(t, j, prev)
                prev = r[0:8, :]
                if c == NG + 2 + 4 * u:
                    gv = gate[...].astype(F32).reshape(1, D)
                    logit = jnp.sum(xu.astype(F32) * gv, axis=-1, keepdims=True)
                    gl[r0:r0 + TM, :] = jnp.broadcast_to(jax.nn.sigmoid(logit), (TM, LANES))

        ndots = 3 * NG * NSUB
        sync([cp_x0[0], cp_wa[0]], [cp_wa[2], cp_gate])
        order0 = ([(c, u) for u in range(NSUB) for c in range(WCH[0])]
                  + [(c, u) for c in range(WCH[0], 3 * NG) for u in range(NSUB)])
        a_proj(0, sync0, order=order0)
        a_proj(1, sync1)
        k1 = (NG + NG // 2) * NSUB + 1
        k2 = (NG - 2) * NSUB + 1
        n2 = NPAIR // 2
        a_proj(2, sync2, rep=[(1 + j * (k1 - 2) // NPAIR, 0, j) for j in range(NPAIR)]
               + [(k1 + j * (ndots - k1 - 1) // n2, 1, j) for j in range(n2)])
        a_proj(3, sync3, rep=[(1 + j * (k2 - 2) // (NPAIR - n2), 1, n2 + j) for j in range(NPAIR - n2)]
               + [(k2 + j * (ndots - k2 - 1) // NPAIR, 2, j) for j in range(NPAIR)])

        for g in range(NG):
            km = jnp.max(kmax[g], axis=0, keepdims=True)
            kmt[g] = jnp.broadcast_to(km, (LANES, LANES)).T

        lchk[...] = jnp.zeros((8, LANES), F32)

        for c in wo_cps:
            c.wait()
        cp_mem.wait()
        hbuf[0:M, :] = mem[...].astype(F32)

        def head_masked_q(h, q0):
            g = h // HPG
            r = h % HPG
            rows = lax.broadcasted_iota(jnp.int32, (LANES, LANES), 0)
            msk = (rows >= r * DHA) & (rows < r * DHA + DHA)
            q = qt[g, :, pl.ds(q0, LANES)]
            return g, jnp.where(msk, q, jnp.zeros_like(q))

        def a_units(h, qb):
            st = {}
            h0 = pl.multiple_of(h * DHA, DHA)

            def setup():
                st["qms"], st["bnd"] = [], []
                for j in range(J):
                    q0 = pl.multiple_of(qb * TQ + j * LANES, LANES)
                    g, qm = head_masked_q(h, q0)
                    st["g"] = g
                    st["qms"].append(qm)
                    bb = jnp.abs(qm.astype(F32)) * kmt[g]
                    bb = jnp.sum(bb, axis=0, keepdims=True) * (1.0 + 2.0 ** -10)
                    st["bnd"].append(jnp.broadcast_to(bb, (8, LANES)))
                st["ls"] = [jnp.zeros((8, LANES), F32) for _ in range(J)]
                st["accs"] = [jnp.zeros((DHA, LANES), F32) for _ in range(J)]
                st["ps"] = {}

            def qk(kb):
                kblk = kk[st["g"], kb * TK:(kb + 1) * TK, :]
                for j in range(J):
                    s = _dot(kblk, st["qms"][j]).reshape(TK // 8, 8, LANES)
                    p = jnp.exp2(s - st["bnd"][j][None])
                    st["ls"][j] = st["ls"][j] + jnp.sum(p, axis=0)
                    st["ps"][(kb, j)] = p.reshape(TK, LANES).astype(BF16)

            def pv(kb):
                vblk = vt[pl.ds(h0, DHA), kb * TK:(kb + 1) * TK]
                for j in range(J):
                    st["accs"][j] = st["accs"][j] + _dot(vblk, st["ps"].pop((kb, j)))

            def finish():
                bad = lchk[...]
                for j in range(J):
                    l1 = jnp.sum(st["ls"][j], axis=0, keepdims=True)
                    l8 = jnp.broadcast_to(l1, (8, LANES))
                    bad = jnp.where(jnp.logical_and(l8 >= L_MIN, l8 <= L_MAX), bad, 1.0)
                    q0 = pl.multiple_of(qb * TQ + j * LANES, LANES)
                    ot[pl.ds(h0, DHA), pl.ds(q0, LANES)] = (st["accs"][j] / l1).astype(BF16)
                lchk[...] = bad

            def unit(kb):
                def f():
                    if kb == 0:
                        setup()
                    if kb < NK:
                        qk(kb)
                    if kb >= A_SKEW:
                        pv(kb - A_SKEW)
                    if kb == NK + A_SKEW - 1:
                        finish()
                return f

            return [unit(kb) for kb in range(NK + A_SKEW)]

        def b_slots(s):
            st = {"qkv": {}, "ps": {}, "os": {}, "outs": [None] * NG}
            r0 = pl.multiple_of(s * SEG, SEG)

            def setup():
                hbuf[M:L, :] = xa[pl.ds(r0, SEG), :].astype(F32)
                st["X"] = hbuf[...]
                row = lax.broadcasted_iota(jnp.int32, (L, L), 0)
                col = lax.broadcasted_iota(jnp.int32, (L, L), 1)
                st["mask"] = (row < M) | (row >= col)

            def proj(h):
                st["qkv"][h] = [_dot(st["X"], pltpu.bitcast(wb[t, h], BF16)) for t in range(3)]

            def qk(h):
                q, k, _ = st["qkv"][h]
                sc = _dot_nt(q, k.astype(BF16)) * bscale
                sc = jnp.where(st["mask"], sc, -1e9)
                m = jnp.max(sc, axis=-1, keepdims=True)
                p = jnp.exp(sc - m)
                st["ps"][h] = p / jnp.sum(p, axis=-1, keepdims=True)

            def pv(h):
                v = st["qkv"].pop(h)[2]
                st["os"][h] = _dot(st["ps"].pop(h), v.astype(BF16))

            def outp(h):
                o = st["os"].pop(h)
                outs = st["outs"]
                for n in range(NG):
                    t = _dot(o, pltpu.bitcast(wob[n, h], BF16))
                    outs[n] = t if outs[n] is None else outs[n] + t
                if h % GRP == GRP - 1:
                    for n in range(NG):
                        if h == GRP - 1:
                            obuf[:, n * LANES:(n + 1) * LANES] = outs[n]
                        else:
                            obuf[:, n * LANES:(n + 1) * LANES] += outs[n]
                        outs[n] = None

            def finish():
                o = obuf[...]
                hbuf[0:M, :] = o[0:M].astype(BF16).astype(F32)
                bbuf[pl.ds(r0, SEG), :] = o[M:L]

            def slot(t):
                def f():
                    if t == 0:
                        setup()
                    if t < HB:
                        proj(t)
                    if 0 <= t - SKEW[0] < HB:
                        qk(t - SKEW[0])
                    if 0 <= t - SKEW[1] < HB:
                        pv(t - SKEW[1])
                    if 0 <= t - SKEW[2] < HB:
                        outp(t - SKEW[2])
                    if t == HB + SKEW[2] - 1:
                        finish()
                return f

            return [slot(t) for t in range(HB + SKEW[2])]

        def main_step(s, a_start, a_end):
            h = s * QPS // NQ
            qb0 = (s * QPS) % NQ
            units = []
            for i in range(QPS):
                u = a_units(h, qb0 + i)
                for k in range(A_SKEW):
                    if len(units) >= A_SKEW:
                        last = units[len(units) - A_SKEW + k]
                        u[k] = (lambda a=u[k], b=last: (a(), b()))
                if units:
                    units = units[:len(units) - A_SKEW]
                units += u
            slots = b_slots(s)
            ns, nu = len(slots), len(units)
            nd = nu - A_SKEW
            last = ns - a_end - A_SKEW
            pos = [a_start + round(i * (last - a_start) / (nd - 1)) for i in range(nd)]
            pos += [last + 1 + k for k in range(A_SKEW)]
            for t in range(-1, ns):
                if t >= 0:
                    slots[t]()
                for i in range(nu):
                    if min(pos[i], ns - 1) == t:
                        units[i]()

        def main_iter(it, carry):
            for k in range(UNROLL):
                main_step(it * UNROLL + k, A_START[k], A_END[k])
            return carry

        lax.fori_loop(0, NSEG // UNROLL, main_iter, 0)

        @pl.when(jnp.max(lchk[...]) > 0.0)
        def _exact_softmax_fallback():
            def body(it, carry):
                h = it // (S // LANES)
                qb = it % (S // LANES)
                h0 = pl.multiple_of(h * DHA, DHA)
                q0 = pl.multiple_of(qb * LANES, LANES)
                g, qm = head_masked_q(h, q0)
                m = jnp.full((8, LANES), -jnp.inf, F32)
                for kb in range(NK):
                    s = _dot(kk[g, kb * TK:(kb + 1) * TK, :], qm)
                    sbuf[kb * TK:(kb + 1) * TK, :] = s
                    m = jnp.maximum(m, jnp.max(s.reshape(TK // 8, 8, LANES), axis=0))
                m1 = jnp.max(m, axis=0, keepdims=True)
                l = jnp.zeros((8, LANES), F32)
                acc = jnp.zeros((DHA, LANES), F32)
                for kb in range(NK):
                    p = jnp.exp2(sbuf[kb * TK:(kb + 1) * TK, :] - m1)
                    l = l + jnp.sum(p.reshape(TK // 8, 8, LANES), axis=0)
                    acc = acc + _dot(vt[pl.ds(h0, DHA), kb * TK:(kb + 1) * TK], p.astype(BF16))
                l1 = jnp.sum(l, axis=0, keepdims=True)
                ot[pl.ds(h0, DHA), pl.ds(q0, LANES)] = (acc / l1).astype(BF16)
                return carry

            lax.fori_loop(0, HA * (S // LANES), body, 0)

        cp_woa.wait()

        out_cps = []
        for i in range(S // TM):
            r0 = i * TM
            a = _dot_tn(ot[:, r0:r0 + TM], woa[...])
            g = gl[r0:r0 + TM, :]
            for n in range(NG):
                sl = slice(n * LANES, (n + 1) * LANES)
                outv[r0:r0 + TM, sl] = (g * a[:, sl] + (1.0 - g) * bbuf[r0:r0 + TM, sl]).astype(BF16)
            cp = pltpu.make_async_copy(outv.at[r0:r0 + TM, :], out_hbm.at[0, r0:r0 + TM, :], sem_out.at[i])
            cp.start()
            out_cps.append(cp)
        for cp in out_cps:
            cp.wait()

    return kernel


@functools.partial(jax.jit, static_argnames=("B_seg_len",))
def pallas_gated_mix__softmax_full_mha__memory_aug_recurrent_mem_tr__prompt_kernel(
    A_x: jax.Array,
    A_wqkv: jax.Array,
    A_wo: jax.Array,
    B_x: jax.Array,
    B_mem0: jax.Array,
    B_Wq: jax.Array,
    B_Wk: jax.Array,
    B_Wv: jax.Array,
    B_Wo: jax.Array,
    B_seg_len: int,
    gate_w: jax.Array,
):
    del B_x
    _, S, D = A_x.shape
    _, HB, DHB = B_Wq.shape
    M = B_mem0.shape[1]
    SEG = int(B_seg_len)
    NG = D // LANES
    wq, wk, wv = (w.reshape(D // 2, 2 * HB, DHB) for w in (B_Wq, B_Wk, B_Wv))

    any_spec = pl.BlockSpec(memory_space=pl.ANY)
    scratch = [
        pltpu.VMEM((S, D), BF16),
        pltpu.VMEM((D, 3 * D), BF16),
        pltpu.VMEM((D, D), BF16),
        pltpu.VMEM((M, D), BF16),
        pltpu.VMEM((D,), BF16),
        pltpu.VMEM((3, HB, D // 2, DHB), U32),
        pltpu.VMEM((NG, HB, DHB // 2, LANES), U32),
        pltpu.VMEM((NG, LANES, S), BF16),
        pltpu.VMEM((NG, S, LANES), BF16),
        pltpu.VMEM((D, S), BF16),
        pltpu.VMEM((D, S), BF16),
        pltpu.VMEM((NG, 8, LANES), F32),
        pltpu.VMEM((NG, LANES, LANES), F32),
        pltpu.VMEM((8, LANES), F32),
        pltpu.VMEM((S, LANES), F32),
        pltpu.VMEM((S, D), F32),
        pltpu.VMEM((M + SEG, D), F32),
        pltpu.VMEM((M + SEG, D), F32),
        pltpu.VMEM((S, LANES), F32),
        pltpu.VMEM((S, D), BF16),
        pltpu.SemaphoreType.DMA((NSUB + 1,)),
        pltpu.SemaphoreType.DMA((len(WCH),)),
        pltpu.SemaphoreType.DMA((3,)),
        pltpu.SemaphoreType.DMA((3 * HB,)),
        pltpu.SemaphoreType.DMA((NG,)),
        pltpu.SemaphoreType.DMA((S // TM,)),
    ]
    return pl.pallas_call(
        _make_kernel(S, D, HB, DHB, M, SEG),
        out_shape=jax.ShapeDtypeStruct((1, S, D), BF16),
        in_specs=[any_spec] * 9,
        out_specs=any_spec,
        scratch_shapes=scratch,
        compiler_params=pltpu.CompilerParams(vmem_limit_bytes=120 * 1024 * 1024),
        name="gated_mix",
    )(A_x, A_wqkv, A_wo, B_mem0, wq, wk, wv, B_Wo, gate_w)
```

```python
import functools
import math

import jax
import jax.numpy as jnp
from jax import lax
import jax.experimental.pallas as pl
import jax.experimental.pallas.tpu as pltpu

F32 = jnp.float32
BF16 = jnp.bfloat16
U32 = jnp.uint32

LANES = 128
HA = 32
TQ = 512
TK = 256
TM = 256
NSUB = 2
WCH = (2, 3, 5, 6, 8)
REP_RC = 16
L_MIN = 2.0 ** -64
L_MAX = 2.0 ** 64
SKEW = (1, 3, 5)
GRP = 8
A_SKEW = 1
A_END = (1, 3)
UNROLL = 2
A_START = (2, 2)


def _dot(a, b):
    return lax.dot_general(a, b, (((1,), (0,)), ((), ())), preferred_element_type=F32)


def _dot_nt(a, b):
    return lax.dot_general(a, b, (((1,), (1,)), ((), ())), preferred_element_type=F32)


def _dot_tn(a, b):
    return lax.dot_general(a, b, (((0,), (0,)), ((), ())), preferred_element_type=F32)


def _make_kernel(S, D, HB, DHB, M, SEG):
    DHA = D // HA
    HPG = LANES // DHA
    NG = D // LANES
    L = M + SEG
    NSEG = S // SEG
    NQ = S // TQ
    NK = S // TK
    J = TQ // LANES
    TB = TM * NSUB
    NBLK = S // TB
    NPAIR = HB // 2
    assert sum(WCH) == 3 * NG
    WOFF = [sum(WCH[:k]) for k in range(len(WCH))]
    QPS = HA * NQ // NSEG
    assert QPS * NSEG == HA * NQ and NQ % QPS == 0
    qscale = (DHA ** -0.5) * math.log2(math.e)
    bscale = DHB ** -0.5

    def kernel(xa_hbm, wqkv_hbm, woa_hbm, mem_hbm, wq_hbm, wk_hbm, wv_hbm, wob_hbm, gate_hbm,
               out_hbm,
               xa, wqkv, woa, mem, gate, wb, wob,
               qt, kk, vt, ot, kmax, kmt, lchk, gl, bbuf, hbuf, obuf, sbuf, outv,
               sem_x, sem_wa, sem_in, sem_w, sem_wo, sem_out):
        cp_x0 = [pltpu.make_async_copy(xa_hbm.at[0, u * TM:(u + 1) * TM, :], xa.at[u * TM:(u + 1) * TM, :],
                                       sem_x.at[u]) for u in range(NSUB)]
        cp_xr = pltpu.make_async_copy(xa_hbm.at[0, TB:S, :], xa.at[TB:S, :], sem_x.at[NSUB])
        cp_wa = [pltpu.make_async_copy(wqkv_hbm.at[:, o * LANES:(o + n) * LANES],
                                       wqkv.at[:, o * LANES:(o + n) * LANES], sem_wa.at[k])
                 for k, (o, n) in enumerate(zip(WOFF, WCH))]
        cp_gate = pltpu.make_async_copy(gate_hbm, gate, sem_in.at[0])
        cp_woa = pltpu.make_async_copy(woa_hbm, woa, sem_in.at[1])
        cp_mem = pltpu.make_async_copy(mem_hbm.at[0], mem, sem_in.at[2])

        def w_copies(t):
            src = (wq_hbm, wk_hbm, wv_hbm)[t].bitcast(U32)
            return [pltpu.make_async_copy(src.at[:, r, :], wb.at[t, 2 * (r % NPAIR) + r // NPAIR],
                                          sem_w.at[t * HB + r]) for r in range(HB)]

        w_cps = [w_copies(t) for t in range(3)]
        wob_u = wob_hbm.bitcast(U32)
        wo_cps = [pltpu.make_async_copy(wob_u.at[:, :, n * LANES:(n + 1) * LANES], wob.at[n], sem_wo.at[n])
                  for n in range(NG)]

        def sync(waits, starts):
            for cp in waits:
                cp.wait()
            for cp in starts:
                cp.start()

        nwa = len(cp_wa)
        sync0 = {WOFF[k] * NSUB: ([cp_wa[k]], []) for k in range(1, nwa)}
        sync0[WCH[0]] = (cp_x0[1:], cp_wa[3:4])
        for k in range(4, nwa):
            sync0[WOFF[k - 3] * NSUB][1].append(cp_wa[k])
        sync0[WOFF[nwa - 3] * NSUB][1].append(cp_xr)
        sync0[WOFF[nwa - 2] * NSUB][0].append(cp_gate)
        sync0[WOFF[nwa - 2] * NSUB][1].extend(w_cps[0])
        sync0[WOFF[nwa - 1] * NSUB][1].extend(w_cps[1])
        sync1 = {0: ([cp_xr], []),
                 2 * NG * NSUB: (w_cps[0], w_cps[2])}
        sync2 = {(NG + NG // 2) * NSUB: (w_cps[1], wo_cps + [cp_mem, cp_woa])}
        sync3 = {(NG - 2) * NSUB: (w_cps[2], [])}
        cp_x0[0].start()
        cp_wa[0].start()
        for cp in cp_x0[1:]:
            cp.start()
        cp_wa[1].start()

        kmax[...] = jnp.zeros(kmax.shape, F32)

        def repack(t, j, anchor):
            z = (pltpu.bitcast(anchor, U32) & jnp.uint32(0x7FFF)) >> 15
            for r in range(0, D // 2, REP_RC):
                zz = jnp.concatenate([z] * (REP_RC // 8), axis=0)
                e = wb[t, 2 * j, r:r + REP_RC, :] | zz
                o = wb[t, 2 * j + 1, r:r + REP_RC, :]
                lo = (e & jnp.uint32(0xFFFF)) | (o << 16)
                wb[t, 2 * j, r:r + REP_RC, :] = lo
                wb[t, 2 * j + 1, r:r + REP_RC, :] = (e >> 16) | (o & jnp.uint32(0xFFFF0000))
                z = (lo[0:8, :] & jnp.uint32(0x7FFF)) >> 15

        def a_proj(i, syncs, rep=(), order=None):
            rep = list(rep)
            prev = None
            if order is None:
                order = [(c, u) for c in range(3 * NG) for u in range(NSUB)]
            for idx, (c, u) in enumerate(order):
                if idx in syncs:
                    sync(*syncs[idx])
                    prev = None
                r0 = i * TB + u * TM
                xu = xa[r0:r0 + TM, :]
                r = _dot(xu, wqkv[:, c * LANES:(c + 1) * LANES])
                if c < NG:
                    qt[c, :, r0:r0 + TM] = (r * qscale).T.astype(BF16)
                elif c < 2 * NG:
                    g = c - NG
                    rb = r.astype(BF16)
                    kk[g, r0:r0 + TM, :] = rb
                    ab = jnp.abs(rb.astype(F32))
                    km = jnp.maximum(kmax[g], jnp.max(ab.reshape(TM // 8, 8, LANES), axis=0))
                    kmax[g] = km
                    if i == NBLK - 1 and u == NSUB - 1:
                        km = jnp.max(km, axis=0, keepdims=True)
                        kmt[g] = jnp.broadcast_to(km, (LANES, LANES)).T
                else:
                    g = c - 2 * NG
                    vt[g * LANES:(g + 1) * LANES, r0:r0 + TM] = r.T.astype(BF16)
                while prev is not None and rep and rep[0][0] <= idx:
                    _, t, j = rep.pop(0)
                    repack(t, j, prev)
                prev = r[0:8, :]
                if c == NG + 2 + 4 * u:
                    gv = gate[...].astype(F32).reshape(1, D)
                    logit = jnp.sum(xu.astype(F32) * gv, axis=-1, keepdims=True)
                    gl[r0:r0 + TM, :] = jnp.broadcast_to(jax.nn.sigmoid(logit), (TM, LANES))

        ndots = 3 * NG * NSUB
        sync([cp_x0[0], cp_wa[0]], [cp_wa[2], cp_gate])
        order0 = ([(c, u) for u in range(NSUB) for c in range(WCH[0])]
                  + [(c, u) for c in range(WCH[0], 3 * NG) for u in range(NSUB)])
        a_proj(0, sync0, order=order0)
        a_proj(1, sync1)
        k1 = (NG + NG // 2) * NSUB + 1
        k2 = (NG - 2) * NSUB + 1
        n2 = NPAIR // 2
        a_proj(2, sync2, rep=[(1 + j * (k1 - 2) // NPAIR, 0, j) for j in range(NPAIR)]
               + [(k1 + j * (ndots - k1 - 1) // n2, 1, j) for j in range(n2)])
        a_proj(3, sync3, rep=[(1 + j * (k2 - 2) // (NPAIR - n2), 1, n2 + j) for j in range(NPAIR - n2)]
               + [(k2 + j * (ndots - k2 - 1) // NPAIR, 2, j) for j in range(NPAIR)])

        lchk[...] = jnp.zeros((8, LANES), F32)

        for c in wo_cps:
            c.wait()
        cp_mem.wait()
        hbuf[0:M, :] = mem[...].astype(F32)

        def head_masked_q(h, q0):
            g = h // HPG
            r = h % HPG
            rows = lax.broadcasted_iota(jnp.int32, (LANES, LANES), 0)
            msk = (rows >= r * DHA) & (rows < r * DHA + DHA)
            q = qt[g, :, pl.ds(q0, LANES)]
            return g, jnp.where(msk, q, jnp.zeros_like(q))

        def a_units(h, qb):
            st = {}
            h0 = pl.multiple_of(h * DHA, DHA)

            def setup():
                st["qms"], st["bnd"] = [], []
                for j in range(J):
                    q0 = pl.multiple_of(qb * TQ + j * LANES, LANES)
                    g, qm = head_masked_q(h, q0)
                    st["g"] = g
                    st["qms"].append(qm)
                    bb = jnp.abs(qm.astype(F32)) * kmt[g]
                    bb = jnp.sum(bb, axis=0, keepdims=True) * (1.0 + 2.0 ** -10)
                    st["bnd"].append(jnp.broadcast_to(bb, (8, LANES)))
                st["ls"] = [jnp.zeros((8, LANES), F32) for _ in range(J)]
                st["accs"] = [jnp.zeros((DHA, LANES), F32) for _ in range(J)]
                st["ps"] = {}

            def qk(kb):
                kblk = kk[st["g"], kb * TK:(kb + 1) * TK, :]
                for j in range(J):
                    s = _dot(kblk, st["qms"][j]).reshape(TK // 8, 8, LANES)
                    p = jnp.exp2(s - st["bnd"][j][None])
                    st["ls"][j] = st["ls"][j] + jnp.sum(p, axis=0)
                    st["ps"][(kb, j)] = p.reshape(TK, LANES).astype(BF16)

            def pv(kb):
                vblk = vt[pl.ds(h0, DHA), kb * TK:(kb + 1) * TK]
                for j in range(J):
                    st["accs"][j] = st["accs"][j] + _dot(vblk, st["ps"].pop((kb, j)))

            def finish():
                bad = lchk[...]
                for j in range(J):
                    l1 = jnp.sum(st["ls"][j], axis=0, keepdims=True)
                    l8 = jnp.broadcast_to(l1, (8, LANES))
                    bad = jnp.where(jnp.logical_and(l8 >= L_MIN, l8 <= L_MAX), bad, 1.0)
                    q0 = pl.multiple_of(qb * TQ + j * LANES, LANES)
                    ot[pl.ds(h0, DHA), pl.ds(q0, LANES)] = (st["accs"][j] / l1).astype(BF16)
                lchk[...] = bad

            def unit(kb):
                def f():
                    if kb == 0:
                        setup()
                    if kb < NK:
                        qk(kb)
                    if kb >= A_SKEW:
                        pv(kb - A_SKEW)
                    if kb == NK + A_SKEW - 1:
                        finish()
                return f

            return [unit(kb) for kb in range(NK + A_SKEW)]

        def b_slots(s):
            st = {"qkv": {}, "ps": {}, "os": {}, "outs": [None] * NG}
            r0 = pl.multiple_of(s * SEG, SEG)

            def setup():
                hbuf[M:L, :] = xa[pl.ds(r0, SEG), :].astype(F32)
                st["X"] = hbuf[...]
                row = lax.broadcasted_iota(jnp.int32, (L, L), 0)
                col = lax.broadcasted_iota(jnp.int32, (L, L), 1)
                st["mask"] = (row < M) | (row >= col)

            def proj(h):
                st["qkv"][h] = [_dot(st["X"], pltpu.bitcast(wb[t, h], BF16)) for t in range(3)]

            def qk(h):
                q, k, _ = st["qkv"][h]
                sc = _dot_nt(q, k.astype(BF16)) * bscale
                sc = jnp.where(st["mask"], sc, -1e9)
                m = jnp.max(sc, axis=-1, keepdims=True)
                p = jnp.exp(sc - m)
                st["ps"][h] = p / jnp.sum(p, axis=-1, keepdims=True)

            def pv(h):
                v = st["qkv"].pop(h)[2]
                st["os"][h] = _dot(st["ps"].pop(h), v.astype(BF16))

            def outp(h):
                o = st["os"].pop(h)
                outs = st["outs"]
                for n in range(NG):
                    t = _dot(o, pltpu.bitcast(wob[n, h], BF16))
                    outs[n] = t if outs[n] is None else outs[n] + t
                if h % GRP == GRP - 1:
                    for n in range(NG):
                        if h == GRP - 1:
                            obuf[:, n * LANES:(n + 1) * LANES] = outs[n]
                        else:
                            obuf[:, n * LANES:(n + 1) * LANES] += outs[n]
                        outs[n] = None

            def finish():
                o = obuf[...]
                hbuf[0:M, :] = o[0:M].astype(BF16).astype(F32)
                bbuf[pl.ds(r0, SEG), :] = o[M:L]

            def slot(t):
                def f():
                    if t == 0:
                        setup()
                    if t < HB:
                        proj(t)
                    if 0 <= t - SKEW[0] < HB:
                        qk(t - SKEW[0])
                    if 0 <= t - SKEW[1] < HB:
                        pv(t - SKEW[1])
                    if 0 <= t - SKEW[2] < HB:
                        outp(t - SKEW[2])
                    if t == HB + SKEW[2] - 1:
                        finish()
                return f

            return [slot(t) for t in range(HB + SKEW[2])]

        def main_step(s, a_start, a_end):
            h = s * QPS // NQ
            qb0 = (s * QPS) % NQ
            units = []
            for i in range(QPS):
                u = a_units(h, qb0 + i)
                for k in range(A_SKEW):
                    if len(units) >= A_SKEW:
                        last = units[len(units) - A_SKEW + k]
                        u[k] = (lambda a=u[k], b=last: (a(), b()))
                if units:
                    units = units[:len(units) - A_SKEW]
                units += u
            slots = b_slots(s)
            ns, nu = len(slots), len(units)
            nd = nu - A_SKEW
            last = ns - a_end - A_SKEW
            pos = [a_start + round(i * (last - a_start) / (nd - 1)) for i in range(nd)]
            pos += [last + 1 + k for k in range(A_SKEW)]
            for t in range(-1, ns):
                if t >= 0:
                    slots[t]()
                for i in range(nu):
                    if min(pos[i], ns - 1) == t:
                        units[i]()

        def main_iter(it, carry):
            for k in range(UNROLL):
                main_step(it * UNROLL + k, A_START[k], A_END[k])
            return carry

        lax.fori_loop(0, NSEG // UNROLL, main_iter, 0)

        @pl.when(jnp.max(lchk[...]) > 0.0)
        def _exact_softmax_fallback():
            def body(it, carry):
                h = it // (S // LANES)
                qb = it % (S // LANES)
                h0 = pl.multiple_of(h * DHA, DHA)
                q0 = pl.multiple_of(qb * LANES, LANES)
                g, qm = head_masked_q(h, q0)
                m = jnp.full((8, LANES), -jnp.inf, F32)
                for kb in range(NK):
                    s = _dot(kk[g, kb * TK:(kb + 1) * TK, :], qm)
                    sbuf[kb * TK:(kb + 1) * TK, :] = s
                    m = jnp.maximum(m, jnp.max(s.reshape(TK // 8, 8, LANES), axis=0))
                m1 = jnp.max(m, axis=0, keepdims=True)
                l = jnp.zeros((8, LANES), F32)
                acc = jnp.zeros((DHA, LANES), F32)
                for kb in range(NK):
                    p = jnp.exp2(sbuf[kb * TK:(kb + 1) * TK, :] - m1)
                    l = l + jnp.sum(p.reshape(TK // 8, 8, LANES), axis=0)
                    acc = acc + _dot(vt[pl.ds(h0, DHA), kb * TK:(kb + 1) * TK], p.astype(BF16))
                l1 = jnp.sum(l, axis=0, keepdims=True)
                ot[pl.ds(h0, DHA), pl.ds(q0, LANES)] = (acc / l1).astype(BF16)
                return carry

            lax.fori_loop(0, HA * (S // LANES), body, 0)

        cp_woa.wait()

        out_cps = []
        bounds = list(range(0, S - TM + 1, TM)) + [S - TM // 2, S]
        for i in range(len(bounds) - 1):
            r0, r1 = bounds[i], bounds[i + 1]
            a = _dot_tn(ot[:, r0:r1], woa[...])
            g = gl[r0:r1, :]
            for n in range(NG):
                sl = slice(n * LANES, (n + 1) * LANES)
                outv[r0:r1, sl] = (g * a[:, sl] + (1.0 - g) * bbuf[r0:r1, sl]).astype(BF16)
            cp = pltpu.make_async_copy(outv.at[r0:r1, :], out_hbm.at[0, r0:r1, :], sem_out.at[i])
            cp.start()
            out_cps.append(cp)
        for cp in out_cps:
            cp.wait()

    return kernel


@functools.partial(jax.jit, static_argnames=("B_seg_len",))
def pallas_gated_mix__softmax_full_mha__memory_aug_recurrent_mem_tr__prompt_kernel(
    A_x: jax.Array,
    A_wqkv: jax.Array,
    A_wo: jax.Array,
    B_x: jax.Array,
    B_mem0: jax.Array,
    B_Wq: jax.Array,
    B_Wk: jax.Array,
    B_Wv: jax.Array,
    B_Wo: jax.Array,
    B_seg_len: int,
    gate_w: jax.Array,
):
    del B_x
    _, S, D = A_x.shape
    _, HB, DHB = B_Wq.shape
    M = B_mem0.shape[1]
    SEG = int(B_seg_len)
    NG = D // LANES
    wq, wk, wv = (w.reshape(D // 2, 2 * HB, DHB) for w in (B_Wq, B_Wk, B_Wv))

    any_spec = pl.BlockSpec(memory_space=pl.ANY)
    scratch = [
        pltpu.VMEM((S, D), BF16),
        pltpu.VMEM((D, 3 * D), BF16),
        pltpu.VMEM((D, D), BF16),
        pltpu.VMEM((M, D), BF16),
        pltpu.VMEM((D,), BF16),
        pltpu.VMEM((3, HB, D // 2, DHB), U32),
        pltpu.VMEM((NG, HB, DHB // 2, LANES), U32),
        pltpu.VMEM((NG, LANES, S), BF16),
        pltpu.VMEM((NG, S, LANES), BF16),
        pltpu.VMEM((D, S), BF16),
        pltpu.VMEM((D, S), BF16),
        pltpu.VMEM((NG, 8, LANES), F32),
        pltpu.VMEM((NG, LANES, LANES), F32),
        pltpu.VMEM((8, LANES), F32),
        pltpu.VMEM((S, LANES), F32),
        pltpu.VMEM((S, D), F32),
        pltpu.VMEM((M + SEG, D), F32),
        pltpu.VMEM((M + SEG, D), F32),
        pltpu.VMEM((S, LANES), F32),
        pltpu.VMEM((S, D), BF16),
        pltpu.SemaphoreType.DMA((NSUB + 1,)),
        pltpu.SemaphoreType.DMA((len(WCH),)),
        pltpu.SemaphoreType.DMA((3,)),
        pltpu.SemaphoreType.DMA((3 * HB,)),
        pltpu.SemaphoreType.DMA((NG,)),
        pltpu.SemaphoreType.DMA((S // TM + 1,)),
    ]
    return pl.pallas_call(
        _make_kernel(S, D, HB, DHB, M, SEG),
        out_shape=jax.ShapeDtypeStruct((1, S, D), BF16),
        in_specs=[any_spec] * 9,
        out_specs=any_spec,
        scratch_shapes=scratch,
        compiler_params=pltpu.CompilerParams(vmem_limit_bytes=120 * 1024 * 1024),
        name="gated_mix",
    )(A_x, A_wqkv, A_wo, B_mem0, wq, wk, wv, B_Wo, gate_w)
```
